```python
import jax
import jax.numpy as jnp

def _softmax(x, axis=-1):
    return jax.nn.softmax(x, axis=axis)

def _gelu(x):
    return jax.nn.gelu(x, approximate=True)

def _silu(x):
    return jax.nn.silu(x)

def _sigmoid(x):
    return jax.nn.sigmoid(x)

def _layernorm(x, axis=-1, eps=1e-05):
    m = jnp.mean(x, axis=axis, keepdims=True)
    v = jnp.var(x, axis=axis, keepdims=True)
    return (x - m) / jnp.sqrt(v + eps)

def _scatter_add(tgt, idx, src, axis=0):
    return tgt.at[idx].add(src)

def _segment_sum(src, seg, n):
    return jax.ops.segment_sum(src, seg, n)

class _Rng:

    def __init__(self, key):
        self._k = key

    def _next(self):
        self._k, sub = jax.random.split(self._k)
        return sub

    def normal(self, shape):
        return jax.random.normal(self._next(), shape, dtype=jnp.bfloat16)

    def randint(self, lo, hi, shape):
        return jax.random.randint(self._next(), shape, lo, hi, dtype=jnp.int32)

    def uniform(self, shape, lo=0.0, hi=1.0):
        return jax.random.uniform(self._next(), shape, jnp.bfloat16, lo, hi)

    def permutation(self, n):
        return jax.random.permutation(self._next(), n)
kernel_name = 'adaLN_cond__sliding_block_cached__mixer_token_mlp__decode'

def setup_inputs():
    _rng = _Rng(jax.random.key(int.from_bytes(__import__("os").urandom(4), "little")))
    _w = lambda a: (lambda t: t.astype(jnp.bfloat16) if jnp.issubdtype(t.dtype, jnp.floating) else t)(jnp.asarray(a))

    def _A_setup():
        B, Sq, D = (1, 1, 640)
        Hq, Hkv, Sk, Dh = (32, 32, 32768, 192)
        assert Hq % Hkv == 0, (Hq, Hkv)
        return {'x': _w((lambda *s: _rng.normal(s) * 0.05)(B, Sq, D)), 'k_cache': _w((lambda *s: _rng.normal(s) * 0.05)(B, Hkv, Sk, Dh)), 'v_cache': _w((lambda *s: _rng.normal(s) * 0.05)(B, Hkv, Sk, Dh)), 'wq': _w((lambda *s: _rng.normal(s) * 0.05)(D, Hq * Dh) * D ** (-0.5)), 'wo': _w((lambda *s: _rng.normal(s) * 0.05)(Hq * Dh, D) * (Hq * Dh) ** (-0.5))}
    _A_in = _A_setup()

    def _B_setup():
        B, S, D, F = (1, 1, 640, 1536)
        return {'x': _w((lambda *s: _rng.normal(s) * 0.05)(B, S, D)), 'w1': _w((lambda *s: _rng.normal(s) * 0.05)(S, F) * S ** (-0.5)), 'b1': _w((lambda *s: _rng.normal(s) * 0.05)(F) * 0.02), 'w2': _w((lambda *s: _rng.normal(s) * 0.05)(F, S) * F ** (-0.5)), 'b2': _w((lambda *s: _rng.normal(s) * 0.05)(S) * 0.02)}
    _B_in = _B_setup()
    return {'A_x': _A_in['x'], 'A_k_cache': _A_in['k_cache'], 'A_v_cache': _A_in['v_cache'], 'A_wq': _A_in['wq'], 'A_wo': _A_in['wo'], 'B_x': _B_in['x'], 'B_w1': _B_in['w1'], 'B_b1': _B_in['b1'], 'B_w2': _B_in['w2'], 'B_b2': _B_in['b2'], 'c': _w((lambda *s: _rng.normal(s) * 0.05)(1, 640)), 'w_mod': _w((lambda *s: _rng.normal(s) * 0.05)(640, 6 * 640) * 640 ** (-0.5))}

def reference(A_x, A_k_cache, A_v_cache, A_wq, A_wo, B_x, B_w1, B_b1, B_w2, B_b2, c, w_mod):

    def _A_ref(x, k_cache, v_cache, wq, wo):
        B, Sq, D = x.shape
        Hq, Dh = (32, 192)
        Hkv, Sk = (k_cache.shape[1], k_cache.shape[2])
        W = min(4096, max(256, Sk // 4))
        rep = Hq // Hkv
        q = (lambda x, *d: x.transpose(*d))((x @ wq).reshape(B, Sq, Hq, Dh), 0, 2, 1, 3)
        k = jnp.repeat(k_cache[:, :, Sk - W:, :], rep, axis=1)
        v = jnp.repeat(v_cache[:, :, Sk - W:, :], rep, axis=1)
        scores = jnp.einsum('bhqd,bhkd->bhqk', q, k) * Dh ** (-0.5)
        p = _softmax(scores, axis=-1)
        o = jnp.einsum('bhqk,bhkd->bhqd', p, v)
        return (lambda x, *d: x.transpose(*d))(o, 0, 2, 1, 3).reshape(B, Sq, Hq * Dh) @ wo

    def _B_ref(x, w1, b1, w2, b2):
        B, S, D = x.shape
        h = _layernorm(x, axis=-1)
        u = jnp.einsum('bsd,sf->bdf', h, w1) + b1
        u = _gelu(u)
        y = jnp.einsum('bdf,fs->bds', u, w2) + b2
        return (lambda x, *d: x.transpose(*d))(y, 0, 2, 1)
    x = A_x
    mod = (_silu(c) @ w_mod).reshape(c.shape[0], 6, 1, -1)
    sa, ca, ga, sb, cb, gb = (mod[:, 0].copy(), mod[:, 1].copy(), mod[:, 2].copy(), mod[:, 3].copy(), mod[:, 4].copy(), mod[:, 5].copy())
    h = _layernorm(x, axis=-1) * (1 + ca) + sa
    x = x + ga * _A_ref(h, A_k_cache, A_v_cache, A_wq, A_wo)
    h = _layernorm(x, axis=-1) * (1 + cb) + sb
    x = x + gb * _B_ref(h, B_w1, B_b1, B_w2, B_b2)
    return x
```

```python
import math

import jax
import jax.numpy as jnp
from jax import lax
import jax.experimental.pallas as pl
import jax.experimental.pallas.tpu as pltpu

F32 = jnp.float32
BF16 = jnp.bfloat16

D = 640
H = 32
DH = 192
F = 1536
EPS = 1e-5
G = DH // 8

LO, HI = 1, 0

_C0 = math.sqrt(2.0 / math.pi)
_C1 = 0.044715
KS = (_C0 * _C1) ** (1.0 / 3.0)
CS = _C0 / KS


def _layernorm(x):
    m = jnp.mean(x, axis=-1, keepdims=True)
    xc = x - m
    v = jnp.mean(xc * xc, axis=-1, keepdims=True)
    return xc * lax.rsqrt(v + EPS)


def _col_bcast(row128):
    return jnp.broadcast_to(row128, (128, 128)).T


def _make_kernel(SK, W):
    KV_HI = 512
    KV_LO = W - KV_HI
    W0 = SK - W
    NB = W // 128

    def kernel(x_hbm, k_hbm, v_hbm, wq_hbm, wo_hbm, w1_hbm, b1_hbm, w2_hbm, b2_hbm,
               c_hbm, wm_hbm, o_ref,
               kbuf, vbuf, wq_v, wo_v, wm_v, x_v, c_v, w1_v, b1_v, w2_v, b2_v,
               qb, w1c, b1c, w2c,
               klo, khi, vlo, vhi, wsem, ssem):
        cp = pltpu.make_async_copy
        m8 = lambda i: pl.multiple_of(i, 8)

        def kv_lo(src, buf, sem, h, j, slot):
            return cp(src.at[pl.ds(m8(h * DH + j * 8), 8), pl.ds(W0, KV_LO)],
                      buf.at[slot, pl.ds(m8(j * 8), 8), pl.ds(0, KV_LO)], sem.at[slot])

        def kv_hi(src, buf, sem, h, j, slot):
            return cp(src.at[pl.ds(m8(h * DH + j * 8), 8), pl.ds(W0 + KV_LO, KV_HI)],
                      buf.at[slot, pl.ds(m8(j * 8), 8), pl.ds(KV_LO, KV_HI)], sem.at[slot])

        def kv_hi_all(buf, sem, slot):
            view = buf.at[slot, :, pl.ds(KV_LO, KV_HI)]
            return cp(view, view, sem.at[slot])

        def issue_k(h, j, slot):
            kv_lo(k_hbm, kbuf, klo, h, j, slot).start(priority=LO)
            kv_hi(k_hbm, kbuf, khi, h, j, slot).start(priority=HI)

        def issue_v(h, j, slot):
            kv_lo(v_hbm, vbuf, vlo, h, j, slot).start(priority=LO)
            kv_hi(v_hbm, vbuf, vhi, h, j, slot).start(priority=HI)

        def wait_k(h, j, slot):
            kv_lo(k_hbm, kbuf, klo, h, j, slot).wait()

        def wait_v(h, j, slot):
            kv_lo(v_hbm, vbuf, vlo, h, j, slot).wait()

        def ma(i):
            r = pl.ds(m8(i * 32), 32)
            return cp(wm_hbm.at[r, pl.ds(0, 2 * D)], wm_v.at[r, pl.ds(0, 2 * D)], wsem.at[0])

        def q_piece(i, c0, n, s):
            r = pl.ds(m8((i // 3) * 16), 16)
            c = pl.ds(pl.multiple_of((i % 3) * 2048 + c0, 128), n)
            return cp(wq_hbm.at[r, c], wq_v.at[r, c], wsem.at[s])
        q_lo = lambda i: q_piece(i, 0, 1792, 1)
        q_hi = lambda i: q_piece(i, 1792, 256, 2)

        def issue_q(i):
            q_lo(i).start(priority=LO)
            q_hi(i).start(priority=HI)

        def o_piece(i, r0, n, s):
            r = pl.ds(m8(i * 64 + r0), n)
            return cp(wo_hbm.at[r, :], wo_v.at[r, :], wsem.at[s])
        o_lo = lambda i: o_piece(i, 0, 56, 3)
        o_hi = lambda i: o_piece(i, 56, 8, 4)

        def issue_o(i):
            o_lo(i).start(priority=LO)
            o_hi(i).start(priority=HI)

        def t_piece(i, c0, n, s):
            r = pl.ds(m8(i * 16), 16)
            c = pl.ds(2 * D + c0, n)
            return cp(wm_hbm.at[r, c], wm_v.at[r, c], wsem.at[s])
        t_lo = lambda i: t_piece(i, 0, 3 * D - 256, 5)
        t_hi = lambda i: t_piece(i, 3 * D - 256, 256, 6)

        def issue_t(i):
            t_lo(i).start(priority=LO)
            t_hi(i).start(priority=HI)

        gb_cp = cp(wm_hbm.at[:, pl.ds(5 * D, D)], wm_v.at[:, pl.ds(5 * D, D)], wsem.at[7])

        def loop(n, body, init=0):
            return lax.fori_loop(0, n, body, init)

        def dma_loop(n, wait, issue):
            def body(i, c):
                wait(i)
                issue(i)
                return c
            loop(n, body)

        ma(0).start(priority=LO)
        smalls = [cp(s, d, ssem.at[n]) for n, (s, d) in enumerate(
            [(c_hbm, c_v), (x_hbm, x_v), (w1_hbm, w1_v), (b1_hbm, b1_v), (w2_hbm, w2_v),
             (b2_hbm, b2_v)])]

        def _ma(i, c):
            ma(i + 1).start(priority=LO)
            return c
        loop(19, _ma)
        for s in smalls:
            s.start(priority=HI)

        dma_loop(20, lambda i: ma(i).wait(), issue_q)
        for i in range(20, 24):
            issue_q(i)
        for s in smalls:
            s.wait()

        c32 = c_v[...].astype(F32)
        sc = (c32 * jax.nn.sigmoid(c32)).astype(BF16)
        sc16 = jnp.broadcast_to(sc, (16, D))
        x32 = x_v[0].astype(F32)
        mod_a = jnp.dot(sc16, wm_v[:, pl.ds(0, 2 * D)], preferred_element_type=F32)
        h16 = (_layernorm(x32) * (1.0 + mod_a[:, D:]) + mod_a[:, :D]).astype(BF16)

        def prep(i, c):
            q_lo(i).wait()
            issue_q(i + 24)
            off = pl.multiple_of(i * 128, 128)
            rows = pl.ds(off, 128)
            w1c[rows, :] = _col_bcast(w1_v[:, pl.ds(off, 128)].astype(F32) * KS)
            w2c[rows, :] = _col_bcast(w2_v[:, pl.ds(off, 128)].astype(F32) * (0.5 / KS))
            return c
        loop(12, prep)
        b1f = b1_v[...].astype(F32) * KS
        for i in range(12):
            b1c[pl.ds(i * 128, 128), :] = _col_bcast(b1f[i:i + 1, :])

        dma_loop(84, lambda i: q_lo(i).wait(), lambda i: issue_q(i + 36))
        dma_loop(24, lambda i: q_lo(i).wait(), issue_o)
        qv = wq_v.at[:, pl.ds(0, 3 * 256)]
        cp(qv, qv, wsem.at[2]).wait()

        scale = DH ** -0.5

        def qproj(i, c):
            def step(u):
                o_lo(0).wait()
                issue_o(i * 6 + u + 24)
            step(0)
            off = pl.multiple_of(i * 512, 512)
            q = jnp.dot(h16, wq_v[:, pl.ds(off, 512)], preferred_element_type=F32)[0:1] * scale
            step(1)
            step(2)
            for t in range(4):
                qb[pl.ds(off + t * 128, 128), :] = _col_bcast(q[:, t * 128:(t + 1) * 128])
            step(3)
            step(4)
            step(5)
            return c
        loop(12, qproj)
        dma_loop(24, lambda i: o_lo(i).wait(), lambda j: issue_k(0, j, 0))
        ov = wo_v.at[pl.ds(0, 96 * 8), :]
        cp(ov, ov, wsem.at[4]).wait()
        dma_loop(24, lambda j: wait_k(0, j, 0), lambda j: issue_v(0, j, 0))
        kv_hi_all(kbuf, khi, 0).wait()

        def qk_phase(h, slot, dma):
            def body(j, acc):
                dma(j)
                k = kbuf[slot, pl.ds(m8(j * 8), 8), :].astype(F32)
                q = qb[pl.ds(m8(h * DH + j * 8), 8), :]
                return acc + k * jnp.concatenate([q] * NB, axis=1)
            acc = loop(G, body, jnp.zeros((8, W), F32))
            s = jnp.sum(acc, axis=0, keepdims=True)
            m = jnp.max(s, axis=1, keepdims=True)
            p = jnp.exp(s - m)
            l = jnp.sum(p, axis=1, keepdims=True)
            return jnp.broadcast_to(p, (8, W)), 1.0 / l

        def proj(a_prev, out, g):
            o = jnp.sum(a_prev, axis=1, keepdims=True)
            return out + o * wo_v[pl.ds(m8(g * 8), 8), :].astype(F32)

        def pv_phase(h, slot, p, inv_l, carry, dma):
            def body(j, carry):
                a_prev, out = carry
                dma(j)
                prod = vbuf[slot, pl.ds(m8(j * 8), 8), :].astype(F32) * p
                parts = [prod[:, c * 128:(c + 1) * 128] for c in range(NB)]
                while len(parts) > 1:
                    parts = [parts[2 * i] + parts[2 * i + 1] for i in range(len(parts) // 2)]
                out = proj(a_prev, out, jnp.maximum(h * G + j - 1, 0))
                return parts[0] * inv_l, out
            return loop(G, body, carry)

        def head(h, carry):
            slot = h % 2
            nslot = 1 - slot

            def dma_a(j):
                wait_v(h, j, slot)
                issue_k(h + 1, j, nslot)
            p, inv_l = qk_phase(h, slot, dma_a)
            kv_hi_all(vbuf, vhi, slot).wait()

            def dma_b(j):
                wait_k(h + 1, j, nslot)
                issue_v(h + 1, j, nslot)
            carry = pv_phase(h, slot, p, inv_l, carry, dma_b)
            kv_hi_all(kbuf, khi, nslot).wait()
            return carry

        carry = (jnp.zeros((8, 128), F32), jnp.zeros((8, D), F32))
        carry = loop(H - 1, head, carry)

        hl = H - 1
        sl = hl % 2

        def dma_a(j):
            wait_v(hl, j, sl)
            issue_t(j)
        p, inv_l = qk_phase(hl, sl, dma_a)
        kv_hi_all(vbuf, vhi, sl).wait()

        def dma_b(j):
            t_lo(j).wait()

            @pl.when(j < 16)
            def _():
                issue_t(j + 24)

            @pl.when(j == 16)
            def _():
                gb_cp.start(priority=LO)
        a_prev, out = pv_phase(hl, sl, p, inv_l, carry, dma_b)
        out = proj(a_prev, out, H * G - 1)
        attn = jnp.sum(out, axis=0, keepdims=True)

        tv = wm_v.at[pl.ds(0, 16 * 16), pl.ds(2 * D, 3 * D - 256)]
        cp(tv, tv, wsem.at[5]).wait()
        tv = wm_v.at[:, pl.ds(0, 256)]
        cp(tv, tv, wsem.at[6]).wait()

        mod_b = jnp.dot(sc16, wm_v[:, pl.ds(2 * D, 3 * D)], preferred_element_type=F32)[0:1]
        x1 = x32 + mod_b[:, :D] * attn
        h2 = _layernorm(x1) * (1.0 + mod_b[:, 2 * D:]) + mod_b[:, D:2 * D]
        hn = jnp.broadcast_to(_layernorm(h2), (8, D))

        def mlp(i, acc):
            for u in range(4):
                rows = pl.ds(m8(i * 32 + u * 8), 8)
                tile = lambda r: jnp.concatenate([r[rows, :]] * (D // 128), axis=1)
                v = hn * tile(w1c) + tile(b1c)
                t = jnp.tanh(v * (v * v + CS))
                acc = acc + (v * tile(w2c)) * (1.0 + t)
            return acc
        y8 = loop(F // 32, mlp, jnp.zeros((8, D), F32))
        y = jnp.sum(y8, axis=0, keepdims=True) + b2_v[...].astype(F32).reshape(1, 1)

        gb_cp.wait()
        gb = jnp.dot(sc16, wm_v[:, pl.ds(5 * D, D)], preferred_element_type=F32)[0:1]
        o_ref[0] = (x1 + gb * y).astype(o_ref.dtype)

    return kernel


@jax.jit
def pallas_adaLN_cond__sliding_block_cached__mixer_token_mlp__decode_kernel(
    A_x: jax.Array,
    A_k_cache: jax.Array,
    A_v_cache: jax.Array,
    A_wq: jax.Array,
    A_wo: jax.Array,
    B_x: jax.Array,
    B_w1: jax.Array,
    B_b1: jax.Array,
    B_w2: jax.Array,
    B_b2: jax.Array,
    c: jax.Array,
    w_mod: jax.Array,
):
    SK = A_k_cache.shape[2]
    W = min(4096, max(256, SK // 4))
    kt = jnp.swapaxes(A_k_cache, 2, 3).reshape(H * DH, SK)
    vt = jnp.swapaxes(A_v_cache, 2, 3).reshape(H * DH, SK)

    vmem = pltpu.VMEM
    dma = pltpu.SemaphoreType.DMA
    return pl.pallas_call(
        _make_kernel(SK, W),
        out_shape=jax.ShapeDtypeStruct(A_x.shape, A_x.dtype),
        in_specs=[pl.BlockSpec(memory_space=pl.ANY)] * 11,
        out_specs=pl.BlockSpec(memory_space=pltpu.VMEM),
        scratch_shapes=[
            vmem((2, DH, W), BF16), vmem((2, DH, W), BF16),
            vmem((D, H * DH), BF16), vmem((H * DH, D), BF16), vmem((D, 6 * D), BF16),
            vmem((1, 1, D), BF16), vmem((1, D), BF16),
            vmem((1, F), BF16), vmem((F // 128, 128), BF16), vmem((1, F), BF16),
            vmem((1,), BF16),
            vmem((H * DH, 128), F32),
            vmem((F, 128), F32), vmem((F, 128), F32), vmem((F, 128), F32),
            dma((2,)), dma((2,)), dma((2,)), dma((2,)), dma((8,)), dma((6,)),
        ],
        compiler_params=pltpu.CompilerParams(
            vmem_limit_bytes=64 * 1024 * 1024,
            disable_bounds_checks=True,
        ),
    )(A_x, kt, vt, A_wq, A_wo, B_w1, B_b1.reshape(F // 128, 128), B_w2.reshape(1, F),
      B_b2, c, w_mod)
```

```python
import math

import jax
import jax.numpy as jnp
from jax import lax
import jax.experimental.pallas as pl
import jax.experimental.pallas.tpu as pltpu

F32 = jnp.float32
BF16 = jnp.bfloat16

D = 640
H = 32
DH = 192
F = 1536
EPS = 1e-5
G = DH // 8
ND = D // 128
NF = F // 128

LO, HI = 1, 0

_C0 = math.sqrt(2.0 / math.pi)
_C1 = 0.044715
KS = (_C0 * _C1) ** (1.0 / 3.0)
CS = _C0 / KS

C_W1, C_B1, C_SC, C_N = 0, NF, 2 * NF, 30

DA, DB = 10, 64
OA, OB = 8, 768


def _layernorm(x):
    m = jnp.mean(x, axis=-1, keepdims=True)
    xc = x - m
    v = jnp.mean(xc * xc, axis=-1, keepdims=True)
    return xc * lax.rsqrt(v + EPS)


def _col_bcast(row128):
    return jnp.broadcast_to(row128, (128, 128)).T


def _tile(x, n):
    return jnp.concatenate([x] * n, axis=1)


def _tree_sum(parts):
    while len(parts) > 1:
        nxt = [parts[2 * i] + parts[2 * i + 1] for i in range(len(parts) // 2)]
        if len(parts) % 2:
            nxt.append(parts[-1])
        parts = nxt
    return parts[0]


def _groups(x):
    return [x[j * 8:(j + 1) * 8, :] for j in range(x.shape[0] // 8)]


def _make_kernel(SK, W):
    KV_HI = 16
    KV_LO = DH - KV_HI
    W0 = SK - W
    NB = W // 128

    def kernel(x_hbm, k_hbm, v_hbm, wq_hbm, wo_hbm, w1_hbm, b1_hbm, w2_hbm, b2_hbm,
               c_hbm, wm_hbm, o_ref,
               kbuf, vbuf, wq_v, wo_v, wm_v, x_v, c_v, w1_v, b1_v, w2_v, b2_v,
               qb, rows, cols, lhs, abuf, sbuf, consts, tbuf,
               klo, khi, vlo, vhi, wsem, tlo, thi, ssem):
        cp = pltpu.make_async_copy
        m8 = lambda i: pl.multiple_of(i, 8)
        m128 = lambda i: pl.multiple_of(i, 128)
        MARK = lambda name: None

        def kv_stream(src, buf, lo_sem, hi_sem, h, slot):
            def piece(c, r0, n, sem):
                return cp(src.at[pl.ds(m8(h * DH + r0), n), pl.ds(m128(W0 + c * 128), 128)],
                          buf.at[slot, c, pl.ds(r0, n), :], sem.at[slot])
            return (lambda c: piece(c, 0, KV_LO, lo_sem),
                    lambda c: piece(c, KV_LO, KV_HI, hi_sem))

        k_stream = lambda h, slot: kv_stream(k_hbm, kbuf, klo, khi, h, slot)
        v_stream = lambda h, slot: kv_stream(v_hbm, vbuf, vlo, vhi, h, slot)

        def w_piece(src, dst, a0, na, b, c0, n, sem):
            idx = (pl.ds(a0, na), pl.ds(m8(b * 8), 8), pl.ds(m128(c0), n))
            return cp(src.at[idx], dst.at[idx], sem)

        def ma(i):
            b = lax.div(i, 5)
            return w_piece(wm_hbm, wm_v, 0, DA, b, (i - 5 * b) * 384, 384, wsem.at[0])

        def q_piece(i, a0, na, s):
            return w_piece(wq_hbm, wq_v, a0, na, i >> 4, (i & 15) * 384, 384, wsem.at[s])
        q_stream = (lambda i: q_piece(i, 0, DA - 1, 1), lambda i: q_piece(i, DA - 1, 1, 2))

        def o_piece(i, a0, na, s):
            return w_piece(wo_hbm, wo_v, a0, na, i, 0, D, wsem.at[s])
        o_stream = (lambda i: o_piece(i, 0, OA - 1, 3), lambda i: o_piece(i, OA - 1, 1, 4))

        def t_piece(i, a0, na, sem):
            b = lax.div(i, 5)
            return w_piece(wm_hbm, wm_v, a0, na, b, 3 * D + (i - 5 * b) * 256, 256, sem.at[b])
        t_stream = (lambda i: t_piece(i, 0, DA - 1, tlo), lambda i: t_piece(i, DA - 1, 1, thi))

        def t_wait(b):
            for a0, na, sem in ((0, DA - 1, tlo), (DA - 1, 1, thi)):
                w_piece(wm_v, wm_v, a0, na, b, 3 * D, 2 * D, sem.at[b]).wait()

        gb_piece = lambda b: w_piece(wm_hbm, wm_v, 0, DA, b, 5 * D, D, wsem.at[5])

        def issue(stream, i):
            stream[0](i).start(priority=LO)
            stream[1](i).start(priority=HI)

        def step(cur, i, nxt=None, inxt=None):
            cur[0](i).wait()
            if nxt is not None:
                issue(nxt, inxt)
            cur[1](i).wait()

        def loop(n, body, init=0):
            return lax.fori_loop(0, n, body, init)

        def dma_loop(n, cur, i0, nxt, n0):
            def body(i, c):
                step(cur, i + i0, nxt, i + n0)
                return c
            loop(n, body)

        def wm_cols(c0, n, a0=0, na=DA):
            return wm_v[a0:a0 + na, :, pl.ds(c0, n)].reshape(na * DB, n)

        MARK('p_issue')
        ma(0).start(priority=LO)
        smalls = [cp(s, d, ssem.at[n]) for n, (s, d) in enumerate(
            [(c_hbm, c_v), (x_hbm, x_v), (w1_hbm, w1_v), (b1_hbm, b1_v), (w2_hbm, w2_v),
             (b2_hbm, b2_v)])]
        for s in smalls:
            s.start(priority=HI)

        def _ma(i, c):
            ma(i + 1).start(priority=LO)
            return c
        loop(39, _ma)

        MARK('p_ma')

        def _ma2(i, c):
            ma(i).wait()
            issue(q_stream, i)
            return c
        loop(40, _ma2)
        for s in smalls:
            s.wait()
        LQ = 40

        MARK('p_moda')
        c32 = c_v[...].astype(F32)
        sc = (c32 * jax.nn.sigmoid(c32)).astype(BF16)
        sc16 = jnp.broadcast_to(sc, (16, D))
        x32 = x_v[0].astype(F32)
        xn = _layernorm(x32)
        w1f = w1_v[...].astype(F32)
        b1f = b1_v[...].astype(F32)
        scf = sc.astype(F32)
        for i in range(NF):
            rows[C_W1 + i:C_W1 + i + 1, :] = w1f[:, i * 128:(i + 1) * 128] * KS
        rows[C_B1:C_B1 + NF, :] = b1f * KS
        for i in range(ND):
            rows[C_SC + i:C_SC + i + 1, :] = scf[:, i * 128:(i + 1) * 128]
        rows[C_SC + ND:C_N, :] = jnp.zeros((C_N - C_SC - ND, 128), F32)
        dma_loop(2, q_stream, 0, q_stream, LQ)
        ca = jnp.dot(sc16, wm_cols(D, D), preferred_element_type=F32)
        dma_loop(3, q_stream, 2, q_stream, LQ + 2)
        sa = jnp.dot(sc16, wm_cols(0, D), preferred_element_type=F32)
        h16 = (xn * (1.0 + ca) + sa).astype(BF16)
        dma_loop(3, q_stream, 5, q_stream, LQ + 5)
        ga = jnp.dot(sc16, wm_cols(2 * D, D), preferred_element_type=F32)[0:8]
        dma_loop(4, q_stream, 8, q_stream, LQ + 8)

        w2h = w2_v[...].astype(F32) * 0.5
        b1row = jnp.concatenate([b1f[i:i + 1, :] for i in range(NF)], axis=1)
        pw = w1f * w2h
        pb = b1row * w2h
        pw_hi = pw.astype(BF16).astype(F32)
        pb_hi = pb.astype(BF16).astype(F32)
        rid = lax.broadcasted_iota(jnp.int32, (16, F), 0)
        lhs[...] = jnp.where(
            rid == 0, pw_hi, jnp.where(
                rid == 1, pw - pw_hi, jnp.where(
                    rid == 2, pb_hi, jnp.where(rid == 3, pb - pb_hi, 0.0)))).astype(BF16)
        sum_w = jnp.sum(pw, axis=1, keepdims=True)
        sum_b = jnp.sum(pb, axis=1, keepdims=True) + b2_v[...].astype(F32).reshape(1, 1)
        consts[0:1, :] = jnp.broadcast_to(sum_w, (1, 128))
        consts[1:2, :] = jnp.broadcast_to(sum_b, (1, 128))

        MARK('p_prep')

        def prep(i, c):
            step(q_stream, 5 * i + 12, q_stream, 5 * i + LQ + 12)
            for u in range(3):
                t = 3 * i + u
                cols[pl.ds(m128(t * 128), 128), :] = _col_bcast(rows[pl.ds(t, 1), :])
            dma_loop(4, q_stream, 5 * i + 13, q_stream, 5 * i + LQ + 13)
            return c
        loop(C_N // 3, prep)

        MARK('p_wq')
        dma_loop(128 - LQ - 62, q_stream, 62, q_stream, LQ + 62)
        dma_loop(8, q_stream, 128 - LQ, o_stream, 0)
        dma_loop(LQ - 8, q_stream, 128 - LQ + 8, o_stream, 8)
        LO_ = LQ

        MARK('p_qproj')
        scale = DH ** -0.5

        def qproj(i0, s0, n, nxt, n0):
            def body(i, c):
                dma_loop(1, o_stream, s0 + i * n, nxt, n0 + i * n)
                off = m128((i + i0) * 384)
                wq = wq_v[:, :, pl.ds(off, 384)].reshape(D, 384)
                q = jnp.dot(h16, wq, preferred_element_type=F32)[0:1] * scale
                dma_loop(2, o_stream, s0 + i * n + 1, nxt, n0 + i * n + 1)
                for t in range(3):
                    qb[pl.ds(off + t * 128, 128), :] = _col_bcast(q[:, t * 128:(t + 1) * 128])
                dma_loop(n - 3, o_stream, s0 + i * n + 3, nxt, n0 + i * n + 3)
                return c
            return body
        loop(8, qproj(0, 0, 7, o_stream, LO_))
        dma_loop(8, o_stream, 56, None, 0)
        loop(8, qproj(8, 64, 4, k_stream(0, 0), 0))
        MARK('p_k0')
        abuf[...] = jnp.zeros((DH, 128), F32)
        dma_loop(NB, k_stream(0, 0), 0, v_stream(0, 0), 0)

        def proj(h, out):
            o = jnp.sum(abuf[...], axis=1, keepdims=True)
            wo = wo_v[h >> 2, pl.ds(pl.multiple_of((h & 3) * DH, 64), DH), :]
            return out + _tree_sum(_groups(o * wo.astype(F32)))

        def phase_a(h, slot, out, cur, nxt):
            q = qb[pl.ds(pl.multiple_of(h * DH, 64), DH), :]

            def body(i, m):
                step(cur, i, nxt, i)
                for u in range(2):
                    c = 2 * i + u
                    s = _tree_sum(_groups(kbuf[slot, c].astype(F32) * q))
                    s = jnp.broadcast_to(jnp.sum(s, axis=0, keepdims=True), (8, 128))
                    sbuf[c] = s
                    m = jnp.maximum(m, s)
                return m
            m = loop(NB // 2, body, jnp.full((8, 128), -jnp.inf, F32))
            step(cur, 16, nxt, 16)
            m = jnp.max(m, axis=1, keepdims=True)
            out = proj(jnp.maximum(h - 1, 0), out)
            dma_loop(3, cur, 17, nxt, 17)
            p = jnp.exp(sbuf[...] - m)
            sbuf[...] = p
            l = _tree_sum([p[c] for c in range(NB)])
            inv_l = 1.0 / jnp.sum(l, axis=1, keepdims=True)
            dma_loop(NB - 20, cur, 20, nxt, 20)
            return inv_l, out

        def pv_tile(slot, c, acc):
            p = sbuf[c]
            return acc + vbuf[slot, c].astype(F32) * jnp.concatenate([p] * G, axis=0)

        def pv_done(acc, inv_l):
            abuf[...] = acc * jnp.concatenate([jnp.broadcast_to(inv_l, (8, 128))] * G, axis=0)

        def head(h, out):
            slot = h & 1
            nslot = 1 - slot
            knext = k_stream(h + 1, nslot)
            inv_l, out = phase_a(h, slot, out, v_stream(h, slot), knext)

            def body(c, acc):
                step(knext, c, v_stream(h + 1, nslot), c)
                return pv_tile(slot, c, acc)
            pv_done(loop(NB, body, jnp.zeros((DH, 128), F32)), inv_l)
            return out

        MARK('main')
        out = loop(H - 1, head, jnp.zeros((8, D), F32))

        MARK('qk31')
        hl = H - 1
        sl = hl % 2
        inv_l, out = phase_a(hl, sl, out, v_stream(hl, sl), t_stream)

        MARK('pv31')

        def body(i, acc):
            step(t_stream, i, t_stream, i + NB)
            for u in range(4):
                acc = pv_tile(sl, 4 * i + u, acc)
            return acc
        acc = loop(8, body, jnp.zeros((DH, 128), F32))
        for b in range(8):
            gb_piece(b).start(priority=LO)
        pv_done(acc, inv_l)
        MARK('proj31')
        out = proj(hl, out)
        attn = jnp.sum(out, axis=0, keepdims=True)
        x1 = x32 + ga * attn
        z = _layernorm(x1)

        MARK('t2')

        def matvec(acc, b):
            ts = []
            for a in range(DA):
                s = cols[pl.ds(m8(C_SC * 128 + a * DB + b * 8), 8), :]
                w = wm_v[a, pl.ds(m8(b * 8), 8), pl.ds(3 * D, 2 * D)]
                ts.append(_tile(s, 2 * ND) * w.astype(F32))
            return acc + _tree_sum(ts)

        def t2(b, acc):
            t_wait(b)
            return matvec(acc, b)

        def h2_of(acc):
            mod = jnp.sum(acc, axis=0, keepdims=True)
            return z * (1.0 + mod[:, D:]) + mod[:, :D]
        step(t_stream, 8)
        step(t_stream, 9)
        acc = matvec(matvec(jnp.zeros((8, 2 * D), F32), 0), 1)
        acc = lax.fori_loop(2, 7, t2, acc)
        MARK('mu0')
        mu0 = jnp.mean(h2_of(acc), axis=1, keepdims=True)
        MARK('w7')
        t_wait(7)
        MARK('ln2')
        acc = matvec(acc, 7)
        d = h2_of(acc) - mu0
        s1 = jnp.mean(d, axis=1, keepdims=True)
        s2 = jnp.mean(d * d, axis=1, keepdims=True)
        var = jnp.maximum(s2 - s1 * s1, 0.0)
        hn = (d - s1) * lax.rsqrt(var + EPS)

        MARK('mlp')
        def tanh_block(b):
            ts = []
            for u in range(16):
                w1c = cols[pl.ds((C_W1 + b) * 128 + u * 8, 8), :]
                b1c = cols[pl.ds((C_B1 + b) * 128 + u * 8, 8), :]
                v = hn * _tile(w1c, ND) + _tile(b1c, ND)
                ts.append(jnp.tanh(v * (v * v + CS)))
            return jnp.concatenate(ts, axis=0).astype(BF16)

        def red(b, t):
            return jnp.dot(lhs[:, b * 128:(b + 1) * 128], t, preferred_element_type=F32)

        NPRE = 10
        r = _tree_sum([red(b, tanh_block(b)) for b in range(NPRE - 1)])
        t = tanh_block(NPRE - 1)
        for j in range(ND):
            tbuf[j] = t[:, j * 128:(j + 1) * 128]
        MARK('mlp2')
        gv = wm_v.at[:, :, pl.ds(5 * D, D)]
        cp(gv, gv, wsem.at[5]).wait()
        gb = jnp.dot(sc16, wm_cols(5 * D, D), preferred_element_type=F32)
        t = jnp.concatenate([tbuf[j] for j in range(ND)], axis=1)
        r = r + red(NPRE - 1, t)
        for b in range(NPRE, NF):
            r = r + red(b, tanh_block(b))
        y = (hn[0:1] * (r[0:1] + r[1:2] + _tile(consts[0:1, :], ND))
             + (r[2:3] + r[3:4] + _tile(consts[1:2, :], ND)))
        o_ref[0] = (x1[0:1] + gb[0:1] * y).astype(o_ref.dtype)
        MARK(None)

    return kernel


@jax.jit
def pallas_adaLN_cond__sliding_block_cached__mixer_token_mlp__decode_kernel(
    A_x: jax.Array,
    A_k_cache: jax.Array,
    A_v_cache: jax.Array,
    A_wq: jax.Array,
    A_wo: jax.Array,
    B_x: jax.Array,
    B_w1: jax.Array,
    B_b1: jax.Array,
    B_w2: jax.Array,
    B_b2: jax.Array,
    c: jax.Array,
    w_mod: jax.Array,
):
    SK = A_k_cache.shape[2]
    W = min(4096, max(256, SK // 4))
    kt = jnp.swapaxes(A_k_cache, 2, 3).reshape(H * DH, SK)
    vt = jnp.swapaxes(A_v_cache, 2, 3).reshape(H * DH, SK)

    vmem = pltpu.VMEM
    dma = pltpu.SemaphoreType.DMA
    return pl.pallas_call(
        _make_kernel(SK, W),
        out_shape=jax.ShapeDtypeStruct(A_x.shape, A_x.dtype),
        in_specs=[pl.BlockSpec(memory_space=pl.ANY)] * 11,
        out_specs=pl.BlockSpec(memory_space=pltpu.VMEM),
        scratch_shapes=[
            vmem((2, W // 128, DH, 128), BF16), vmem((2, W // 128, DH, 128), BF16),
            vmem((DA, DB, H * DH), BF16), vmem((OA, OB, D), BF16), vmem((DA, DB, 6 * D), BF16),
            vmem((1, 1, D), BF16), vmem((1, D), BF16),
            vmem((1, F), BF16), vmem((NF, 128), BF16), vmem((1, F), BF16),
            vmem((1,), BF16),
            vmem((H * DH, 128), F32), vmem((C_N, 128), F32), vmem((C_N * 128, 128), F32),
            vmem((16, F), BF16), vmem((DH, 128), F32), vmem((W // 128, 8, 128), F32),
            vmem((2, 128), F32), vmem((ND, 128, 128), BF16),
            dma((2,)), dma((2,)), dma((2,)), dma((2,)), dma((6,)), dma((8,)), dma((8,)),
            dma((6,)),
        ],
        compiler_params=pltpu.CompilerParams(
            vmem_limit_bytes=64 * 1024 * 1024,
            disable_bounds_checks=True,
            disable_semaphore_checks=True,
        ),
    )(A_x, kt, vt, A_wq.reshape(DA, DB, H * DH), A_wo.reshape(OA, OB, D), B_w1,
      B_b1.reshape(NF, 128), B_w2.reshape(1, F), B_b2, c, w_mod.reshape(DA, DB, 6 * D))
```

```python
import math

import jax
import jax.numpy as jnp
from jax import lax
import jax.experimental.pallas as pl
import jax.experimental.pallas.tpu as pltpu

F32 = jnp.float32
BF16 = jnp.bfloat16

D = 640
H = 32
DH = 192
F = 1536
EPS = 1e-5
G = DH // 8
ND = D // 128
NF = F // 128

LO, HI = 1, 0

_C0 = math.sqrt(2.0 / math.pi)
_C1 = 0.044715
KS = (_C0 * _C1) ** (1.0 / 3.0)
CS = _C0 / KS

C_W1, C_B1, C_SC, C_W2, C_N = 0, NF, 2 * NF, 2 * NF + 1, 27

DA, DB = 10, 64
TA, TB = 15, 128


def _pair_view(w):
    r, c = w.shape
    t = w.reshape(r // 8, 8, c // 128, 128).transpose(0, 2, 1, 3)
    return t.reshape(TA, TB, 16, 128)


def _layernorm(x):
    m = jnp.mean(x, axis=-1, keepdims=True)
    xc = x - m
    v = jnp.mean(xc * xc, axis=-1, keepdims=True)
    return xc * lax.rsqrt(v + EPS)


def _layernorm_shifted(x, mu0):
    d = x - mu0
    s1 = jnp.mean(d, axis=-1, keepdims=True)
    s2 = jnp.mean(d * d, axis=-1, keepdims=True)
    var = jnp.maximum(s2 - s1 * s1, 0.0)
    return (d - s1) * lax.rsqrt(var + EPS)


def _col_bcast(row128):
    return jnp.broadcast_to(row128, (128, 128)).T


def _tile(x, n):
    return jnp.concatenate([x] * n, axis=1)


def _tree_sum(parts):
    while len(parts) > 1:
        nxt = [parts[2 * i] + parts[2 * i + 1] for i in range(len(parts) // 2)]
        if len(parts) % 2:
            nxt.append(parts[-1])
        parts = nxt
    return parts[0]


def _groups(x):
    return [x[j * 8:(j + 1) * 8, :] for j in range(x.shape[0] // 8)]


def _make_kernel(SK, W):
    KV_HI = 16
    KV_LO = DH - KV_HI
    W0 = SK - W
    NB = W // 128

    def kernel(x_hbm, k_hbm, v_hbm, wq_hbm, wo_hbm, w1_hbm, b1_hbm, w2_hbm, b2_hbm,
               c_hbm, wm_hbm, o_ref,
               kbuf, vbuf, wq_v, wo_v, wm_v, x_v, c_v, w1_v, b1_v, w2_v, b2_v,
               qb, rows, cols, lhs, abuf, sbuf, consts, modb, gbuf,
               klo, khi, vlo, vhi, wsem, ssem):
        cp = pltpu.make_async_copy
        m8 = lambda i: pl.multiple_of(i, 8)
        m128 = lambda i: pl.multiple_of(i, 128)
        MARK = lambda name: None

        def kv_stream(src, buf, lo_sem, hi_sem, h, slot, sem_of):
            def piece(c, r0, n, sem):
                return cp(src.at[pl.ds(m8(h * DH + r0), n), pl.ds(m128(W0 + c * 128), 128)],
                          buf.at[slot, c, pl.ds(r0, n), :], sem.at[sem_of(c)])
            return (lambda c: piece(c, 0, KV_LO, lo_sem),
                    lambda c: piece(c, KV_LO, KV_HI, hi_sem))

        k_stream = lambda h, slot: kv_stream(k_hbm, kbuf, klo, khi, h, slot, lambda c: slot)
        v_stream = lambda h, slot: kv_stream(v_hbm, vbuf, vlo, vhi, h, slot,
                                             lambda c: slot * (NB // 4) + (c >> 2))

        def w_piece(src, dst, a0, na, b, c0, n, sem):
            idx = (pl.ds(a0, na), pl.ds(m8(b * 8), 8), pl.ds(m128(c0), n))
            return cp(src.at[idx], dst.at[idx], sem)

        def m_pieces(b, part):
            out = []
            for na, c0, n in ([(DA, c * 384, 384) for c in range(5)]
                              + [(8, (3 + c) * D, D) for c in range(2)]):
                a0, na = {'all': (0, na), 'lo': (0, na - 1), 'hi': (na - 1, 1)}[part]
                out.append(w_piece(wm_hbm, wm_v, a0, na, b, c0, n,
                                   wsem.at[8 if part == 'hi' else 0]))
            return out

        def pair_stream(src, dst, s):
            dst = dst.reshape(TA, TB, 16, 128)

            def piece(i, a0, na, sem):
                idx = (pl.ds(a0, na), pl.ds(i, 1))
                return cp(src.at[idx], dst.at[idx], sem)
            return (lambda i: piece(i, 0, TA - 2, wsem.at[s]),
                    lambda i: piece(i, TA - 2, 2, wsem.at[s + 1]))
        q_stream = pair_stream(wq_hbm, wq_v, 1)
        o_stream = pair_stream(wo_hbm, wo_v, 3)

        def t8_piece(i):
            idx = (8, pl.ds(m8((i & 1) * 32), 32), pl.ds(m128(3 * D + (i >> 1) * 128), 128))
            return cp(wm_hbm.at[idx], wm_v.at[idx], wsem.at[5])
        t8_stream = (None, t8_piece)

        def slab(a, s, src):
            idx = (a, slice(None), pl.ds(3 * D, 2 * D))
            return cp(src.at[idx], wm_v.at[idx], wsem.at[s])

        gb_piece = lambda j: cp(wm_hbm.at[:, :, pl.ds(5 * D + j * 128, 128)], gbuf.at[j],
                                wsem.at[7])

        def issue(stream, i):
            if stream[0] is not None:
                stream[0](i).start(priority=LO)
            stream[1](i).start(priority=HI)

        def step(cur, i, nxt=None, inxt=None):
            cur[0](i).wait()
            if nxt is not None:
                issue(nxt, inxt)
            cur[1](i).wait()

        def loop(n, body, init=0):
            return lax.fori_loop(0, n, body, init)

        def dma_loop(n, cur, i0, nxt, n0):
            def body(i, c):
                step(cur, i + i0, nxt, i + n0)
                return c
            loop(n, body)

        def wm_cols(c0, n, a0=0, na=DA):
            return wm_v[a0:a0 + na, :, pl.ds(c0, n)].reshape(na * DB, n)

        MARK('p_issue')
        for m in m_pieces(0, 'all'):
            m.start(priority=LO)
        smalls = [cp(s, d, ssem.at[n]) for n, (s, d) in enumerate(
            [(c_hbm, c_v), (x_hbm, x_v), (w1_hbm, w1_v), (b1_hbm, b1_v), (w2_hbm, w2_v),
             (b2_hbm, b2_v)])]
        for s in smalls:
            s.start(priority=HI)

        def _ma(b, c):
            for m in m_pieces(b + 1, 'all'):
                m.start(priority=LO)
            return c
        loop(3, _ma)

        MARK('p_ma')

        def _ma2(b, c):
            for m, lo, hi in zip(m_pieces(b, 'all'), m_pieces(b + 4, 'lo'), m_pieces(b + 4, 'hi')):
                m.wait()
                lo.start(priority=LO)
                hi.start(priority=HI)
            return c
        loop(4, _ma2)

        def _ma3(b, c):
            for u, (lo, hi) in enumerate(zip(m_pieces(b + 4, 'lo'), m_pieces(b + 4, 'hi'))):
                lo.wait()
                issue(q_stream, 7 * b + u)
                hi.wait()
            return c
        loop(4, _ma3)
        for s in smalls:
            s.wait()
        LQ = 28

        MARK('p_moda')
        c32 = c_v[...].astype(F32)
        sc = (c32 * jax.nn.sigmoid(c32)).astype(BF16)
        sc16 = jnp.broadcast_to(sc, (16, D))
        x32 = x_v[0].astype(F32)
        xn = _layernorm(x32)
        consts[2:3, :] = jnp.broadcast_to(jnp.mean(x32, axis=1, keepdims=True), (1, 128))
        w2h = w2_v[...].astype(F32) * 0.5
        w1f = w1_v[...].astype(F32)
        b1f = b1_v[...].astype(F32)
        scf = sc.astype(F32)
        for i in range(NF):
            rows[C_W1 + i:C_W1 + i + 1, :] = w1f[:, i * 128:(i + 1) * 128] * KS
        rows[C_B1:C_B1 + NF, :] = b1f * KS
        rows[C_SC:C_SC + 1, :] = scf[:, D - 128:]
        rows[C_W2:C_W2 + 1, :] = w2h[:, F - 128:] * (1.0 / KS)
        rows[C_W2 + 1:C_N, :] = jnp.zeros((C_N - C_W2 - 1, 128), F32)
        dma_loop(2, q_stream, 0, q_stream, LQ)
        ca = jnp.dot(sc16, wm_cols(D, D), preferred_element_type=F32)
        dma_loop(3, q_stream, 2, q_stream, LQ + 2)
        sa = jnp.dot(sc16, wm_cols(0, D), preferred_element_type=F32)
        h8 = (xn * (1.0 + ca) + sa)[0:8].astype(BF16).astype(F32)
        dma_loop(3, q_stream, 5, q_stream, LQ + 5)
        ga = jnp.dot(sc16, wm_cols(2 * D, D), preferred_element_type=F32)[0:8]
        dma_loop(3, q_stream, 8, q_stream, LQ + 8)
        sb = jnp.dot(sc16[:, :512], wm_cols(3 * D, D, 0, 8), preferred_element_type=F32)[0:1]
        modb[:, :D] = sb
        dma_loop(3, q_stream, 11, q_stream, LQ + 11)
        modb[:, D:] = jnp.dot(sc16[:, :512], wm_cols(4 * D, D, 0, 8),
                              preferred_element_type=F32)[0:1]
        consts[3:4, :] = jnp.broadcast_to(jnp.mean(sb, axis=1, keepdims=True), (1, 128))
        dma_loop(3, q_stream, 14, q_stream, LQ + 14)

        b1row = jnp.concatenate([b1f[i:i + 1, :] for i in range(NF)], axis=1)
        pw = w1f * w2h
        pb = b1row * w2h
        pw_hi = pw.astype(BF16).astype(F32)
        pb_hi = pb.astype(BF16).astype(F32)
        rid = lax.broadcasted_iota(jnp.int32, (8, F), 0)
        lhs[...] = jnp.where(
            rid == 0, pw_hi, jnp.where(
                rid == 1, pw - pw_hi, jnp.where(
                    rid == 2, pb_hi, jnp.where(rid == 3, pb - pb_hi, 0.0))))
        sum_w = jnp.sum(pw, axis=1, keepdims=True)
        sum_b = jnp.sum(pb, axis=1, keepdims=True) + b2_v[...].astype(F32).reshape(1, 1)
        consts[0:1, :] = jnp.broadcast_to(sum_w, (1, 128))
        consts[1:2, :] = jnp.broadcast_to(sum_b, (1, 128))

        MARK('p_prep')

        def prep(i, c):
            step(q_stream, 5 * i + 17, q_stream, 5 * i + LQ + 17)
            for u in range(3):
                t = 3 * i + u
                cols[pl.ds(m128(t * 128), 128), :] = _col_bcast(rows[pl.ds(t, 1), :])
            dma_loop(4, q_stream, 5 * i + 18, q_stream, 5 * i + LQ + 18)
            return c
        loop(C_N // 3, prep)

        MARK('p_wq')
        dma_loop(128 - LQ - 62, q_stream, 62, q_stream, LQ + 62)
        dma_loop(LQ, q_stream, 128 - LQ, o_stream, 0)

        MARK('p_qproj')
        scale = DH ** -0.5

        def q_cols(i, q):
            for t in range(2):
                qb[pl.ds(m128(i * 256 + t * 128), 128), :] = _col_bcast(
                    q[0:1, t * 128:(t + 1) * 128])

        def qproj(i0, s0, n, nxt, n0):
            def body(i, q_prev):
                step(o_stream, s0 + i * n, nxt, n0 + i * n)
                q_cols(jnp.maximum(i + i0 - 1, 0), q_prev)
                w = wq_v[:, i + i0].astype(F32)
                w = jnp.concatenate([w[:, 0:8].reshape(D, 128), w[:, 8:16].reshape(D, 128)],
                                    axis=1)
                q = jnp.dot(h8, w, precision=lax.Precision.DEFAULT,
                            preferred_element_type=F32) * scale
                dma_loop(n - 1, o_stream, s0 + i * n + 1, nxt, n0 + i * n + 1)
                return q
            return body
        k0, v0 = k_stream(0, 0), v_stream(0, 0)
        q = loop(20, qproj(0, 0, 5, o_stream, LQ), jnp.zeros((8, 256), F32))
        q = loop(4, qproj(20, 100, 7, k0, 0), q)
        for c in range(LQ, NB):
            issue(k0, c)
        MARK('p_k0')
        step(k0, 0, v0, 0)
        q_cols(23, q)
        abuf[...] = jnp.zeros((DH, 128), F32)
        dma_loop(NB - 1, k0, 1, v0, 1)

        def proj(h, a, out):
            o = jnp.sum(a, axis=1, keepdims=True)
            outs = [out, None]
            for jj in range(G // 2):
                tiles = _groups(wo_v[h, jj * ND:(jj + 1) * ND].astype(F32).reshape(16 * ND, 128))
                for e in range(2):
                    j = 2 * jj + e
                    w = jnp.concatenate(tiles[e * ND:(e + 1) * ND], axis=1)
                    t = o[j * 8:(j + 1) * 8] * w
                    outs[e] = t if outs[e] is None else outs[e] + t
            return outs[0] + outs[1]

        def phase_a(h, slot, out, cur, nxt):
            q = qb[pl.ds(pl.multiple_of(h * DH, 64), DH), :]

            def body(i, m):
                step(cur, i, nxt, i)
                for u in range(2):
                    c = 2 * i + u
                    s = _tree_sum(_groups(kbuf[slot, c].astype(F32) * q))
                    s = jnp.broadcast_to(jnp.sum(s, axis=0, keepdims=True), (8, 128))
                    sbuf[c] = s
                    m = jnp.maximum(m, s)
                return m
            m = loop(NB // 2, body, jnp.full((8, 128), -jnp.inf, F32))
            step(cur, 16, nxt, 16)
            m = jnp.max(m, axis=1, keepdims=True)
            out = proj(jnp.maximum(h - 1, 0), abuf[...], out)
            dma_loop(3, cur, 17, nxt, 17)
            p = jnp.exp(sbuf[...] - m)
            sbuf[...] = p
            l = _tree_sum([p[c] for c in range(NB)])
            inv_l = 1.0 / jnp.sum(l, axis=1, keepdims=True)
            return inv_l, out

        def pv_tile(slot, c, acc):
            p = sbuf[c]
            return acc + vbuf[slot, c].astype(F32) * jnp.concatenate([p] * G, axis=0)

        def pv_done(acc, inv_l):
            return acc * jnp.concatenate([jnp.broadcast_to(inv_l, (8, 128))] * G, axis=0)

        def head(h, out):
            slot = h & 1
            nslot = 1 - slot
            knext = k_stream(h + 1, nslot)
            inv_l, out = phase_a(h, slot, out, v_stream(h, slot), knext)
            dma_loop(NB - 20, v_stream(h, slot), 20, knext, 20)

            def body(c, acc):
                step(knext, c, v_stream(h + 1, nslot), c)
                return pv_tile(slot, c, acc)
            abuf[...] = pv_done(loop(NB, body, jnp.zeros((DH, 128), F32)), inv_l)
            return out

        MARK('main')
        out = loop(H - 1, head, jnp.zeros((8, D), F32))

        MARK('qk31')
        hl = H - 1
        sl = hl % 2
        vl = v_stream(hl, sl)
        slab(9, 6, wm_hbm).start(priority=LO)
        for j in range(ND):
            gb_piece(j).start(priority=LO)
        inv_l, out = phase_a(hl, sl, out, vl, t8_stream)

        MARK('pv31')

        def body(i, acc):
            step(vl, 20 + i)
            for u in range(5):
                acc = pv_tile(sl, 5 * i + u, acc)
            return acc
        acc = loop(4, body, jnp.zeros((DH, 128), F32))

        def body(i, acc):
            step(vl, 24 + i)
            return pv_tile(sl, 20 + i, acc)
        acc = loop(8, body, acc)
        slab(8, 5, wm_v).wait()

        def matvec(acc, a):
            for u in range(DB // 8):
                s = cols[pl.ds(C_SC * 128 + (a - 8) * DB + u * 8, 8), :]
                t = _tile(s, 2 * ND) * wm_v[a, pl.ds(u * 8, 8), pl.ds(3 * D, 2 * D)].astype(F32)
                acc = t if acc is None else acc + t
            return acc

        MARK('proj31')
        for c in range(28, NB):
            acc = pv_tile(sl, c, acc)
        out = proj(hl, pv_done(acc, inv_l), out)
        macc = matvec(None, 8)
        attn = jnp.sum(out, axis=0, keepdims=True)
        x1 = x32 + ga * attn
        z = _layernorm_shifted(x1, _tile(consts[2:3, :], ND))

        MARK('w9')
        slab(9, 6, wm_hbm).wait()
        MARK('ln2')
        mod = jnp.sum(matvec(macc, 9), axis=0, keepdims=True) + modb[...]
        h2 = z * (1.0 + mod[:, D:]) + mod[:, :D]
        hn = _layernorm_shifted(h2, _tile(consts[3:4, :], ND))

        MARK('mlp')

        def tanh_rows(b, u, hn):
            w1c = cols[pl.ds((C_W1 + b) * 128 + u * 8, 8), :]
            b1c = cols[pl.ds((C_B1 + b) * 128 + u * 8, 8), :]
            v = hn * _tile(w1c, ND) + _tile(b1c, ND)
            return v, jnp.tanh(v * (v * v + CS))

        r = None
        for b in range(NF - 1):
            ts = [tanh_rows(b, u, hn)[1] for u in range(16)]
            rb = jnp.dot(lhs[:, b * 128:(b + 1) * 128], jnp.concatenate(ts, axis=0),
                         precision=lax.Precision.DEFAULT, preferred_element_type=F32)
            r = rb if r is None else r + rb
        hl_ = hn + ts[0] * 0.0
        yacc = None
        for u in range(16):
            v, t = tanh_rows(NF - 1, u, hl_)
            g = (v * _tile(cols[pl.ds(C_W2 * 128 + u * 8, 8), :], ND)) * t
            yacc = g if yacc is None else yacc + g
        y = (hn[0:1] * (r[0:1] + r[1:2] + _tile(consts[0:1, :], ND))
             + (r[2:3] + r[3:4] + _tile(consts[1:2, :], ND))
             + jnp.sum(yacc, axis=0, keepdims=True))
        MARK('gbw')
        cp(gbuf, gbuf, wsem.at[7]).wait()
        MARK('gb')
        gb = jnp.concatenate(
            [jnp.dot(sc16, gbuf[j].reshape(D, 128), preferred_element_type=F32)
             for j in range(ND)], axis=1)
        o_ref[0] = (x1[0:1] + gb[0:1] * y).astype(o_ref.dtype)
        MARK(None)

    return kernel


@jax.jit
def pallas_adaLN_cond__sliding_block_cached__mixer_token_mlp__decode_kernel(
    A_x: jax.Array,
    A_k_cache: jax.Array,
    A_v_cache: jax.Array,
    A_wq: jax.Array,
    A_wo: jax.Array,
    B_x: jax.Array,
    B_w1: jax.Array,
    B_b1: jax.Array,
    B_w2: jax.Array,
    B_b2: jax.Array,
    c: jax.Array,
    w_mod: jax.Array,
):
    SK = A_k_cache.shape[2]
    W = min(4096, max(256, SK // 4))
    kt = jnp.swapaxes(A_k_cache, 2, 3).reshape(H * DH, SK)
    vt = jnp.swapaxes(A_v_cache, 2, 3).reshape(H * DH, SK)

    vmem = pltpu.VMEM
    dma = pltpu.SemaphoreType.DMA
    return pl.pallas_call(
        _make_kernel(SK, W),
        out_shape=jax.ShapeDtypeStruct(A_x.shape, A_x.dtype),
        in_specs=[pl.BlockSpec(memory_space=pl.ANY)] * 11,
        out_specs=pl.BlockSpec(memory_space=pltpu.VMEM),
        scratch_shapes=[
            vmem((2, W // 128, DH, 128), BF16), vmem((2, W // 128, DH, 128), BF16),
            vmem((D // 8, H * DH // 256, 16, 128), BF16), vmem((H, G * ND // 2, 16, 128), BF16),
            vmem((DA, DB, 5 * D), BF16),
            vmem((1, 1, D), BF16), vmem((1, D), BF16),
            vmem((1, F), BF16), vmem((NF, 128), BF16), vmem((1, F), BF16),
            vmem((1,), BF16),
            vmem((H * DH, 128), F32), vmem((C_N, 128), F32), vmem((C_N * 128, 128), F32),
            vmem((8, F), F32), vmem((DH, 128), F32), vmem((W // 128, 8, 128), F32),
            vmem((4, 128), F32), vmem((1, 2 * D), F32),
            vmem((ND, DA, DB, 128), BF16),
            dma((2,)), dma((2,)), dma((16,)), dma((16,)), dma((9,)), dma((6,)),
        ],
        compiler_params=pltpu.CompilerParams(
            vmem_limit_bytes=64 * 1024 * 1024,
            disable_bounds_checks=True,
            disable_semaphore_checks=True,
        ),
    )(A_x, kt, vt, _pair_view(A_wq), _pair_view(A_wo), B_w1,
      B_b1.reshape(NF, 128), B_w2.reshape(1, F), B_b2, c, w_mod.reshape(DA, DB, 6 * D))
```

```python
import math

import jax
import jax.numpy as jnp
from jax import lax
import jax.experimental.pallas as pl
import jax.experimental.pallas.tpu as pltpu

F32 = jnp.float32
BF16 = jnp.bfloat16

D = 640
H = 32
DH = 192
F = 1536
EPS = 1e-5
G = DH // 8
ND = D // 128
NF = F // 128

LO, HI = 1, 0

_C0 = math.sqrt(2.0 / math.pi)
_C1 = 0.044715
KS = (_C0 * _C1) ** (1.0 / 3.0)
CS = _C0 / KS

C_W1, C_B1, C_SC, C_W2, C_N = 0, NF, 2 * NF, 2 * NF + ND, 30

DA, DB = 10, 64
TA, TB = 15, 128


def _pair_view(w):
    r, c = w.shape
    t = w.reshape(r // 8, 8, c // 128, 128).transpose(0, 2, 1, 3)
    return t.reshape(TA, TB, 16, 128)


def _layernorm(x):
    m = jnp.mean(x, axis=-1, keepdims=True)
    xc = x - m
    v = jnp.mean(xc * xc, axis=-1, keepdims=True)
    return xc * lax.rsqrt(v + EPS)


def _moments(x, mu0):
    d = x - mu0
    return d, jnp.sum(d, axis=-1, keepdims=True), jnp.sum(d * d, axis=-1, keepdims=True)


def _normalize(d, s1, s2):
    s1 = s1 * (1.0 / D)
    var = jnp.maximum(s2 * (1.0 / D) - s1 * s1, 0.0)
    return (d - s1) * lax.rsqrt(var + EPS)


def _col_bcast(row128):
    return jnp.broadcast_to(row128, (128, 128)).T


def _tile(x, n):
    return jnp.concatenate([x] * n, axis=1)


def _tree_sum(parts):
    while len(parts) > 1:
        nxt = [parts[2 * i] + parts[2 * i + 1] for i in range(len(parts) // 2)]
        if len(parts) % 2:
            nxt.append(parts[-1])
        parts = nxt
    return parts[0]


def _groups(x):
    return [x[j * 8:(j + 1) * 8, :] for j in range(x.shape[0] // 8)]


def _make_kernel(SK, W):
    KV_HI = 16
    KV_LO = DH - KV_HI
    W0 = SK - W
    NB = W // 128

    def kernel(x_hbm, k_hbm, v_hbm, wq_hbm, wo_hbm, w1_hbm, b1_hbm, w2_hbm, b2_hbm,
               c_hbm, wm_hbm, o_ref,
               kbuf, vbuf, wq_v, wo_v, wm_v, x_v, c_v, w1_v, b1_v, w2_v, b2_v,
               qb, rows, cols, lhs, abuf, sbuf, consts, modb, gbuf,
               klo, khi, vlo, vhi, wsem, ssem):
        cp = pltpu.make_async_copy
        m8 = lambda i: pl.multiple_of(i, 8)
        m128 = lambda i: pl.multiple_of(i, 128)
        MARK = lambda name: None

        def kv_stream(src, buf, lo_sem, hi_sem, h, slot, sem_of):
            def piece(c, r0, n, sem):
                return cp(src.at[pl.ds(m8(h * DH + r0), n), pl.ds(m128(W0 + c * 128), 128)],
                          buf.at[slot, c, pl.ds(r0, n), :], sem.at[sem_of(c)])
            return (lambda c: piece(c, 0, KV_LO, lo_sem),
                    lambda c: piece(c, KV_LO, KV_HI, hi_sem))

        k_stream = lambda h, slot: kv_stream(k_hbm, kbuf, klo, khi, h, slot, lambda c: slot)
        v_stream = lambda h, slot: kv_stream(v_hbm, vbuf, vlo, vhi, h, slot,
                                             lambda c: slot * (NB // 4) + (c >> 2))

        def w_piece(src, dst, a0, na, b, c0, n, sem):
            idx = (pl.ds(a0, na), pl.ds(m8(b * 8), 8), pl.ds(m128(c0), n))
            return cp(src.at[idx], dst.at[idx], sem)

        def m_pieces(b, part):
            out = []
            for na, c0, n in ([(DA, c * 384, 384) for c in range(5)]
                              + [(8, (3 + c) * D, D) for c in range(2)]):
                a0, na = {'all': (0, na), 'lo': (0, na - 1), 'hi': (na - 1, 1)}[part]
                out.append(w_piece(wm_hbm, wm_v, a0, na, b, c0, n,
                                   wsem.at[8 if part == 'hi' else 0]))
            return out

        def pair_stream(src, dst, s):
            dst = dst.reshape(TA, TB, 16, 128)

            def piece(i, a0, na, sem):
                idx = (pl.ds(a0, na), pl.ds(i, 1))
                return cp(src.at[idx], dst.at[idx], sem)
            return (lambda i: piece(i, 0, TA - 2, wsem.at[s]),
                    lambda i: piece(i, TA - 2, 2, wsem.at[s + 1]))
        q_stream = pair_stream(wq_hbm, wq_v, 1)
        o_stream = pair_stream(wo_hbm, wo_v, 3)

        def t8_piece(i):
            idx = (8, pl.ds(m8((i & 1) * 32), 32), pl.ds(m128(3 * D + (i >> 1) * 128), 128))
            return cp(wm_hbm.at[idx], wm_v.at[idx], wsem.at[5])
        t8_stream = (None, t8_piece)

        def slab(a, s, src):
            idx = (a, slice(None), pl.ds(3 * D, 2 * D))
            return cp(src.at[idx], wm_v.at[idx], wsem.at[s])

        gb_piece = lambda j: cp(wm_hbm.at[:, :, pl.ds(5 * D + j * 128, 128)], gbuf.at[j],
                                wsem.at[9 if j == ND - 1 else 7])

        def issue(stream, i):
            if stream[0] is not None:
                stream[0](i).start(priority=LO)
            stream[1](i).start(priority=HI)

        def step(cur, i, nxt=None, inxt=None):
            cur[0](i).wait()
            if nxt is not None:
                issue(nxt, inxt)
            cur[1](i).wait()

        def loop(n, body, init=0):
            return lax.fori_loop(0, n, body, init)

        def dma_loop(n, cur, i0, nxt, n0):
            def body(i, c):
                step(cur, i + i0, nxt, i + n0)
                return c
            loop(n, body)

        def wm_cols(c0, n, a0=0, na=DA):
            return wm_v[a0:a0 + na, :, pl.ds(c0, n)].reshape(na * DB, n)

        MARK('p_issue')
        for m in m_pieces(0, 'all'):
            m.start(priority=LO)
        smalls = [cp(s, d, ssem.at[n]) for n, (s, d) in enumerate(
            [(c_hbm, c_v), (x_hbm, x_v), (w1_hbm, w1_v), (b1_hbm, b1_v), (w2_hbm, w2_v),
             (b2_hbm, b2_v)])]
        for s in smalls:
            s.start(priority=HI)

        def _ma(b, c):
            for m in m_pieces(b + 1, 'all'):
                m.start(priority=LO)
            return c
        loop(3, _ma)

        MARK('p_ma')

        def _ma2(b, c):
            for m, lo, hi in zip(m_pieces(b, 'all'), m_pieces(b + 4, 'lo'), m_pieces(b + 4, 'hi')):
                m.wait()
                lo.start(priority=LO)
                hi.start(priority=HI)
            return c
        loop(4, _ma2)

        def _ma3(b, c):
            for u, (lo, hi) in enumerate(zip(m_pieces(b + 4, 'lo'), m_pieces(b + 4, 'hi'))):
                lo.wait()
                issue(q_stream, 7 * b + u)
                hi.wait()
            return c
        loop(4, _ma3)
        for s in smalls:
            s.wait()
        LQ = 28

        MARK('p_moda')
        c32 = c_v[...].astype(F32)
        sc = (c32 * jax.nn.sigmoid(c32)).astype(BF16)
        sc16 = jnp.broadcast_to(sc, (16, D))
        x32 = x_v[0].astype(F32)
        xn = _layernorm(x32)
        consts[2:3, :] = jnp.broadcast_to(jnp.mean(x32, axis=1, keepdims=True), (1, 128))
        w2h = w2_v[...].astype(F32) * 0.5
        w1f = w1_v[...].astype(F32)
        b1f = b1_v[...].astype(F32)
        scf = sc.astype(F32)
        for i in range(NF):
            rows[C_W1 + i:C_W1 + i + 1, :] = w1f[:, i * 128:(i + 1) * 128] * KS
        rows[C_B1:C_B1 + NF, :] = b1f * KS
        for i in range(ND):
            rows[C_SC + i:C_SC + i + 1, :] = scf[:, i * 128:(i + 1) * 128]
        rows[C_W2:C_W2 + 1, :] = w2h[:, F - 128:] * (1.0 / KS)
        dma_loop(2, q_stream, 0, q_stream, LQ)
        ca = jnp.dot(sc16, wm_cols(D, D), preferred_element_type=F32)
        dma_loop(3, q_stream, 2, q_stream, LQ + 2)
        sa = jnp.dot(sc16, wm_cols(0, D), preferred_element_type=F32)
        h8 = (xn * (1.0 + ca) + sa)[0:8].astype(BF16).astype(F32)
        dma_loop(3, q_stream, 5, q_stream, LQ + 5)
        ga = jnp.dot(sc16, wm_cols(2 * D, D), preferred_element_type=F32)[0:8]
        dma_loop(3, q_stream, 8, q_stream, LQ + 8)
        sb = jnp.dot(sc16[:, :512], wm_cols(3 * D, D, 0, 8), preferred_element_type=F32)[0:1]
        modb[:, :D] = sb
        dma_loop(3, q_stream, 11, q_stream, LQ + 11)
        modb[:, D:] = jnp.dot(sc16[:, :512], wm_cols(4 * D, D, 0, 8),
                              preferred_element_type=F32)[0:1]
        consts[3:4, :] = jnp.broadcast_to(jnp.mean(sb, axis=1, keepdims=True), (1, 128))
        dma_loop(3, q_stream, 14, q_stream, LQ + 14)

        b1row = jnp.concatenate([b1f[i:i + 1, :] for i in range(NF)], axis=1)
        pw = w1f * w2h
        pb = b1row * w2h
        pw_hi = pw.astype(BF16).astype(F32)
        pb_hi = pb.astype(BF16).astype(F32)
        rid = lax.broadcasted_iota(jnp.int32, (8, F), 0)
        lhs[...] = jnp.where(
            rid == 0, pw_hi, jnp.where(
                rid == 1, pw - pw_hi, jnp.where(
                    rid == 2, pb_hi, jnp.where(rid == 3, pb - pb_hi, 0.0))))
        sum_w = jnp.sum(pw, axis=1, keepdims=True)
        sum_b = jnp.sum(pb, axis=1, keepdims=True) + b2_v[...].astype(F32).reshape(1, 1)
        consts[0:1, :] = jnp.broadcast_to(sum_w, (1, 128))
        consts[1:2, :] = jnp.broadcast_to(sum_b, (1, 128))

        MARK('p_prep')

        def prep(i, c):
            step(q_stream, 5 * i + 17, q_stream, 5 * i + LQ + 17)
            for u in range(3):
                t = 3 * i + u
                cols[pl.ds(m128(t * 128), 128), :] = _col_bcast(rows[pl.ds(t, 1), :])
            dma_loop(4, q_stream, 5 * i + 18, q_stream, 5 * i + LQ + 18)
            return c
        loop(C_N // 3, prep)

        MARK('p_wq')
        dma_loop(128 - LQ - 67, q_stream, 67, q_stream, LQ + 67)
        dma_loop(LQ, q_stream, 128 - LQ, o_stream, 0)

        MARK('p_qproj')
        scale = DH ** -0.5

        def q_cols(i, q):
            for t in range(2):
                qb[pl.ds(m128(i * 256 + t * 128), 128), :] = _col_bcast(
                    q[0:1, t * 128:(t + 1) * 128])

        def qproj(i0, s0, n, nxt, n0):
            def body(i, q_prev):
                step(o_stream, s0 + i * n, nxt, n0 + i * n)
                q_cols(jnp.maximum(i + i0 - 1, 0), q_prev)
                w = wq_v[:, i + i0].astype(F32)
                w = jnp.concatenate([w[:, 0:8].reshape(D, 128), w[:, 8:16].reshape(D, 128)],
                                    axis=1)
                q = jnp.dot(h8, w, precision=lax.Precision.DEFAULT,
                            preferred_element_type=F32) * scale
                dma_loop(n - 1, o_stream, s0 + i * n + 1, nxt, n0 + i * n + 1)
                return q
            return body
        k0, v0 = k_stream(0, 0), v_stream(0, 0)
        q = loop(20, qproj(0, 0, 5, o_stream, LQ), jnp.zeros((8, 256), F32))
        q = loop(4, qproj(20, 100, 7, k0, 0), q)
        for c in range(LQ, NB):
            issue(k0, c)
        MARK('p_k0')
        step(k0, 0, v0, 0)
        q_cols(23, q)
        abuf[...] = jnp.zeros((DH, 128), F32)
        dma_loop(NB - 1, k0, 1, v0, 1)

        def proj(h, a, out):
            o = jnp.sum(a, axis=1, keepdims=True)
            outs = [out, None]
            for jj in range(G // 2):
                tiles = _groups(wo_v[h, jj * ND:(jj + 1) * ND].astype(F32).reshape(16 * ND, 128))
                for e in range(2):
                    j = 2 * jj + e
                    w = jnp.concatenate(tiles[e * ND:(e + 1) * ND], axis=1)
                    t = o[j * 8:(j + 1) * 8] * w
                    outs[e] = t if outs[e] is None else outs[e] + t
            return outs[0] + outs[1]

        def phase_a(h, slot, out, cur, nxt):
            q = qb[pl.ds(pl.multiple_of(h * DH, 64), DH), :]

            def body(i, m):
                step(cur, i, nxt, i)
                for u in range(2):
                    c = 2 * i + u
                    s = _tree_sum(_groups(kbuf[slot, c].astype(F32) * q))
                    s = jnp.broadcast_to(jnp.sum(s, axis=0, keepdims=True), (8, 128))
                    sbuf[c] = s
                    m = jnp.maximum(m, s)
                return m
            m = loop(NB // 2, body, jnp.full((8, 128), -jnp.inf, F32))
            step(cur, 16, nxt, 16)
            m = jnp.max(m, axis=1, keepdims=True)
            out = proj(jnp.maximum(h - 1, 0), abuf[...], out)
            dma_loop(3, cur, 17, nxt, 17)
            p = jnp.exp(sbuf[...] - m)
            sbuf[...] = p
            l = _tree_sum([p[c] for c in range(NB)])
            inv_l = 1.0 / jnp.sum(l, axis=1, keepdims=True)
            return inv_l, out

        def pv_tile(slot, c, acc):
            p = sbuf[c]
            return acc + vbuf[slot, c].astype(F32) * jnp.concatenate([p] * G, axis=0)

        def pv_done(acc, inv_l):
            return acc * jnp.concatenate([jnp.broadcast_to(inv_l, (8, 128))] * G, axis=0)

        def head(h, out):
            slot = h & 1
            nslot = 1 - slot
            knext = k_stream(h + 1, nslot)
            inv_l, out = phase_a(h, slot, out, v_stream(h, slot), knext)
            dma_loop(NB - 20, v_stream(h, slot), 20, knext, 20)

            def body(c, acc):
                step(knext, c, v_stream(h + 1, nslot), c)
                return pv_tile(slot, c, acc)
            abuf[...] = pv_done(loop(NB, body, jnp.zeros((DH, 128), F32)), inv_l)
            return out

        MARK('main')
        out = loop(H - 1, head, jnp.zeros((8, D), F32))

        MARK('qk31')
        hl = H - 1
        sl = hl % 2
        vl = v_stream(hl, sl)
        slab(9, 6, wm_hbm).start(priority=LO)
        for j in range(ND):
            gb_piece(j).start(priority=LO)
        inv_l, out = phase_a(hl, sl, out, vl, t8_stream)

        MARK('pv31')

        def body(i, acc):
            step(vl, 20 + i)
            for u in range(5):
                acc = pv_tile(sl, 5 * i + u, acc)
            return acc
        acc = loop(4, body, jnp.zeros((DH, 128), F32))

        def body(i, acc):
            step(vl, 24 + i)
            return pv_tile(sl, 20 + i, acc)
        acc = loop(8, body, acc)
        slab(8, 5, wm_v).wait()

        def matvec(acc, a):
            for u in range(DB // 8):
                s = cols[pl.ds(C_SC * 128 + a * DB + u * 8, 8), :]
                t = _tile(s, 2 * ND) * wm_v[a, pl.ds(u * 8, 8), pl.ds(3 * D, 2 * D)].astype(F32)
                acc = t if acc is None else acc + t
            return acc

        MARK('proj31')
        for c in range(28, NB):
            acc = pv_tile(sl, c, acc)
        out = proj(hl, pv_done(acc, inv_l), out)
        macc = matvec(None, 8)
        attn = jnp.sum(out, axis=0, keepdims=True)
        x1 = x32 + ga * attn
        mom = _moments(x1, _tile(consts[2:3, :], ND))

        MARK('w9')
        slab(9, 6, wm_hbm).wait()
        MARK('ln2')
        mod = jnp.sum(matvec(macc, 9), axis=0, keepdims=True) + modb[...]
        h2 = _normalize(*mom) * (1.0 + mod[:, D:]) + mod[:, :D]
        hn = _normalize(*_moments(h2, _tile(consts[3:4, :], ND)))

        MARK('mlp')

        def tanh_rows(b, u, hn):
            w1c = cols[pl.ds((C_W1 + b) * 128 + u * 8, 8), :]
            b1c = cols[pl.ds((C_B1 + b) * 128 + u * 8, 8), :]
            v = hn * _tile(w1c, ND) + _tile(b1c, ND)
            return v, jnp.tanh(v * (v * v + CS))

        r = None
        for b in range(NF - 1):
            ts = [tanh_rows(b, u, hn)[1] for u in range(16)]
            rb = jnp.dot(lhs[:, b * 128:(b + 1) * 128], jnp.concatenate(ts, axis=0),
                         precision=lax.Precision.DEFAULT, preferred_element_type=F32)
            r = rb if r is None else r + rb
        hl_ = hn + ts[0] * 0.0
        yacc = None
        for u in range(16):
            v, t = tanh_rows(NF - 1, u, hl_)
            g = (v * _tile(cols[pl.ds(C_W2 * 128 + u * 8, 8), :], ND)) * t
            yacc = g if yacc is None else yacc + g
        y = (hn[0:1] * (r[0:1] + r[1:2] + _tile(consts[0:1, :], ND))
             + (r[2:3] + r[3:4] + _tile(consts[1:2, :], ND))
             + jnp.sum(yacc, axis=0, keepdims=True))
        def gate_vpu(j):
            accs = [None] * 4
            for a in range(DA):
                w = _groups(gbuf[j, a].astype(F32))
                for u in range(DB // 8):
                    t = cols[pl.ds(C_SC * 128 + a * DB + u * 8, 8), :] * w[u]
                    accs[u % 4] = t if accs[u % 4] is None else accs[u % 4] + t
            return jnp.sum(_tree_sum(accs), axis=0, keepdims=True)

        MARK('gbw')
        for j in range(ND - 1):
            gb_piece(j).wait()
        MARK('gb')
        gb = [gate_vpu(j) for j in range(ND - 1)]
        res = x1[0:1, :D - 128] + jnp.concatenate(gb, axis=1) * y[:, :D - 128]
        MARK('gbw2')
        gb_piece(ND - 1).wait()
        MARK('gb2')
        res2 = x1[0:1, D - 128:] + gate_vpu(ND - 1) * y[:, D - 128:]
        o_ref[0] = jnp.concatenate([res, res2], axis=1).astype(o_ref.dtype)
        MARK(None)

    return kernel


@jax.jit
def pallas_adaLN_cond__sliding_block_cached__mixer_token_mlp__decode_kernel(
    A_x: jax.Array,
    A_k_cache: jax.Array,
    A_v_cache: jax.Array,
    A_wq: jax.Array,
    A_wo: jax.Array,
    B_x: jax.Array,
    B_w1: jax.Array,
    B_b1: jax.Array,
    B_w2: jax.Array,
    B_b2: jax.Array,
    c: jax.Array,
    w_mod: jax.Array,
):
    SK = A_k_cache.shape[2]
    W = min(4096, max(256, SK // 4))
    kt = jnp.swapaxes(A_k_cache, 2, 3).reshape(H * DH, SK)
    vt = jnp.swapaxes(A_v_cache, 2, 3).reshape(H * DH, SK)

    vmem = pltpu.VMEM
    dma = pltpu.SemaphoreType.DMA
    return pl.pallas_call(
        _make_kernel(SK, W),
        out_shape=jax.ShapeDtypeStruct(A_x.shape, A_x.dtype),
        in_specs=[pl.BlockSpec(memory_space=pl.ANY)] * 11,
        out_specs=pl.BlockSpec(memory_space=pltpu.VMEM),
        scratch_shapes=[
            vmem((2, W // 128, DH, 128), BF16), vmem((2, W // 128, DH, 128), BF16),
            vmem((D // 8, H * DH // 256, 16, 128), BF16), vmem((H, G * ND // 2, 16, 128), BF16),
            vmem((DA, DB, 5 * D), BF16),
            vmem((1, 1, D), BF16), vmem((1, D), BF16),
            vmem((1, F), BF16), vmem((NF, 128), BF16), vmem((1, F), BF16),
            vmem((1,), BF16),
            vmem((H * DH, 128), F32), vmem((C_N, 128), F32), vmem((C_N * 128, 128), F32),
            vmem((8, F), F32), vmem((DH, 128), F32), vmem((W // 128, 8, 128), F32),
            vmem((4, 128), F32), vmem((1, 2 * D), F32),
            vmem((ND, DA, DB, 128), BF16),
            dma((2,)), dma((2,)), dma((16,)), dma((16,)), dma((10,)), dma((6,)),
        ],
        compiler_params=pltpu.CompilerParams(
            vmem_limit_bytes=64 * 1024 * 1024,
            disable_bounds_checks=True,
            disable_semaphore_checks=True,
        ),
    )(A_x, kt, vt, _pair_view(A_wq), _pair_view(A_wo), B_w1,
      B_b1.reshape(NF, 128), B_w2.reshape(1, F), B_b2, c, w_mod.reshape(DA, DB, 6 * D))
```

```python
import math

import jax
import jax.numpy as jnp
from jax import lax
import jax.experimental.pallas as pl
import jax.experimental.pallas.tpu as pltpu

F32 = jnp.float32
BF16 = jnp.bfloat16

D = 640
H = 32
DH = 192
F = 1536
EPS = 1e-5
G = DH // 8
ND = D // 128
NF = F // 128

LO, HI = 1, 0

_C0 = math.sqrt(2.0 / math.pi)
_C1 = 0.044715
KS = (_C0 * _C1) ** (1.0 / 3.0)
CS = _C0 / KS

ORDER = 'ZZVVRZVRZVVRVRV'
NZ = ORDER.count('Z')
NV = NF - NZ
C_W1, C_B1, C_SC, C_W2, C_N = 0, NV, 2 * NV, 2 * NV + ND, 24

DA, DB = 10, 64
TA, TB = 15, 128


class _Group:
    def __init__(self, copies):
        self.copies = copies

    def start(self, priority):
        for c in self.copies:
            c.start(priority=priority)

    def wait(self):
        for c in self.copies:
            c.wait()


def _pair_view(w):
    r, c = w.shape
    t = w.reshape(r // 8, 8, c // 128, 128).transpose(0, 2, 1, 3)
    return t.reshape(TA, TB, 16, 128)


def _layernorm(x):
    m = jnp.mean(x, axis=-1, keepdims=True)
    xc = x - m
    v = jnp.mean(xc * xc, axis=-1, keepdims=True)
    return xc * lax.rsqrt(v + EPS)


def _moments(x, mu0):
    d = x - mu0
    return d, jnp.sum(d, axis=-1, keepdims=True), jnp.sum(d * d, axis=-1, keepdims=True)


def _normalize(d, s1, s2):
    s1 = s1 * (1.0 / D)
    var = jnp.maximum(s2 * (1.0 / D) - s1 * s1, 0.0)
    return (d - s1) * lax.rsqrt(var + EPS)


def _col_bcast(row128):
    return jnp.broadcast_to(row128, (128, 128)).T


def _tile(x, n):
    return jnp.concatenate([x] * n, axis=1)


def _tree_sum(parts):
    while len(parts) > 1:
        nxt = [parts[2 * i] + parts[2 * i + 1] for i in range(len(parts) // 2)]
        if len(parts) % 2:
            nxt.append(parts[-1])
        parts = nxt
    return parts[0]


def _groups(x):
    return [x[j * 8:(j + 1) * 8, :] for j in range(x.shape[0] // 8)]


def _make_kernel(SK, W):
    KV_HI = 16
    KV_LO = DH - KV_HI
    W0 = SK - W
    NB = W // 128

    def kernel(x_hbm, k_hbm, v_hbm, wq_hbm, wo_hbm, w1_hbm, b1_hbm, w2_hbm, b2_hbm,
               c_hbm, wm_hbm, o_ref,
               kbuf, vbuf, wq_v, wo_v, wm_v, x_v, c_v, w1_v, b1_v, w2_v, b2_v,
               qb, rows, cols, lhs, abuf, sbuf, consts, modb, gbuf, acol,
               klo, khi, vlo, vhi, wsem, ssem):
        cp = pltpu.make_async_copy
        m8 = lambda i: pl.multiple_of(i, 8)
        m128 = lambda i: pl.multiple_of(i, 128)
        MARK = lambda name: None

        def kv_stream(src, buf, lo_sem, hi_sem, h, slot, sem_of):
            def piece(c, r0, n, sem):
                return cp(src.at[pl.ds(m8(h * DH + r0), n), pl.ds(m128(W0 + c * 128), 128)],
                          buf.at[slot, c, pl.ds(r0, n), :], sem.at[sem_of(c)])
            return (lambda c: piece(c, 0, KV_LO, lo_sem),
                    lambda c: piece(c, KV_LO, KV_HI, hi_sem))

        k_stream = lambda h, slot: kv_stream(k_hbm, kbuf, klo, khi, h, slot, lambda c: slot)
        v_stream = lambda h, slot: kv_stream(v_hbm, vbuf, vlo, vhi, h, slot,
                                             lambda c: slot * (NB // 4) + (c >> 2))

        def w_piece(src, dst, a0, na, b, c0, n, sem):
            idx = (pl.ds(a0, na), pl.ds(m8(b * 8), 8), pl.ds(m128(c0), n))
            return cp(src.at[idx], dst.at[idx], sem)

        def m_pieces(b, part):
            out = []
            for na, c0, n in ([(DA, c * 384, 384) for c in range(5)]
                              + [(8, (3 + c) * D, D) for c in range(2)]):
                a0, na = {'all': (0, na), 'lo': (0, na - 1), 'hi': (na - 1, 1)}[part]
                out.append(w_piece(wm_hbm, wm_v, a0, na, b, c0, n,
                                   wsem.at[8 if part == 'hi' else 0]))
            return out

        def pair_stream(src, dst, s):
            dst = dst.reshape(TA, TB, 16, 128)

            def piece(i, a0, na, r0, nr, sem):
                idx = (pl.ds(a0, na), i, pl.ds(r0, nr))
                return cp(src.at[idx], dst.at[idx], sem)
            return (lambda i: _Group([piece(i, 0, TA, 0, 8, wsem.at[s]),
                                      piece(i, 0, TA - 3, 8, 8, wsem.at[s])]),
                    lambda i: piece(i, TA - 3, 3, 8, 8, wsem.at[s + 1]))
        q_stream = pair_stream(wq_hbm, wq_v, 1)
        o_stream = pair_stream(wo_hbm, wo_v, 3)

        def t8_piece(i):
            idx = (8, pl.ds(m8((i & 1) * 32), 32), pl.ds(m128(3 * D + (i >> 1) * 128), 128))
            return cp(wm_hbm.at[idx], wm_v.at[idx], wsem.at[5])
        t8_stream = (None, t8_piece)

        def slab(a, s, src):
            idx = (a, slice(None), pl.ds(3 * D, 2 * D))
            return cp(src.at[idx], wm_v.at[idx], wsem.at[s])

        gb_piece = lambda j: cp(wm_hbm.at[:, :, pl.ds(5 * D + j * 128, 128)], gbuf.at[j],
                                wsem.at[9 if j == ND - 1 else 7])

        def issue(stream, i):
            if stream[0] is not None:
                stream[0](i).start(priority=LO)
            stream[1](i).start(priority=HI)

        def step(cur, i, nxt=None, inxt=None):
            cur[0](i).wait()
            if nxt is not None:
                issue(nxt, inxt)
            cur[1](i).wait()

        def loop(n, body, init=0):
            return lax.fori_loop(0, n, body, init)

        def dma_loop(n, cur, i0, nxt, n0):
            def body(i, c):
                step(cur, i + i0, nxt, i + n0)
                return c
            loop(n, body)

        def wm_cols(c0, n, a0=0, na=DA):
            return wm_v[a0:a0 + na, :, pl.ds(c0, n)].reshape(na * DB, n)

        MARK('p_issue')
        for m in m_pieces(0, 'all'):
            m.start(priority=LO)
        smalls = [cp(s, d, ssem.at[n]) for n, (s, d) in enumerate(
            [(c_hbm, c_v), (x_hbm, x_v), (w1_hbm, w1_v), (b1_hbm, b1_v), (w2_hbm, w2_v),
             (b2_hbm, b2_v)])]
        for s in smalls:
            s.start(priority=HI)

        def _ma(b, c):
            for m in m_pieces(b + 1, 'all'):
                m.start(priority=LO)
            return c
        loop(3, _ma)

        MARK('p_ma')

        def _ma2(b, c):
            for m, lo, hi in zip(m_pieces(b, 'all'), m_pieces(b + 4, 'lo'), m_pieces(b + 4, 'hi')):
                m.wait()
                lo.start(priority=LO)
                hi.start(priority=HI)
            return c
        loop(4, _ma2)

        def _ma3(b, c):
            for u, (lo, hi) in enumerate(zip(m_pieces(b + 4, 'lo'), m_pieces(b + 4, 'hi'))):
                lo.wait()
                issue(q_stream, 7 * b + u)
                hi.wait()
            return c
        loop(4, _ma3)
        for s in smalls:
            s.wait()
        LQ = 28

        MARK('p_moda')
        c32 = c_v[...].astype(F32)
        sc = (c32 * jax.nn.sigmoid(c32)).astype(BF16)
        sc16 = jnp.broadcast_to(sc, (16, D))
        x32 = x_v[0].astype(F32)
        xn = _layernorm(x32)
        consts[2:3, :] = jnp.broadcast_to(jnp.mean(x32, axis=1, keepdims=True), (1, 128))
        w2h = w2_v[...].astype(F32) * 0.5
        w1f = w1_v[...].astype(F32)
        b1f = b1_v[...].astype(F32)
        scf = sc.astype(F32)
        for i in range(NV):
            rows[C_W1 + i:C_W1 + i + 1, :] = w1f[:, (NZ + i) * 128:(NZ + i + 1) * 128] * KS
        rows[C_B1:C_B1 + NV, :] = b1f[NZ:] * KS
        rows[C_W2 + 1:C_N, :] = jnp.zeros((C_N - C_W2 - 1, 128), F32)
        for i in range(ND):
            rows[C_SC + i:C_SC + i + 1, :] = scf[:, i * 128:(i + 1) * 128]
        rows[C_W2:C_W2 + 1, :] = w2h[:, F - 128:] * (1.0 / KS)
        dma_loop(2, q_stream, 0, q_stream, LQ)
        ca = jnp.dot(sc16, wm_cols(D, D), preferred_element_type=F32)
        dma_loop(3, q_stream, 2, q_stream, LQ + 2)
        sa = jnp.dot(sc16, wm_cols(0, D), preferred_element_type=F32)
        h8 = (xn * (1.0 + ca) + sa)[0:8].astype(BF16).astype(F32)
        dma_loop(3, q_stream, 5, q_stream, LQ + 5)
        ga = jnp.dot(sc16, wm_cols(2 * D, D), preferred_element_type=F32)[0:8]
        dma_loop(3, q_stream, 8, q_stream, LQ + 8)
        sb = jnp.dot(sc16[:, :512], wm_cols(3 * D, D, 0, 8), preferred_element_type=F32)[0:1]
        modb[:, :D] = sb
        dma_loop(3, q_stream, 11, q_stream, LQ + 11)
        modb[:, D:] = jnp.dot(sc16[:, :512], wm_cols(4 * D, D, 0, 8),
                              preferred_element_type=F32)[0:1]
        consts[3:4, :] = jnp.broadcast_to(jnp.mean(sb, axis=1, keepdims=True), (1, 128))
        dma_loop(3, q_stream, 14, q_stream, LQ + 14)

        b1row = jnp.concatenate([b1f[i:i + 1, :] for i in range(NF)], axis=1)
        pw = w1f * w2h
        pb = b1row * w2h
        pw_hi = pw.astype(BF16).astype(F32)
        pb_hi = pb.astype(BF16).astype(F32)
        rid = lax.broadcasted_iota(jnp.int32, (8, F), 0)
        lhs[...] = jnp.where(
            rid == 0, pw_hi, jnp.where(
                rid == 1, pw - pw_hi, jnp.where(
                    rid == 2, pb_hi, jnp.where(rid == 3, pb - pb_hi, 0.0))))
        sum_w = jnp.sum(pw, axis=1, keepdims=True)
        sum_b = jnp.sum(pb, axis=1, keepdims=True) + b2_v[...].astype(F32).reshape(1, 1)
        consts[0:1, :] = jnp.broadcast_to(sum_w, (1, 128))
        consts[1:2, :] = jnp.broadcast_to(sum_b, (1, 128))

        dma_loop(3, q_stream, 17, q_stream, LQ + 17)
        lo_of = lambda a: a - a.astype(BF16).astype(F32)
        al = w1f[:, :NZ * 128] * KS
        be = b1row[:, :NZ * 128] * KS
        a3 = al * al * al
        a2 = 3.0 * al * al * be
        a1 = al * (3.0 * be * be + CS)
        a0 = be * (be * be + CS)
        a0l = lo_of(a0)
        kid = lax.broadcasted_iota(jnp.int32, (16, NZ * 128), 0)
        at = jnp.zeros((16, NZ * 128), F32)
        for k, a in enumerate([a3, a3, lo_of(a3), a2, a2, lo_of(a2), a1, a1, lo_of(a1), a0, a0l, lo_of(a0l)]):
            at = jnp.where(kid == k, a, at)
        for b in range(NZ):
            acol[b * 128:(b + 1) * 128, :] = jnp.concatenate(
                [at[:, b * 128:(b + 1) * 128], jnp.zeros((112, 128), F32)], axis=0).T

        MARK('p_prep')

        def prep(i, c):
            step(q_stream, 5 * i + 20, q_stream, 5 * i + LQ + 20)
            for u in range(3):
                t = 3 * i + u
                cols[pl.ds(m128(t * 128), 128), :] = _col_bcast(rows[pl.ds(t, 1), :])
            dma_loop(4, q_stream, 5 * i + 21, q_stream, 5 * i + LQ + 21)
            return c
        loop(C_N // 3, prep)

        MARK('p_wq')
        dma_loop(128 - LQ - 60, q_stream, 60, q_stream, LQ + 60)
        dma_loop(LQ, q_stream, 128 - LQ, o_stream, 0)

        MARK('p_qproj')
        scale = DH ** -0.5

        def q_cols(i, q):
            for t in range(2):
                qb[pl.ds(m128(i * 256 + t * 128), 128), :] = _col_bcast(
                    q[0:1, t * 128:(t + 1) * 128])

        def qproj(i0, s0, n, nxt, n0):
            def body(i, q_prev):
                step(o_stream, s0 + i * n, nxt, n0 + i * n)
                q_cols(jnp.maximum(i + i0 - 1, 0), q_prev)
                w = wq_v[:, i + i0].astype(F32)
                w = jnp.concatenate([w[:, 0:8].reshape(D, 128), w[:, 8:16].reshape(D, 128)],
                                    axis=1)
                q = jnp.dot(h8, w, precision=lax.Precision.DEFAULT,
                            preferred_element_type=F32) * scale
                dma_loop(n - 1, o_stream, s0 + i * n + 1, nxt, n0 + i * n + 1)
                return q
            return body
        k0, v0 = k_stream(0, 0), v_stream(0, 0)
        q = loop(20, qproj(0, 0, 5, o_stream, LQ), jnp.zeros((8, 256), F32))
        q = loop(4, qproj(20, 100, 7, k0, 0), q)
        for c in range(LQ, NB):
            issue(k0, c)
        MARK('p_k0')
        step(k0, 0, v0, 0)
        q_cols(23, q)
        abuf[...] = jnp.zeros((DH, 128), F32)
        dma_loop(NB - 1, k0, 1, v0, 1)

        def proj(h, a, out):
            o = jnp.sum(a, axis=1, keepdims=True)
            outs = [out, None]
            for jj in range(G // 2):
                tiles = _groups(wo_v[h, jj * ND:(jj + 1) * ND].astype(F32).reshape(16 * ND, 128))
                for e in range(2):
                    j = 2 * jj + e
                    w = jnp.concatenate(tiles[e * ND:(e + 1) * ND], axis=1)
                    t = o[j * 8:(j + 1) * 8] * w
                    outs[e] = t if outs[e] is None else outs[e] + t
            return outs[0] + outs[1]

        def phase_a(h, slot, out, cur, nxt):
            q = qb[pl.ds(pl.multiple_of(h * DH, 64), DH), :]

            def body(i, m):
                step(cur, i, nxt, i)
                for u in range(2):
                    c = 2 * i + u
                    s = _tree_sum(_groups(kbuf[slot, c].astype(F32) * q))
                    s = jnp.broadcast_to(jnp.sum(s, axis=0, keepdims=True), (8, 128))
                    sbuf[c] = s
                    m = jnp.maximum(m, s)
                return m
            m = loop(NB // 2, body, jnp.full((8, 128), -jnp.inf, F32))
            step(cur, 16, nxt, 16)
            m = jnp.max(m, axis=1, keepdims=True)
            out = proj(jnp.maximum(h - 1, 0), abuf[...], out)
            dma_loop(3, cur, 17, nxt, 17)
            p = jnp.exp(sbuf[...] - m)
            sbuf[...] = p
            l = _tree_sum([p[c] for c in range(NB)])
            inv_l = 1.0 / jnp.sum(l, axis=1, keepdims=True)
            return inv_l, out

        def pv_tile(slot, c, acc):
            p = sbuf[c]
            return acc + vbuf[slot, c].astype(F32) * jnp.concatenate([p] * G, axis=0)

        def pv_done(acc, inv_l):
            return acc * jnp.concatenate([jnp.broadcast_to(inv_l, (8, 128))] * G, axis=0)

        def head(h, out):
            slot = h & 1
            nslot = 1 - slot
            knext = k_stream(h + 1, nslot)
            inv_l, out = phase_a(h, slot, out, v_stream(h, slot), knext)
            dma_loop(NB - 20, v_stream(h, slot), 20, knext, 20)

            def body(c, acc):
                step(knext, c, v_stream(h + 1, nslot), c)
                return pv_tile(slot, c, acc)
            abuf[...] = pv_done(loop(NB, body, jnp.zeros((DH, 128), F32)), inv_l)
            return out

        MARK('main')
        out = loop(H - 1, head, jnp.zeros((8, D), F32))

        MARK('qk31')
        hl = H - 1
        sl = hl % 2
        vl = v_stream(hl, sl)
        slab(9, 6, wm_hbm).start(priority=LO)
        for j in range(ND):
            gb_piece(j).start(priority=LO)
        inv_l, out = phase_a(hl, sl, out, vl, t8_stream)

        MARK('pv31')

        def body(i, acc):
            step(vl, 20 + i)
            for u in range(5):
                acc = pv_tile(sl, 5 * i + u, acc)
            return acc
        acc = loop(4, body, jnp.zeros((DH, 128), F32))

        def body(i, acc):
            step(vl, 24 + i)
            return pv_tile(sl, 20 + i, acc)
        acc = loop(8, body, acc)
        slab(8, 5, wm_v).wait()

        def matvec(acc, a):
            for u in range(DB // 8):
                s = cols[pl.ds(C_SC * 128 + a * DB + u * 8, 8), :]
                t = _tile(s, 2 * ND) * wm_v[a, pl.ds(u * 8, 8), pl.ds(3 * D, 2 * D)].astype(F32)
                acc = t if acc is None else acc + t
            return acc

        MARK('proj31')
        for c in range(28, NB):
            acc = pv_tile(sl, c, acc)
        out = proj(hl, pv_done(acc, inv_l), out)
        macc = matvec(None, 8)
        attn = jnp.sum(out, axis=0, keepdims=True)
        x1 = x32 + ga * attn
        mom = _moments(x1, _tile(consts[2:3, :], ND))

        MARK('w9')
        slab(9, 6, wm_hbm).wait()
        MARK('ln2')
        mod = jnp.sum(matvec(macc, 9), axis=0, keepdims=True) + modb[...]
        h2 = _normalize(*mom) * (1.0 + mod[:, D:]) + mod[:, :D]
        hn = _normalize(*_moments(h2, _tile(consts[3:4, :], ND)))

        MARK('mlp')

        def tanh_rows(b, u, hn):
            w1c = cols[pl.ds((C_W1 + b - NZ) * 128 + u * 8, 8), :]
            b1c = cols[pl.ds((C_B1 + b - NZ) * 128 + u * 8, 8), :]
            v = hn * _tile(w1c, ND) + _tile(b1c, ND)
            return v, jnp.tanh(v * (v * v + CS))

        p2 = hn * hn
        sid = lax.broadcasted_iota(jnp.int32, (8, D), 0)
        pw_ = jnp.where(sid < 3, p2 * hn, jnp.where(sid < 6, p2, hn))
        ptop = jnp.where((sid == 1) | (sid == 4) | (sid == 7), lo_of(pw_), pw_)
        pbot = jnp.where(sid == 0, hn, jnp.where(sid < 4, 1.0, 0.0))
        pmat = jnp.concatenate([ptop, pbot], axis=0)
        r = None
        nz, nv = 0, NZ
        zs = []
        for kind in ORDER:
            if kind == 'V':
                b = nv
                nv += 1
                ts = [tanh_rows(b, u, hn)[1] for u in range(16)]
                t = jnp.concatenate(ts, axis=0)
            elif kind == 'Z':
                zs.append(jnp.dot(acol[len(zs) * 128:(len(zs) + 1) * 128, 0:16], pmat,
                                  precision=lax.Precision.DEFAULT, preferred_element_type=F32))
                continue
            else:
                b = nz
                nz += 1
                t = jnp.tanh(zs[b])
            rb = jnp.dot(lhs[:, b * 128:(b + 1) * 128], t,
                         precision=lax.Precision.DEFAULT, preferred_element_type=F32)
            r = rb if r is None else r + rb
        hl_ = hn + ts[0] * 0.0
        yacc = None
        for u in range(16):
            v, t = tanh_rows(NF - 1, u, hl_)
            g = (v * _tile(cols[pl.ds(C_W2 * 128 + u * 8, 8), :], ND)) * t
            yacc = g if yacc is None else yacc + g
        y = (hn[0:1] * (r[0:1] + r[1:2] + _tile(consts[0:1, :], ND))
             + (r[2:3] + r[3:4] + _tile(consts[1:2, :], ND))
             + jnp.sum(yacc, axis=0, keepdims=True))
        def gate_vpu(j):
            accs = [None] * 4
            for a in range(DA):
                w = _groups(gbuf[j, a].astype(F32))
                for u in range(DB // 8):
                    t = cols[pl.ds(C_SC * 128 + a * DB + u * 8, 8), :] * w[u]
                    accs[u % 4] = t if accs[u % 4] is None else accs[u % 4] + t
            return jnp.sum(_tree_sum(accs), axis=0, keepdims=True)

        def gate_mxu(j):
            return jnp.dot(sc16, gbuf[j].reshape(D, 128), preferred_element_type=F32)[0:1]

        MARK('gbw')
        for j in range(ND - 1):
            gb_piece(j).wait()
        MARK('gb')
        gb = [gate_vpu(j) for j in range(4)]
        res = x1[0:1, :D - 128] + jnp.concatenate(gb, axis=1) * y[:, :D - 128]
        MARK('gbw2')
        gb_piece(ND - 1).wait()
        MARK('gb2')
        res2 = x1[0:1, D - 128:] + gate_vpu(ND - 1) * y[:, D - 128:]
        o_ref[0] = jnp.concatenate([res, res2], axis=1).astype(o_ref.dtype)
        MARK(None)

    return kernel


@jax.jit
def pallas_adaLN_cond__sliding_block_cached__mixer_token_mlp__decode_kernel(
    A_x: jax.Array,
    A_k_cache: jax.Array,
    A_v_cache: jax.Array,
    A_wq: jax.Array,
    A_wo: jax.Array,
    B_x: jax.Array,
    B_w1: jax.Array,
    B_b1: jax.Array,
    B_w2: jax.Array,
    B_b2: jax.Array,
    c: jax.Array,
    w_mod: jax.Array,
):
    SK = A_k_cache.shape[2]
    W = min(4096, max(256, SK // 4))
    kt = jnp.swapaxes(A_k_cache, 2, 3).reshape(H * DH, SK)
    vt = jnp.swapaxes(A_v_cache, 2, 3).reshape(H * DH, SK)

    vmem = pltpu.VMEM
    dma = pltpu.SemaphoreType.DMA
    return pl.pallas_call(
        _make_kernel(SK, W),
        out_shape=jax.ShapeDtypeStruct(A_x.shape, A_x.dtype),
        in_specs=[pl.BlockSpec(memory_space=pl.ANY)] * 11,
        out_specs=pl.BlockSpec(memory_space=pltpu.VMEM),
        scratch_shapes=[
            vmem((2, W // 128, DH, 128), BF16), vmem((2, W // 128, DH, 128), BF16),
            vmem((D // 8, H * DH // 256, 16, 128), BF16), vmem((H, G * ND // 2, 16, 128), BF16),
            vmem((DA, DB, 5 * D), BF16),
            vmem((1, 1, D), BF16), vmem((1, D), BF16),
            vmem((1, F), BF16), vmem((NF, 128), BF16), vmem((1, F), BF16),
            vmem((1,), BF16),
            vmem((H * DH, 128), F32), vmem((C_N, 128), F32), vmem((C_N * 128, 128), F32),
            vmem((8, F), F32), vmem((DH, 128), F32), vmem((W // 128, 8, 128), F32),
            vmem((4, 128), F32), vmem((1, 2 * D), F32),
            vmem((ND, DA, DB, 128), BF16), vmem((NZ * 128, 128), F32),
            dma((2,)), dma((2,)), dma((16,)), dma((16,)), dma((10,)), dma((6,)),
        ],
        compiler_params=pltpu.CompilerParams(
            vmem_limit_bytes=64 * 1024 * 1024,
            disable_bounds_checks=True,
            disable_semaphore_checks=True,
        ),
    )(A_x, kt, vt, _pair_view(A_wq), _pair_view(A_wo), B_w1,
      B_b1.reshape(NF, 128), B_w2.reshape(1, F), B_b2, c, w_mod.reshape(DA, DB, 6 * D))
```

```python
import math

import jax
import jax.numpy as jnp
from jax import lax
import jax.experimental.pallas as pl
import jax.experimental.pallas.tpu as pltpu

F32 = jnp.float32
BF16 = jnp.bfloat16

D = 640
H = 32
DH = 192
F = 1536
EPS = 1e-5
G = DH // 8
ND = D // 128
NF = F // 128

LO, HI = 1, 0

_C0 = math.sqrt(2.0 / math.pi)
_C1 = 0.044715
KS = (_C0 * _C1) ** (1.0 / 3.0)
CS = _C0 / KS

ORDER = 'ZVZVVRZVRVVRVV'
NZ = ORDER.count('Z')
NV = NF - NZ
C_W1, C_B1, C_SC, C_N = 0, NV, 2 * NV, 24

DA, DB = 10, 64
TA, TB = 15, 128


class _Group:
    def __init__(self, copies):
        self.copies = copies

    def start(self, priority):
        for c in self.copies:
            c.start(priority=priority)

    def wait(self):
        for c in self.copies:
            c.wait()


def _pair_view(w):
    r, c = w.shape
    t = w.reshape(r // 8, 8, c // 128, 128).transpose(0, 2, 1, 3)
    return t.reshape(TA, TB, 16, 128)


def _layernorm(x):
    m = jnp.mean(x, axis=-1, keepdims=True)
    xc = x - m
    v = jnp.mean(xc * xc, axis=-1, keepdims=True)
    return xc * lax.rsqrt(v + EPS)


def _moments(d):
    return _tree_sum(_blocks(d)), _tree_sum(_blocks(d * d))


def _lane_sums(xs):
    return [jnp.sum(x, axis=-1, keepdims=True) for x in xs]


def _normalize(d, s1, s2):
    s1 = s1 * (1.0 / D)
    var = jnp.maximum(s2 * (1.0 / D) - s1 * s1, 0.0)
    return (d - s1) * lax.rsqrt(var + EPS)


def _col_bcast(row128):
    return jnp.broadcast_to(row128, (128, 128)).T


def _tile(x, n):
    return jnp.concatenate([x] * n, axis=1)


def _tree_sum(parts):
    while len(parts) > 1:
        nxt = [parts[2 * i] + parts[2 * i + 1] for i in range(len(parts) // 2)]
        if len(parts) % 2:
            nxt.append(parts[-1])
        parts = nxt
    return parts[0]


def _blocks(x):
    return [x[:, j * 128:(j + 1) * 128] for j in range(x.shape[1] // 128)]


def _groups(x):
    return [x[j * 8:(j + 1) * 8, :] for j in range(x.shape[0] // 8)]


def _make_kernel(SK, W):
    KV_HI = 16
    KV_LO = DH - KV_HI
    W0 = SK - W
    NB = W // 128

    def kernel(x_hbm, k_hbm, v_hbm, wq_hbm, wo_hbm, w1_hbm, b1_hbm, w2_hbm, b2_hbm,
               c_hbm, wm_hbm, o_ref,
               kbuf, vbuf, wq_v, wo_v, wm_v, x_v, c_v, w1_v, b1_v, w2_v, b2_v,
               qb, rows, cols, lhs, abuf, sbuf, consts, modb, gbuf, acol, wo_last, tbuf,
               klo, khi, vlo, vhi, wsem, ssem):
        cp = pltpu.make_async_copy
        m8 = lambda i: pl.multiple_of(i, 8)
        m128 = lambda i: pl.multiple_of(i, 128)
        MARK = lambda name: None

        def kv_stream(src, buf, lo_sem, hi_sem, h, slot, sem_of):
            def piece(c, r0, n, sem):
                return cp(src.at[pl.ds(m8(h * DH + r0), n), pl.ds(m128(W0 + c * 128), 128)],
                          buf.at[slot, c, pl.ds(r0, n), :], sem.at[sem_of(c)])
            return (lambda c: piece(c, 0, KV_LO, lo_sem),
                    lambda c: piece(c, KV_LO, KV_HI, hi_sem))

        k_stream = lambda h, slot: kv_stream(k_hbm, kbuf, klo, khi, h, slot, lambda c: slot)
        v_stream = lambda h, slot: kv_stream(v_hbm, vbuf, vlo, vhi, h, slot,
                                             lambda c: slot * NB + c)

        def w_piece(src, dst, a0, na, b, c0, n, sem):
            idx = (pl.ds(a0, na), pl.ds(m8(b * 8), 8), pl.ds(m128(c0), n))
            return cp(src.at[idx], dst.at[idx], sem)

        def m_pieces(b, part):
            out = []
            for na, c0, n in ([(DA, c * 384, 384) for c in range(5)]
                              + [(8, (3 + c) * D, D) for c in range(2)]):
                a0, na = {'all': (0, na), 'lo': (0, na - 1), 'hi': (na - 1, 1)}[part]
                out.append(w_piece(wm_hbm, wm_v, a0, na, b, c0, n,
                                   wsem.at[8 if part == 'hi' else 0]))
            return out

        def pair_stream(src, dst, s):
            dst = dst.reshape(TA, TB, 16, 128)

            def piece(i, a0, na, r0, nr, sem):
                idx = (pl.ds(a0, na), i, pl.ds(r0, nr))
                return cp(src.at[idx], dst.at[idx], sem)
            return (lambda i: _Group([piece(i, 0, TA, 0, 8, wsem.at[s]),
                                      piece(i, 0, TA - 3, 8, 8, wsem.at[s])]),
                    lambda i: piece(i, TA - 3, 3, 8, 8, wsem.at[s + 1]))
        q_stream = pair_stream(wq_hbm, wq_v, 1)
        o_stream = pair_stream(wo_hbm, wo_v, 3)

        def t8_piece(i):
            idx = (8, pl.ds(m8((i & 1) * 32), 32), pl.ds(m128(3 * D + (i >> 1) * 128), 128))
            return cp(wm_hbm.at[idx], wm_v.at[idx], wsem.at[5])
        t8_stream = (None, t8_piece)

        def slab(a, s, src):
            idx = (a, slice(None), pl.ds(3 * D, 2 * D))
            return cp(src.at[idx], wm_v.at[idx], wsem.at[s])

        gb_piece = lambda j: cp(wm_hbm.at[:, :, pl.ds(5 * D + j * 128, 128)], gbuf.at[j],
                                wsem.at[(7, 7, 7, 9, 10)[j]])

        def issue(stream, i):
            if stream[0] is not None:
                stream[0](i).start(priority=LO)
            stream[1](i).start(priority=HI)

        def step(cur, i, nxt=None, inxt=None):
            cur[0](i).wait()
            if nxt is not None:
                issue(nxt, inxt)
            cur[1](i).wait()

        def loop(n, body, init=0):
            return lax.fori_loop(0, n, body, init)

        def dma_loop(n, cur, i0, nxt, n0):
            def body(i, c):
                step(cur, i + i0, nxt, i + n0)
                return c
            loop(n, body)

        def wm_cols(c0, n, a0=0, na=DA):
            return wm_v[a0:a0 + na, :, pl.ds(c0, n)].reshape(na * DB, n)

        MARK('p_issue')
        for m in m_pieces(0, 'all'):
            m.start(priority=LO)
        smalls = [cp(s, d, ssem.at[n]) for n, (s, d) in enumerate(
            [(c_hbm, c_v), (x_hbm, x_v), (w1_hbm, w1_v), (b1_hbm, b1_v), (w2_hbm, w2_v),
             (b2_hbm, b2_v)])]
        for s in smalls:
            s.start(priority=HI)

        def _ma(b, c):
            for m in m_pieces(b + 1, 'all'):
                m.start(priority=LO)
            return c
        loop(3, _ma)

        MARK('p_ma')

        def _ma2(b, c):
            for m, lo, hi in zip(m_pieces(b, 'all'), m_pieces(b + 4, 'lo'), m_pieces(b + 4, 'hi')):
                m.wait()
                lo.start(priority=LO)
                hi.start(priority=HI)
            return c
        loop(4, _ma2)

        def _ma3(b, c):
            for u, (lo, hi) in enumerate(zip(m_pieces(b + 4, 'lo'), m_pieces(b + 4, 'hi'))):
                lo.wait()
                issue(q_stream, 7 * b + u)
                hi.wait()
            return c
        loop(4, _ma3)
        for s in smalls:
            s.wait()
        LQ = 28

        MARK('p_moda')
        c32 = c_v[...].astype(F32)
        sc = (c32 * jax.nn.sigmoid(c32)).astype(BF16)
        sc16 = jnp.broadcast_to(sc, (16, D))
        x32 = x_v[0].astype(F32)
        xn = _layernorm(x32)
        consts[2:3, :] = jnp.broadcast_to(jnp.mean(x32, axis=1, keepdims=True), (1, 128))
        w2h = w2_v[...].astype(F32) * 0.5
        w1f = w1_v[...].astype(F32)
        b1f = b1_v[...].astype(F32)
        scf = sc.astype(F32)
        for i in range(NV):
            rows[C_W1 + i:C_W1 + i + 1, :] = w1f[:, (NZ + i) * 128:(NZ + i + 1) * 128] * KS
        rows[C_B1:C_B1 + NV, :] = b1f[NZ:] * KS
        rows[C_SC + ND:C_N, :] = jnp.zeros((C_N - C_SC - ND, 128), F32)
        for i in range(ND):
            rows[C_SC + i:C_SC + i + 1, :] = scf[:, i * 128:(i + 1) * 128]
        dma_loop(2, q_stream, 0, q_stream, LQ)
        ca = jnp.dot(sc16, wm_cols(D, D), preferred_element_type=F32)
        dma_loop(3, q_stream, 2, q_stream, LQ + 2)
        sa = jnp.dot(sc16, wm_cols(0, D), preferred_element_type=F32)
        h8 = (xn * (1.0 + ca) + sa)[0:8].astype(BF16).astype(F32)
        dma_loop(3, q_stream, 5, q_stream, LQ + 5)
        ga = jnp.dot(sc16, wm_cols(2 * D, D), preferred_element_type=F32)[0:8]
        dma_loop(3, q_stream, 8, q_stream, LQ + 8)
        sb = jnp.dot(sc16[:, :512], wm_cols(3 * D, D, 0, 8), preferred_element_type=F32)[0:1]
        modb[:, :D] = sb
        dma_loop(3, q_stream, 11, q_stream, LQ + 11)
        modb[:, D:] = jnp.dot(sc16[:, :512], wm_cols(4 * D, D, 0, 8),
                              preferred_element_type=F32)[0:1]
        consts[3:4, :] = jnp.broadcast_to(jnp.mean(sb, axis=1, keepdims=True), (1, 128))
        dma_loop(3, q_stream, 14, q_stream, LQ + 14)

        b1row = jnp.concatenate([b1f[i:i + 1, :] for i in range(NF)], axis=1)
        pw = w1f * w2h
        pb = b1row * w2h
        pw_hi = pw.astype(BF16).astype(F32)
        pb_hi = pb.astype(BF16).astype(F32)
        rid = lax.broadcasted_iota(jnp.int32, (8, F), 0)
        lhs[...] = jnp.where(
            rid == 0, pw_hi, jnp.where(
                rid == 1, pw - pw_hi, jnp.where(
                    rid == 2, pb_hi, jnp.where(rid == 3, pb - pb_hi, 0.0))))
        sum_w = jnp.sum(pw, axis=1, keepdims=True)
        sum_b = jnp.sum(pb, axis=1, keepdims=True) + b2_v[...].astype(F32).reshape(1, 1)
        consts[0:1, :] = jnp.broadcast_to(sum_w, (1, 128))
        consts[1:2, :] = jnp.broadcast_to(sum_b, (1, 128))

        dma_loop(3, q_stream, 17, q_stream, LQ + 17)
        lo_of = lambda a: a - a.astype(BF16).astype(F32)
        al = w1f[:, :NZ * 128] * KS
        be = b1row[:, :NZ * 128] * KS
        a3 = al * al * al
        a2 = 3.0 * al * al * be
        a1 = al * (3.0 * be * be + CS)
        a0 = be * (be * be + CS)
        a0l = lo_of(a0)
        kid = lax.broadcasted_iota(jnp.int32, (16, NZ * 128), 0)
        at = jnp.zeros((16, NZ * 128), F32)
        for k, a in enumerate([a3, a3, lo_of(a3), a2, a2, lo_of(a2), a1, a1, lo_of(a1), a0, a0l, lo_of(a0l)]):
            at = jnp.where(kid == k, a, at)
        for b in range(NZ):
            acol[b * 128:(b + 1) * 128, :] = jnp.concatenate(
                [at[:, b * 128:(b + 1) * 128], jnp.zeros((112, 128), F32)], axis=0).T

        MARK('p_prep')

        def prep(i, c):
            step(q_stream, 5 * i + 20, q_stream, 5 * i + LQ + 20)
            for u in range(3):
                t = 3 * i + u
                cols[pl.ds(m128(t * 128), 128), :] = _col_bcast(rows[pl.ds(t, 1), :])
            dma_loop(4, q_stream, 5 * i + 21, q_stream, 5 * i + LQ + 21)
            return c
        loop(C_N // 3, prep)

        MARK('p_wq')
        dma_loop(128 - LQ - 60, q_stream, 60, q_stream, LQ + 60)
        dma_loop(LQ, q_stream, 128 - LQ, o_stream, 0)

        MARK('p_qproj')
        scale = DH ** -0.5

        def q_cols(i, q):
            for t in range(2):
                qb[pl.ds(m128(i * 256 + t * 128), 128), :] = _col_bcast(
                    q[0:1, t * 128:(t + 1) * 128])

        def qproj(i0, s0, n, nxt, n0):
            def body(i, q_prev):
                step(o_stream, s0 + i * n, nxt, n0 + i * n)
                q_cols(jnp.maximum(i + i0 - 1, 0), q_prev)
                w = wq_v[:, i + i0].astype(F32)
                w = jnp.concatenate([w[:, 0:8].reshape(D, 128), w[:, 8:16].reshape(D, 128)],
                                    axis=1)
                q = jnp.dot(h8, w, precision=lax.Precision.DEFAULT,
                            preferred_element_type=F32) * scale
                dma_loop(n - 1, o_stream, s0 + i * n + 1, nxt, n0 + i * n + 1)
                return q
            return body
        k0, v0 = k_stream(0, 0), v_stream(0, 0)
        q = loop(20, qproj(0, 0, 5, o_stream, LQ), jnp.zeros((8, 256), F32))
        q = loop(4, qproj(20, 100, 7, k0, 0), q)
        for c in range(LQ, NB):
            issue(k0, c)
        MARK('p_k0')
        step(k0, 0, v0, 0)
        q_cols(23, q)
        abuf[...] = jnp.zeros((DH, 128), F32)
        wo_last[...] = wo_v[H - 1].astype(F32).reshape(G * ND, 8, 128)
        dma_loop(NB - 1, k0, 1, v0, 1)

        def proj(h, a, out):
            o = jnp.sum(a, axis=1, keepdims=True)
            outs = [out, None]
            for jj in range(G // 2):
                tiles = _groups(wo_v[h, jj * ND:(jj + 1) * ND].astype(F32).reshape(16 * ND, 128))
                for e in range(2):
                    j = 2 * jj + e
                    w = jnp.concatenate(tiles[e * ND:(e + 1) * ND], axis=1)
                    t = o[j * 8:(j + 1) * 8] * w
                    outs[e] = t if outs[e] is None else outs[e] + t
            return outs[0] + outs[1]

        def phase_a(h, slot, out, cur, nxt, tps, n1):
            q = qb[pl.ds(pl.multiple_of(h * DH, 64), DH), :]

            def body(i, m):
                step(cur, i, nxt, i)
                for u in range(tps):
                    c = tps * i + u
                    s = _tree_sum(_groups(kbuf[slot, c].astype(F32) * q))
                    s = jnp.broadcast_to(jnp.sum(s, axis=0, keepdims=True), (8, 128))
                    sbuf[c] = s
                    m = jnp.maximum(m, s)
                return m
            n0 = NB // tps
            m = loop(n0, body, jnp.full((8, 128), -jnp.inf, F32))
            if n1 == 1:
                step(cur, n0, nxt, n0)
            else:
                dma_loop(n1, cur, n0, nxt, n0)
            m = jnp.max(m, axis=1, keepdims=True)
            out = proj(jnp.maximum(h - 1, 0), abuf[...], out)
            dma_loop(3, cur, n0 + n1, nxt, n0 + n1)
            p = jnp.exp(sbuf[...] - m)
            sbuf[...] = p
            l = _tree_sum([p[c] for c in range(NB)])
            inv_l = 1.0 / jnp.sum(l, axis=1, keepdims=True)
            return inv_l, out

        def pv_tile(slot, c, acc):
            p = sbuf[c]
            return acc + vbuf[slot, c].astype(F32) * jnp.concatenate([p] * G, axis=0)

        def pv_done(acc, inv_l):
            return acc * jnp.concatenate([jnp.broadcast_to(inv_l, (8, 128))] * G, axis=0)

        def head(h, out):
            slot = h & 1
            nslot = 1 - slot
            knext = k_stream(h + 1, nslot)
            inv_l, out = phase_a(h, slot, out, v_stream(h, slot), knext, 2, 1)
            dma_loop(NB - 20, v_stream(h, slot), 20, knext, 20)

            def body(c, acc):
                step(knext, c, v_stream(h + 1, nslot), c)
                return pv_tile(slot, c, acc)
            abuf[...] = pv_done(loop(NB, body, jnp.zeros((DH, 128), F32)), inv_l)
            return out

        MARK('main')
        out = loop(H - 1, head, jnp.zeros((8, D), F32))

        MARK('qk31')
        hl = H - 1
        sl = hl % 2
        vl = v_stream(hl, sl)
        slab(9, 6, wm_hbm).start(priority=LO)
        for j in range(ND):
            gb_piece(j).start(priority=LO)
        inv_l, out = phase_a(hl, sl, out, vl, t8_stream, 4, 3)

        MARK('pv31')

        def pv2(i0, nxt):
            def body(i, acc):
                i = i + i0
                step(vl, 14 + i, nxt, 14 + i)
                return pv_tile(sl, 2 * i + 1, pv_tile(sl, 2 * i, acc))
            return body
        acc = loop(6, pv2(0, t8_stream), jnp.zeros((DH, 128), F32))
        acc = loop(8, pv2(6, None), acc)
        xp = x32 + ga * jnp.sum(out, axis=0, keepdims=True)
        gl = ga * inv_l

        def body(i, acc):
            step(vl, 28 + i)
            return pv_tile(sl, 28 + i, acc)
        acc = loop(3, body, acc)
        def matvec(acc, a):
            for u in range(DB // 8):
                s = cols[pl.ds(C_SC * 128 + a * DB + u * 8, 8), :]
                t = _tile(s, 2 * ND) * wm_v[a, pl.ds(u * 8, 8), pl.ds(3 * D, 2 * D)].astype(F32)
                acc = t if acc is None else acc + t
            return acc

        slab(8, 5, wm_v).wait()
        macc = matvec(None, 8)
        MARK('wlast')
        step(vl, NB - 1)
        MARK('proj31')
        o = jnp.sum(pv_tile(sl, NB - 1, acc), axis=1, keepdims=True)
        outs = [None, None]
        for j in range(G):
            w = jnp.concatenate([wo_last[j * ND + n] for n in range(ND)], axis=1)
            t = o[j * 8:(j + 1) * 8] * w
            outs[j & 1] = t if outs[j & 1] is None else outs[j & 1] + t
        x1 = xp + gl * jnp.sum(outs[0] + outs[1], axis=0, keepdims=True)
        d1 = x1 - _tile(consts[2:3, :], ND)
        mom = _moments(d1)

        MARK('w9')
        slab(9, 6, wm_hbm).wait()
        MARK('ln2')
        mom = _lane_sums(mom)
        mod = jnp.sum(matvec(macc, 9), axis=0, keepdims=True) + modb[...]
        scale_b = jnp.broadcast_to(1.0 + mod[:, D:], (8, D))
        shift_b = jnp.broadcast_to(mod[:, :D] - _tile(consts[3:4, :], ND), (8, D))
        d2 = _normalize(d1, *mom) * scale_b + shift_b
        hn = _normalize(d2, *_lane_sums(_moments(d2)))

        MARK('mlp')

        def tanh_rows(b, u, hn):
            w1c = cols[pl.ds((C_W1 + b - NZ) * 128 + u * 8, 8), :]
            b1c = cols[pl.ds((C_B1 + b - NZ) * 128 + u * 8, 8), :]
            v = hn * _tile(w1c, ND) + _tile(b1c, ND)
            return v, jnp.tanh(v * (v * v + CS))

        p2 = hn * hn
        sid = lax.broadcasted_iota(jnp.int32, (8, D), 0)
        pw_ = jnp.where(sid < 3, p2 * hn, jnp.where(sid < 6, p2, hn))
        ptop = jnp.where((sid == 1) | (sid == 4) | (sid == 7), lo_of(pw_), pw_)
        pbot = jnp.where(sid == 0, hn, jnp.where(sid < 4, 1.0, 0.0))
        pmat = jnp.concatenate([ptop, pbot], axis=0)
        r = None
        nz, nv = 0, NZ
        zs = []
        for kind in ORDER:
            if kind == 'V':
                b = nv
                nv += 1
                ts = [tanh_rows(b, u, hn)[1] for u in range(16)]
                t = jnp.concatenate(ts, axis=0)
            elif kind == 'Z':
                zs.append(jnp.dot(acol[len(zs) * 128:(len(zs) + 1) * 128, 0:16], pmat,
                                  precision=lax.Precision.DEFAULT, preferred_element_type=F32))
                continue
            else:
                b = nz
                nz += 1
                t = jnp.tanh(zs[b])
            rb = jnp.dot(lhs[:, b * 128:(b + 1) * 128], t,
                         precision=lax.Precision.DEFAULT, preferred_element_type=F32)
            r = rb if r is None else r + rb
        hl_ = hn + _tile(_tree_sum(_blocks(ts[0])) * 0.0, ND)
        for u in range(16):
            tbuf[u * 8:(u + 1) * 8, :] = tanh_rows(NF - 1, u, hl_)[1]

        def gates(js):
            na = 4 if len(js) == 1 else 2
            accs = [[None] * na for _ in js]
            for a in range(DA):
                ws = [_groups(gbuf[j, a].astype(F32)) for j in js]
                for u in range(DB // 8):
                    s = cols[pl.ds(C_SC * 128 + a * DB + u * 8, 8), :]
                    for acc, w in zip(accs, ws):
                        t = s * w[u]
                        acc[u % na] = t if acc[u % na] is None else acc[u % na] + t
            return jnp.concatenate(
                [jnp.sum(_tree_sum(acc), axis=0, keepdims=True) for acc in accs], axis=1)

        MARK('gbw')
        for j in range(3):
            gb_piece(j).wait()
        MARK('gb')
        r = r + jnp.dot(lhs[:, F - 128:], tbuf[...],
                        precision=lax.Precision.DEFAULT, preferred_element_type=F32)
        gb = [gates(range(3))]
        y = (hn[0:1] * (r[0:1] + r[1:2] + _tile(consts[0:1, :], ND))
             + (r[2:3] + r[3:4] + _tile(consts[1:2, :], ND)))
        MARK('gbw2')
        gb_piece(3).wait()
        MARK('gb2')
        gb.append(gates([3]))
        MARK('gbw3')
        gb_piece(4).wait()
        MARK('gb3')
        gb.append(gates([4]))
        o_ref[0] = (x1[0:1] + jnp.concatenate(gb, axis=1) * y).astype(o_ref.dtype)
        MARK(None)

    return kernel


@jax.jit
def pallas_adaLN_cond__sliding_block_cached__mixer_token_mlp__decode_kernel(
    A_x: jax.Array,
    A_k_cache: jax.Array,
    A_v_cache: jax.Array,
    A_wq: jax.Array,
    A_wo: jax.Array,
    B_x: jax.Array,
    B_w1: jax.Array,
    B_b1: jax.Array,
    B_w2: jax.Array,
    B_b2: jax.Array,
    c: jax.Array,
    w_mod: jax.Array,
):
    SK = A_k_cache.shape[2]
    W = min(4096, max(256, SK // 4))
    kt = jnp.swapaxes(A_k_cache, 2, 3).reshape(H * DH, SK)
    vt = jnp.swapaxes(A_v_cache, 2, 3).reshape(H * DH, SK)

    vmem = pltpu.VMEM
    dma = pltpu.SemaphoreType.DMA
    return pl.pallas_call(
        _make_kernel(SK, W),
        out_shape=jax.ShapeDtypeStruct(A_x.shape, A_x.dtype),
        in_specs=[pl.BlockSpec(memory_space=pl.ANY)] * 11,
        out_specs=pl.BlockSpec(memory_space=pltpu.VMEM),
        scratch_shapes=[
            vmem((2, W // 128, DH, 128), BF16), vmem((2, W // 128, DH, 128), BF16),
            vmem((D // 8, H * DH // 256, 16, 128), BF16), vmem((H, G * ND // 2, 16, 128), BF16),
            vmem((DA, DB, 5 * D), BF16),
            vmem((1, 1, D), BF16), vmem((1, D), BF16),
            vmem((1, F), BF16), vmem((NF, 128), BF16), vmem((1, F), BF16),
            vmem((1,), BF16),
            vmem((H * DH, 128), F32), vmem((C_N, 128), F32), vmem((C_N * 128, 128), F32),
            vmem((8, F), F32), vmem((DH, 128), F32), vmem((W // 128, 8, 128), F32),
            vmem((4, 128), F32), vmem((1, 2 * D), F32),
            vmem((ND, DA, DB, 128), BF16), vmem((NZ * 128, 128), F32),
            vmem((G * ND, 8, 128), F32), vmem((128, D), F32),
            dma((2,)), dma((2,)), dma((64,)), dma((64,)), dma((11,)), dma((6,)),
        ],
        compiler_params=pltpu.CompilerParams(
            vmem_limit_bytes=64 * 1024 * 1024,
            disable_bounds_checks=True,
            disable_semaphore_checks=True,
        ),
    )(A_x, kt, vt, _pair_view(A_wq), _pair_view(A_wo), B_w1,
      B_b1.reshape(NF, 128), B_w2.reshape(1, F), B_b2, c, w_mod.reshape(DA, DB, 6 * D))
```

```python
import math

import jax
import jax.numpy as jnp
from jax import lax
import jax.experimental.pallas as pl
import jax.experimental.pallas.tpu as pltpu

F32 = jnp.float32
BF16 = jnp.bfloat16

D = 640
H = 32
DH = 192
F = 1536
EPS = 1e-5
G = DH // 8
ND = D // 128
NF = F // 128

LO, HI = 1, 0

_C0 = math.sqrt(2.0 / math.pi)
_C1 = 0.044715
KS = (_C0 * _C1) ** (1.0 / 3.0)
CS = _C0 / KS

ORDER = 'ZVZVVRZVRVVRVV'
NZ = ORDER.count('Z')
NV = NF - NZ
C_W1, C_B1, C_SC, C_N = 0, NV, 2 * NV, 24

DA, DB = 10, 64
TA, TB = 15, 128


class _Group:
    def __init__(self, copies):
        self.copies = copies

    def start(self, priority):
        for c in self.copies:
            c.start(priority=priority)

    def wait(self):
        for c in self.copies:
            c.wait()


def _pair_view(w):
    r, c = w.shape
    t = w.reshape(r // 8, 8, c // 128, 128).transpose(0, 2, 1, 3)
    return t.reshape(TA, TB, 16, 128)


def _layernorm(x):
    m = jnp.mean(x, axis=-1, keepdims=True)
    xc = x - m
    v = jnp.mean(xc * xc, axis=-1, keepdims=True)
    return xc * lax.rsqrt(v + EPS)


def _moments(d):
    return _tree_sum(_blocks(d)), _tree_sum(_blocks(d * d))


def _lane_sums(xs):
    return [jnp.sum(x, axis=-1, keepdims=True) for x in xs]


def _normalize(d, s1, s2):
    s1 = s1 * (1.0 / D)
    var = jnp.maximum(s2 * (1.0 / D) - s1 * s1, 0.0)
    return (d - s1) * lax.rsqrt(var + EPS)


def _col_bcast(row128):
    return jnp.broadcast_to(row128, (128, 128)).T


def _tile(x, n):
    return jnp.concatenate([x] * n, axis=1)


def _tree_sum(parts):
    while len(parts) > 1:
        nxt = [parts[2 * i] + parts[2 * i + 1] for i in range(len(parts) // 2)]
        if len(parts) % 2:
            nxt.append(parts[-1])
        parts = nxt
    return parts[0]


def _blocks(x):
    return [x[:, j * 128:(j + 1) * 128] for j in range(x.shape[1] // 128)]


def _groups(x):
    return [x[j * 8:(j + 1) * 8, :] for j in range(x.shape[0] // 8)]


def _make_kernel(SK, W):
    KV_HI = 16
    KV_LO = DH - KV_HI
    W0 = SK - W
    NB = W // 128

    def kernel(x_hbm, k_hbm, v_hbm, wq_hbm, wo_hbm, w1_hbm, b1_hbm, w2_hbm, b2_hbm,
               c_hbm, wm_hbm, o_ref,
               kbuf, vbuf, wq_v, wo_v, wm_v, x_v, c_v, w1_v, b1_v, w2_v, b2_v,
               qb, rows, cols, lhs, abuf, sbuf, consts, modb, gbuf, acol, wo_last, tbuf,
               klo, khi, vlo, vhi, wsem, ssem):
        cp = pltpu.make_async_copy
        m8 = lambda i: pl.multiple_of(i, 8)
        m128 = lambda i: pl.multiple_of(i, 128)
        MARK = lambda name: None

        def kv_stream(src, buf, lo_sem, hi_sem, h, slot, sem_of):
            def piece(c, r0, n, sem):
                return cp(src.at[pl.ds(m8(h * DH + r0), n), pl.ds(m128(W0 + c * 128), 128)],
                          buf.at[slot, c, pl.ds(r0, n), :], sem.at[sem_of(c)])
            return (lambda c: piece(c, 0, KV_LO, lo_sem),
                    lambda c: piece(c, KV_LO, KV_HI, hi_sem))

        k_stream = lambda h, slot: kv_stream(k_hbm, kbuf, klo, khi, h, slot, lambda c: slot)
        v_stream = lambda h, slot: kv_stream(v_hbm, vbuf, vlo, vhi, h, slot,
                                             lambda c: slot * NB + c)

        def w_piece(src, dst, a0, na, b, c0, n, sem):
            idx = (pl.ds(a0, na), pl.ds(m8(b * 8), 8), pl.ds(m128(c0), n))
            return cp(src.at[idx], dst.at[idx], sem)

        def m_pieces(b, part):
            out = []
            for na, c0, n in ([(DA, c * 384, 384) for c in range(5)]
                              + [(8, (3 + c) * D, D) for c in range(2)]):
                a0, na = {'all': (0, na), 'lo': (0, na - 1), 'hi': (na - 1, 1)}[part]
                out.append(w_piece(wm_hbm, wm_v, a0, na, b, c0, n,
                                   wsem.at[8 if part == 'hi' else 0]))
            return out

        def pair_stream(src, dst, s):

            def piece(i, a0, na, r0, nr, sem):
                idx = (pl.ds(a0, na), i, pl.ds(r0, nr))
                return cp(src.at[idx], dst.at[idx], sem)
            return (lambda i: _Group([piece(i, 0, TA, 0, 8, wsem.at[s]),
                                      piece(i, 0, TA - 3, 8, 8, wsem.at[s])]),
                    lambda i: piece(i, TA - 3, 3, 8, 8, wsem.at[s + 1]))
        q_stream = pair_stream(wq_hbm, wq_v, 1)
        o_stream = pair_stream(wo_hbm, wo_v, 3)

        def t8_piece(i):
            idx = (8, pl.ds(m8((i & 1) * 32), 32), pl.ds(m128(3 * D + (i >> 1) * 128), 128))
            return cp(wm_hbm.at[idx], wm_v.at[idx], wsem.at[5])
        t8_stream = (None, t8_piece)

        def slab(a, s, src):
            idx = (a, slice(None), pl.ds(3 * D, 2 * D))
            return cp(src.at[idx], wm_v.at[idx], wsem.at[s])

        gb_piece = lambda j: cp(wm_hbm.at[:, :, pl.ds(5 * D + j * 128, 128)], gbuf.at[j],
                                wsem.at[(7, 7, 7, 9, 10)[j]])

        def issue(stream, i):
            if stream[0] is not None:
                stream[0](i).start(priority=LO)
            stream[1](i).start(priority=HI)

        def step(cur, i, nxt=None, inxt=None):
            cur[0](i).wait()
            if nxt is not None:
                issue(nxt, inxt)
            cur[1](i).wait()

        def pairs(ref, ps):
            return jnp.stack([ref[p >> 7, p & 127] for p in ps])

        def loop(n, body, init=0):
            return lax.fori_loop(0, n, body, init)

        def dma_loop(n, cur, i0, nxt, n0):
            def body(i, c):
                step(cur, i + i0, nxt, i + n0)
                return c
            loop(n, body)

        def wm_cols(c0, n, a0=0, na=DA):
            return wm_v[a0:a0 + na, :, pl.ds(c0, n)].reshape(na * DB, n)

        MARK('p_issue')
        for m in m_pieces(0, 'all'):
            m.start(priority=LO)
        smalls = [cp(s, d, ssem.at[n]) for n, (s, d) in enumerate(
            [(c_hbm, c_v), (x_hbm, x_v), (w1_hbm, w1_v), (b1_hbm, b1_v), (w2_hbm, w2_v),
             (b2_hbm, b2_v)])]
        for s in smalls:
            s.start(priority=HI)

        def _ma(b, c):
            for m in m_pieces(b + 1, 'all'):
                m.start(priority=LO)
            return c
        loop(3, _ma)

        MARK('p_ma')

        def _ma2(b, c):
            for m, lo, hi in zip(m_pieces(b, 'all'), m_pieces(b + 4, 'lo'), m_pieces(b + 4, 'hi')):
                m.wait()
                lo.start(priority=LO)
                hi.start(priority=HI)
            return c
        loop(4, _ma2)

        def _ma3(b, c):
            for u, (lo, hi) in enumerate(zip(m_pieces(b + 4, 'lo'), m_pieces(b + 4, 'hi'))):
                lo.wait()
                issue(q_stream, 7 * b + u)
                hi.wait()
            return c
        loop(4, _ma3)
        for s in smalls:
            s.wait()
        LQ = 28

        MARK('p_moda')
        c32 = c_v[...].astype(F32)
        sc = (c32 * jax.nn.sigmoid(c32)).astype(BF16)
        sc16 = jnp.broadcast_to(sc, (16, D))
        x32 = x_v[0].astype(F32)
        xn = _layernorm(x32)
        consts[2:3, :] = jnp.broadcast_to(jnp.mean(x32, axis=1, keepdims=True), (1, 128))
        w2h = w2_v[...].astype(F32) * 0.5
        w1f = w1_v[...].astype(F32)
        b1f = b1_v[...].astype(F32)
        scf = sc.astype(F32)
        for i in range(NV):
            rows[C_W1 + i:C_W1 + i + 1, :] = w1f[:, (NZ + i) * 128:(NZ + i + 1) * 128] * KS
        rows[C_B1:C_B1 + NV, :] = b1f[NZ:] * KS
        rows[C_SC + ND:C_N, :] = jnp.zeros((C_N - C_SC - ND, 128), F32)
        for i in range(ND):
            rows[C_SC + i:C_SC + i + 1, :] = scf[:, i * 128:(i + 1) * 128]
        dma_loop(2, q_stream, 0, q_stream, LQ)
        ca = jnp.dot(sc16, wm_cols(D, D), preferred_element_type=F32)
        dma_loop(3, q_stream, 2, q_stream, LQ + 2)
        sa = jnp.dot(sc16, wm_cols(0, D), preferred_element_type=F32)
        h8 = (xn * (1.0 + ca) + sa)[0:8].astype(BF16).astype(F32)
        dma_loop(3, q_stream, 5, q_stream, LQ + 5)
        ga = jnp.dot(sc16, wm_cols(2 * D, D), preferred_element_type=F32)[0:8]
        dma_loop(3, q_stream, 8, q_stream, LQ + 8)
        sb = jnp.dot(sc16[:, :512], wm_cols(3 * D, D, 0, 8), preferred_element_type=F32)[0:1]
        modb[:, :D] = sb
        dma_loop(3, q_stream, 11, q_stream, LQ + 11)
        modb[:, D:] = jnp.dot(sc16[:, :512], wm_cols(4 * D, D, 0, 8),
                              preferred_element_type=F32)[0:1]
        consts[3:4, :] = jnp.broadcast_to(jnp.mean(sb, axis=1, keepdims=True), (1, 128))
        dma_loop(3, q_stream, 14, q_stream, LQ + 14)

        b1row = jnp.concatenate([b1f[i:i + 1, :] for i in range(NF)], axis=1)
        pw = w1f * w2h
        pb = b1row * w2h
        pw_hi = pw.astype(BF16).astype(F32)
        pb_hi = pb.astype(BF16).astype(F32)
        rid = lax.broadcasted_iota(jnp.int32, (8, F), 0)
        lhs[...] = jnp.where(
            rid == 0, pw_hi, jnp.where(
                rid == 1, pw - pw_hi, jnp.where(
                    rid == 2, pb_hi, jnp.where(rid == 3, pb - pb_hi, 0.0))))
        sum_w = jnp.sum(pw, axis=1, keepdims=True)
        sum_b = jnp.sum(pb, axis=1, keepdims=True) + b2_v[...].astype(F32).reshape(1, 1)
        consts[0:1, :] = jnp.broadcast_to(sum_w, (1, 128))
        consts[1:2, :] = jnp.broadcast_to(sum_b, (1, 128))

        dma_loop(3, q_stream, 17, q_stream, LQ + 17)
        lo_of = lambda a: a - a.astype(BF16).astype(F32)
        al = w1f[:, :NZ * 128] * KS
        be = b1row[:, :NZ * 128] * KS
        a3 = al * al * al
        a2 = 3.0 * al * al * be
        a1 = al * (3.0 * be * be + CS)
        a0 = be * (be * be + CS)
        a0l = lo_of(a0)
        kid = lax.broadcasted_iota(jnp.int32, (16, NZ * 128), 0)
        at = jnp.zeros((16, NZ * 128), F32)
        for k, a in enumerate([a3, a3, lo_of(a3), a2, a2, lo_of(a2), a1, a1, lo_of(a1), a0, a0l, lo_of(a0l)]):
            at = jnp.where(kid == k, a, at)
        for b in range(NZ):
            acol[b * 128:(b + 1) * 128, :] = jnp.concatenate(
                [at[:, b * 128:(b + 1) * 128], jnp.zeros((112, 128), F32)], axis=0).T

        MARK('p_prep')

        def prep(i, c):
            step(q_stream, 5 * i + 20, q_stream, 5 * i + LQ + 20)
            for u in range(3):
                t = 3 * i + u
                cols[pl.ds(m128(t * 128), 128), :] = _col_bcast(rows[pl.ds(t, 1), :])
            dma_loop(4, q_stream, 5 * i + 21, q_stream, 5 * i + LQ + 21)
            return c
        loop(C_N // 3, prep)

        MARK('p_wq')
        dma_loop(128 - LQ - 60, q_stream, 60, q_stream, LQ + 60)
        dma_loop(LQ, q_stream, 128 - LQ, o_stream, 0)

        MARK('p_qproj')
        scale = DH ** -0.5

        def q_cols(i, q):
            for t in range(2):
                qb[pl.ds(m128(i * 256 + t * 128), 128), :] = _col_bcast(
                    q[0:1, t * 128:(t + 1) * 128])

        def qproj(i0, s0, n, nxt, n0):
            def body(i, q_prev):
                step(o_stream, s0 + i * n, nxt, n0 + i * n)
                q_cols(jnp.maximum(i + i0 - 1, 0), q_prev)
                w = pairs(wq_v, [24 * g + i + i0 for g in range(80)]).astype(F32)
                w = jnp.concatenate([w[:, 0:8].reshape(D, 128), w[:, 8:16].reshape(D, 128)],
                                    axis=1)
                q = jnp.dot(h8, w, precision=lax.Precision.DEFAULT,
                            preferred_element_type=F32) * scale
                dma_loop(n - 1, o_stream, s0 + i * n + 1, nxt, n0 + i * n + 1)
                return q
            return body
        k0, v0 = k_stream(0, 0), v_stream(0, 0)
        q = loop(20, qproj(0, 0, 5, o_stream, LQ), jnp.zeros((8, 256), F32))
        q = loop(4, qproj(20, 100, 7, k0, 0), q)
        for c in range(LQ, NB):
            issue(k0, c)
        MARK('p_k0')
        step(k0, 0, v0, 0)
        q_cols(23, q)
        abuf[...] = jnp.zeros((DH, 128), F32)
        wo_last[...] = pairs(wo_v, [60 * (H - 1) + p for p in range(60)]).astype(F32).reshape(G * ND, 8, 128)
        dma_loop(NB - 1, k0, 1, v0, 1)

        def proj(h, a, out):
            o = jnp.sum(a, axis=1, keepdims=True)
            outs = [out, None]
            for jj in range(G // 2):
                tiles = _groups(pairs(wo_v, [60 * h + jj * ND + p for p in range(ND)]).astype(F32).reshape(16 * ND, 128))
                for e in range(2):
                    j = 2 * jj + e
                    w = jnp.concatenate(tiles[e * ND:(e + 1) * ND], axis=1)
                    t = o[j * 8:(j + 1) * 8] * w
                    outs[e] = t if outs[e] is None else outs[e] + t
            return outs[0] + outs[1]

        def phase_a(h, slot, out, cur, nxt, tps, n1):
            q = qb[pl.ds(pl.multiple_of(h * DH, 64), DH), :]

            def body(i, m):
                step(cur, i, nxt, i)
                for u in range(tps):
                    c = tps * i + u
                    s = _tree_sum(_groups(kbuf[slot, c].astype(F32) * q))
                    s = jnp.broadcast_to(jnp.sum(s, axis=0, keepdims=True), (8, 128))
                    sbuf[c] = s
                    m = jnp.maximum(m, s)
                return m
            n0 = NB // tps
            m = loop(n0, body, jnp.full((8, 128), -jnp.inf, F32))
            if n1 == 1:
                step(cur, n0, nxt, n0)
            else:
                dma_loop(n1, cur, n0, nxt, n0)
            m = jnp.max(m, axis=1, keepdims=True)
            out = proj(jnp.maximum(h - 1, 0), abuf[...], out)
            dma_loop(3, cur, n0 + n1, nxt, n0 + n1)
            p = jnp.exp(sbuf[...] - m)
            sbuf[...] = p
            l = _tree_sum([p[c] for c in range(NB)])
            inv_l = 1.0 / jnp.sum(l, axis=1, keepdims=True)
            return inv_l, out

        def pv_tile(slot, c, acc):
            p = sbuf[c]
            return acc + vbuf[slot, c].astype(F32) * jnp.concatenate([p] * G, axis=0)

        def pv_done(acc, inv_l):
            return acc * jnp.concatenate([jnp.broadcast_to(inv_l, (8, 128))] * G, axis=0)

        def head(h, out):
            slot = h & 1
            nslot = 1 - slot
            knext = k_stream(h + 1, nslot)
            inv_l, out = phase_a(h, slot, out, v_stream(h, slot), knext, 2, 1)
            dma_loop(NB - 20, v_stream(h, slot), 20, knext, 20)

            def body(c, acc):
                step(knext, c, v_stream(h + 1, nslot), c)
                return pv_tile(slot, c, acc)
            abuf[...] = pv_done(loop(NB, body, jnp.zeros((DH, 128), F32)), inv_l)
            return out

        MARK('main')
        out = loop(H - 1, head, jnp.zeros((8, D), F32))

        MARK('qk31')
        hl = H - 1
        sl = hl % 2
        vl = v_stream(hl, sl)
        slab(9, 6, wm_hbm).start(priority=LO)
        for j in range(ND):
            gb_piece(j).start(priority=LO)
        inv_l, out = phase_a(hl, sl, out, vl, t8_stream, 4, 3)

        MARK('pv31')

        def pv2(i0, nxt):
            def body(i, acc):
                i = i + i0
                step(vl, 14 + i, nxt, 14 + i)
                return pv_tile(sl, 2 * i + 1, pv_tile(sl, 2 * i, acc))
            return body
        acc = loop(6, pv2(0, t8_stream), jnp.zeros((DH, 128), F32))
        acc = loop(8, pv2(6, None), acc)
        xp = x32 + ga * jnp.sum(out, axis=0, keepdims=True)
        gl = ga * inv_l

        def body(i, acc):
            step(vl, 28 + i)
            return pv_tile(sl, 28 + i, acc)
        acc = loop(3, body, acc)
        def matvec(acc, a):
            for u in range(DB // 8):
                s = cols[pl.ds(C_SC * 128 + a * DB + u * 8, 8), :]
                t = _tile(s, 2 * ND) * wm_v[a, pl.ds(u * 8, 8), pl.ds(3 * D, 2 * D)].astype(F32)
                acc = t if acc is None else acc + t
            return acc

        slab(8, 5, wm_v).wait()
        macc = matvec(None, 8)
        MARK('wlast')
        step(vl, NB - 1)
        MARK('proj31')
        o = jnp.sum(pv_tile(sl, NB - 1, acc), axis=1, keepdims=True)
        outs = [None, None]
        for j in range(G):
            w = jnp.concatenate([wo_last[j * ND + n] for n in range(ND)], axis=1)
            t = o[j * 8:(j + 1) * 8] * w
            outs[j & 1] = t if outs[j & 1] is None else outs[j & 1] + t
        x1 = xp + gl * jnp.sum(outs[0] + outs[1], axis=0, keepdims=True)
        d1 = x1 - _tile(consts[2:3, :], ND)
        mom = _moments(d1)

        MARK('w9')
        slab(9, 6, wm_hbm).wait()
        MARK('ln2')
        mom = _lane_sums(mom)
        mod = jnp.sum(matvec(macc, 9), axis=0, keepdims=True) + modb[...]
        scale_b = jnp.broadcast_to(1.0 + mod[:, D:], (8, D))
        shift_b = jnp.broadcast_to(mod[:, :D] - _tile(consts[3:4, :], ND), (8, D))
        d2 = _normalize(d1, *mom) * scale_b + shift_b
        hn = _normalize(d2, *_lane_sums(_moments(d2)))

        MARK('mlp')

        def tanh_rows(b, u, hn):
            w1c = cols[pl.ds((C_W1 + b - NZ) * 128 + u * 8, 8), :]
            b1c = cols[pl.ds((C_B1 + b - NZ) * 128 + u * 8, 8), :]
            v = hn * _tile(w1c, ND) + _tile(b1c, ND)
            return v, jnp.tanh(v * (v * v + CS))

        p2 = hn * hn
        sid = lax.broadcasted_iota(jnp.int32, (8, D), 0)
        pw_ = jnp.where(sid < 3, p2 * hn, jnp.where(sid < 6, p2, hn))
        ptop = jnp.where((sid == 1) | (sid == 4) | (sid == 7), lo_of(pw_), pw_)
        pbot = jnp.where(sid == 0, hn, jnp.where(sid < 4, 1.0, 0.0))
        pmat = jnp.concatenate([ptop, pbot], axis=0)
        r = None
        nz, nv = 0, NZ
        zs = []
        for kind in ORDER:
            if kind == 'V':
                b = nv
                nv += 1
                ts = [tanh_rows(b, u, hn)[1] for u in range(16)]
                t = jnp.concatenate(ts, axis=0)
            elif kind == 'Z':
                zs.append(jnp.dot(acol[len(zs) * 128:(len(zs) + 1) * 128, 0:16], pmat,
                                  precision=lax.Precision.DEFAULT, preferred_element_type=F32))
                continue
            else:
                b = nz
                nz += 1
                t = jnp.tanh(zs[b])
            rb = jnp.dot(lhs[:, b * 128:(b + 1) * 128], t,
                         precision=lax.Precision.DEFAULT, preferred_element_type=F32)
            r = rb if r is None else r + rb
        hl_ = hn + _tile(_tree_sum(_blocks(ts[0])) * 0.0, ND)
        for u in range(16):
            tbuf[u * 8:(u + 1) * 8, :] = tanh_rows(NF - 1, u, hl_)[1]

        def gates(js):
            na = 4 if len(js) == 1 else 2
            accs = [[None] * na for _ in js]
            for a in range(DA):
                ws = [_groups(gbuf[j, a].astype(F32)) for j in js]
                for u in range(DB // 8):
                    s = cols[pl.ds(C_SC * 128 + a * DB + u * 8, 8), :]
                    for acc, w in zip(accs, ws):
                        t = s * w[u]
                        acc[u % na] = t if acc[u % na] is None else acc[u % na] + t
            return jnp.concatenate(
                [jnp.sum(_tree_sum(acc), axis=0, keepdims=True) for acc in accs], axis=1)

        MARK('gbw')
        for j in range(3):
            gb_piece(j).wait()
        MARK('gb')
        r = r + jnp.dot(lhs[:, F - 128:], tbuf[...],
                        precision=lax.Precision.DEFAULT, preferred_element_type=F32)
        gb = [gates(range(3))]
        y = (hn[0:1] * (r[0:1] + r[1:2] + _tile(consts[0:1, :], ND))
             + (r[2:3] + r[3:4] + _tile(consts[1:2, :], ND)))
        MARK('gbw2')
        gb_piece(3).wait()
        MARK('gb2')
        gb.append(gates([3]))
        MARK('gbw3')
        gb_piece(4).wait()
        MARK('gb3')
        gb.append(gates([4]))
        o_ref[0] = (x1[0:1] + jnp.concatenate(gb, axis=1) * y).astype(o_ref.dtype)
        MARK(None)

    return kernel


@jax.jit
def pallas_adaLN_cond__sliding_block_cached__mixer_token_mlp__decode_kernel(
    A_x: jax.Array,
    A_k_cache: jax.Array,
    A_v_cache: jax.Array,
    A_wq: jax.Array,
    A_wo: jax.Array,
    B_x: jax.Array,
    B_w1: jax.Array,
    B_b1: jax.Array,
    B_w2: jax.Array,
    B_b2: jax.Array,
    c: jax.Array,
    w_mod: jax.Array,
):
    SK = A_k_cache.shape[2]
    W = min(4096, max(256, SK // 4))
    kt = jnp.swapaxes(A_k_cache, 2, 3).reshape(H * DH, SK)
    vt = jnp.swapaxes(A_v_cache, 2, 3).reshape(H * DH, SK)

    vmem = pltpu.VMEM
    dma = pltpu.SemaphoreType.DMA
    return pl.pallas_call(
        _make_kernel(SK, W),
        out_shape=jax.ShapeDtypeStruct(A_x.shape, A_x.dtype),
        in_specs=[pl.BlockSpec(memory_space=pl.ANY)] * 11,
        out_specs=pl.BlockSpec(memory_space=pltpu.VMEM),
        scratch_shapes=[
            vmem((2, W // 128, DH, 128), BF16), vmem((2, W // 128, DH, 128), BF16),
            vmem((TA, TB, 16, 128), BF16), vmem((TA, TB, 16, 128), BF16),
            vmem((DA, DB, 5 * D), BF16),
            vmem((1, 1, D), BF16), vmem((1, D), BF16),
            vmem((1, F), BF16), vmem((NF, 128), BF16), vmem((1, F), BF16),
            vmem((1,), BF16),
            vmem((H * DH, 128), F32), vmem((C_N, 128), F32), vmem((C_N * 128, 128), F32),
            vmem((8, F), F32), vmem((DH, 128), F32), vmem((W // 128, 8, 128), F32),
            vmem((4, 128), F32), vmem((1, 2 * D), F32),
            vmem((ND, DA, DB, 128), BF16), vmem((NZ * 128, 128), F32),
            vmem((G * ND, 8, 128), F32), vmem((128, D), F32),
            dma((2,)), dma((2,)), dma((64,)), dma((64,)), dma((11,)), dma((6,)),
        ],
        compiler_params=pltpu.CompilerParams(
            vmem_limit_bytes=64 * 1024 * 1024,
            disable_bounds_checks=True,
            disable_semaphore_checks=True,
        ),
    )(A_x, kt, vt, _pair_view(A_wq), _pair_view(A_wo), B_w1,
      B_b1.reshape(NF, 128), B_w2.reshape(1, F), B_b2, c, w_mod.reshape(DA, DB, 6 * D))
```

```python
import math

import jax
import jax.numpy as jnp
from jax import lax
import jax.experimental.pallas as pl
import jax.experimental.pallas.tpu as pltpu

F32 = jnp.float32
BF16 = jnp.bfloat16

D = 640
H = 32
DH = 192
F = 1536
EPS = 1e-5
G = DH // 8
ND = D // 128
NF = F // 128

LO, HI = 1, 0

_C0 = math.sqrt(2.0 / math.pi)
_C1 = 0.044715
KS = (_C0 * _C1) ** (1.0 / 3.0)
CS = _C0 / KS

ORDER = 'ZVZVVRZVRVZRVVS'
NZ = ORDER.count('Z')
NV = NF - NZ
C_W1, C_B1, C_SC, C_N = 0, NV, 2 * NV, 24

DA, DB = 10, 64
TA, TB = 15, 128


class _Group:
    def __init__(self, copies):
        self.copies = copies

    def start(self, priority):
        for c in self.copies:
            c.start(priority=priority)

    def wait(self):
        for c in self.copies:
            c.wait()


def _pair_view(w):
    r, c = w.shape
    t = w.reshape(r // 8, 8, c // 128, 128).transpose(0, 2, 1, 3)
    return t.reshape(TA, TB, 16, 128)


def _layernorm(x):
    m = jnp.mean(x, axis=-1, keepdims=True)
    xc = x - m
    v = jnp.mean(xc * xc, axis=-1, keepdims=True)
    return xc * lax.rsqrt(v + EPS)


def _moments(d):
    return _tree_sum(_blocks(d)), _tree_sum(_blocks(d * d))


def _lane_sums(xs):
    return [jnp.sum(x, axis=-1, keepdims=True) for x in xs]


def _normalize(d, s1, s2):
    s1 = s1 * (1.0 / D)
    var = jnp.maximum(s2 * (1.0 / D) - s1 * s1, 0.0)
    return (d - s1) * lax.rsqrt(var + EPS)


def _col_bcast(row128):
    return jnp.broadcast_to(row128, (128, 128)).T


def _tile(x, n):
    return jnp.concatenate([x] * n, axis=1)


def _tree_sum(parts):
    while len(parts) > 1:
        nxt = [parts[2 * i] + parts[2 * i + 1] for i in range(len(parts) // 2)]
        if len(parts) % 2:
            nxt.append(parts[-1])
        parts = nxt
    return parts[0]


def _split(a):
    hi = a.astype(BF16).astype(F32)
    return [hi, a - hi]


def _stack_rows(xs, n):
    rid = lax.broadcasted_iota(jnp.int32, (n, xs[0].shape[1]), 0)
    out = jnp.zeros(rid.shape, F32)
    for k, x in enumerate(xs):
        out = jnp.where(rid == k, x, out)
    return out


def _blocks(x):
    return [x[:, j * 128:(j + 1) * 128] for j in range(x.shape[1] // 128)]


def _groups(x):
    return [x[j * 8:(j + 1) * 8, :] for j in range(x.shape[0] // 8)]


def _make_kernel(SK, W):
    KV_HI = 16
    KV_LO = DH - KV_HI
    W0 = SK - W
    NB = W // 128

    def kernel(x_hbm, k_hbm, v_hbm, wq_hbm, wo_hbm, w1_hbm, b1_hbm, w2_hbm, b2_hbm,
               c_hbm, wm_hbm, o_ref,
               kbuf, vbuf, wq_v, wo_v, wm_v, x_v, c_v, w1_v, b1_v, w2_v, b2_v,
               qb, rows, cols, lhs, abuf, sbuf, consts, mods, acol, wo_last, tbuf,
               klo, khi, vlo, vhi, wsem, ssem):
        cp = pltpu.make_async_copy
        m8 = lambda i: pl.multiple_of(i, 8)
        m128 = lambda i: pl.multiple_of(i, 128)
        MARK = lambda name: None

        def kv_stream(src, buf, lo_sem, hi_sem, h, slot, sem_of):
            def piece(c, r0, n, sem):
                return cp(src.at[pl.ds(m8(h * DH + r0), n), pl.ds(m128(W0 + c * 128), 128)],
                          buf.at[slot, c, pl.ds(r0, n), :], sem.at[sem_of(c)])
            return (lambda c: piece(c, 0, KV_LO, lo_sem),
                    lambda c: piece(c, KV_LO, KV_HI, hi_sem))

        k_stream = lambda h, slot: kv_stream(k_hbm, kbuf, klo, khi, h, slot, lambda c: slot)
        v_stream = lambda h, slot: kv_stream(v_hbm, vbuf, vlo, vhi, h, slot,
                                             lambda c: slot * NB + c)

        def w_piece(src, dst, a0, na, b, c0, n, sem):
            idx = (pl.ds(a0, na), pl.ds(m8(b * 8), 8), pl.ds(m128(c0), n))
            return cp(src.at[idx], dst.at[idx], sem)

        def m_pieces(b, part):
            out = []
            for na, c0, n in ([(DA, c * 384, 384) for c in range(5)]
                              + [(8, (3 + c) * D, D) for c in range(2)]):
                a0, na = {'all': (0, na), 'lo': (0, na - 1), 'hi': (na - 1, 1)}[part]
                out.append(w_piece(wm_hbm, wm_v, a0, na, b, c0, n,
                                   wsem.at[8 if part == 'hi' else 0]))
            return out

        def pair_stream(src, dst, s):

            def piece(i, a0, na, r0, nr, sem):
                idx = (pl.ds(a0, na), i, pl.ds(r0, nr))
                return cp(src.at[idx], dst.at[idx], sem)
            return (lambda i: _Group([piece(i, 0, TA, 0, 8, wsem.at[s]),
                                      piece(i, 0, TA - 3, 8, 8, wsem.at[s])]),
                    lambda i: piece(i, TA - 3, 3, 8, 8, wsem.at[s + 1]))
        q_stream = pair_stream(wq_hbm, wq_v, 1)
        o_stream = pair_stream(wo_hbm, wo_v, 3)

        def t8_piece(i):
            idx = (8, pl.ds(m8((i & 1) * 32), 32), pl.ds(m128(3 * D + (i >> 1) * 128), 128))
            return cp(wm_hbm.at[idx], wm_v.at[idx], wsem.at[5])
        t8_stream = (None, t8_piece)

        def slab(a, s, src):
            idx = (a, slice(None), pl.ds(3 * D, 2 * D))
            return cp(src.at[idx], wm_v.at[idx], wsem.at[s])

        GB_ORDER = (0, 4, 2, 6, 1, 5, 3, 7)
        gb_piece = lambda b: w_piece(wm_hbm, wm_v, 0, DA, b, 5 * D, D,
                                     wsem.at[9 if b == GB_ORDER[-1] else 7])

        def issue(stream, i):
            if stream[0] is not None:
                stream[0](i).start(priority=LO)
            stream[1](i).start(priority=HI)

        def step(cur, i, nxt=None, inxt=None):
            cur[0](i).wait()
            if nxt is not None:
                issue(nxt, inxt)
            cur[1](i).wait()

        def pairs(ref, ps):
            return jnp.stack([ref[p >> 7, p & 127] for p in ps])

        def loop(n, body, init=0):
            return lax.fori_loop(0, n, body, init)

        def dma_loop(n, cur, i0, nxt, n0):
            def body(i, c):
                step(cur, i + i0, nxt, i + n0)
                return c
            loop(n, body)

        MARK('p_issue')
        for m in m_pieces(0, 'all'):
            m.start(priority=LO)
        smalls = [cp(s, d, ssem.at[n]) for n, (s, d) in enumerate(
            [(c_hbm, c_v), (x_hbm, x_v), (w1_hbm, w1_v), (b1_hbm, b1_v), (w2_hbm, w2_v),
             (b2_hbm, b2_v)])]
        for s in smalls:
            s.start(priority=HI)

        def _ma(b, c):
            for m in m_pieces(b + 1, 'all'):
                m.start(priority=LO)
            return c
        loop(3, _ma)

        MARK('p_ma')

        def _ma2(b, c):
            for m, lo, hi in zip(m_pieces(b, 'all'), m_pieces(b + 4, 'lo'), m_pieces(b + 4, 'hi')):
                m.wait()
                lo.start(priority=LO)
                hi.start(priority=HI)
            return c
        loop(4, _ma2)

        def _ma3(b, c):
            for u, (lo, hi) in enumerate(zip(m_pieces(b + 4, 'lo'), m_pieces(b + 4, 'hi'))):
                lo.wait()
                issue(q_stream, 7 * b + u)
                hi.wait()
            return c
        loop(4, _ma3)
        for s in smalls:
            s.wait()
        LQ = 28

        MARK('p_moda')
        pos = [0]

        def qsteps(n):
            dma_loop(n, q_stream, pos[0], q_stream, LQ + pos[0])
            pos[0] += n

        def qloop(n, k, fn):
            p0 = pos[0]

            def body(i, c):
                step(q_stream, p0 + k * i, q_stream, LQ + p0 + k * i)
                fn(i)
                dma_loop(k - 1, q_stream, p0 + k * i + 1, q_stream, LQ + p0 + k * i + 1)
                return c
            loop(n, body)
            pos[0] += n * k

        c32 = c_v[...].astype(F32)
        sc = (c32 * jax.nn.sigmoid(c32)).astype(BF16)
        sc16 = jnp.broadcast_to(sc, (16, D))
        w2h = w2_v[...].astype(F32) * 0.5
        w1f = w1_v[...].astype(F32)
        b1f = b1_v[...].astype(F32)
        scf = sc.astype(F32)
        for i in range(NV):
            rows[C_W1 + i:C_W1 + i + 1, :] = w1f[:, (NZ + i) * 128:(NZ + i + 1) * 128] * KS
        rows[C_B1:C_B1 + NV, :] = b1f[NZ:] * KS
        rows[C_SC + ND:C_N, :] = jnp.zeros((C_N - C_SC - ND, 128), F32)
        for i in range(ND):
            rows[C_SC + i:C_SC + i + 1, :] = scf[:, i * 128:(i + 1) * 128]

        def mod_a(i):
            c = pl.ds(m128(i * 384), 384)
            mods[:, c] = jnp.dot(sc16, wm_v[:, :, c].reshape(D, 384),
                                 preferred_element_type=F32)[0:8]
        qloop(5, 4, mod_a)

        def mod_b(i):
            c = pl.ds(m128(3 * D + i * 256), 256)
            mods[:, c] = jnp.dot(sc16[:, :512], wm_v[0:8, :, c].reshape(512, 256),
                                 preferred_element_type=F32)[0:8]
        qloop(5, 3, mod_b)

        x32 = x_v[0].astype(F32)
        h8 = (_layernorm(x32) * (1.0 + mods[:, D:2 * D]) + mods[:, :D]).astype(BF16).astype(F32)
        consts[2:3, :] = jnp.broadcast_to(jnp.mean(x32, axis=1, keepdims=True), (1, 128))
        consts[3:4, :] = jnp.broadcast_to(
            jnp.mean(mods[0:1, 3 * D:4 * D], axis=1, keepdims=True), (1, 128))
        qsteps(4)

        b1row = jnp.concatenate([b1f[i:i + 1, :] for i in range(NF)], axis=1)
        pw = w1f * w2h
        pb = b1row * w2h
        lhs[...] = _stack_rows(_split(pw) + _split(pb), 8)
        sum_w = jnp.sum(pw, axis=1, keepdims=True)
        sum_b = jnp.sum(pb, axis=1, keepdims=True) + b2_v[...].astype(F32).reshape(1, 1)
        consts[0:1, :] = jnp.broadcast_to(sum_w, (1, 128))
        consts[1:2, :] = jnp.broadcast_to(sum_b, (1, 128))
        qsteps(4)

        al = w1f[:, :NZ * 128] * KS
        be = b1row[:, :NZ * 128] * KS
        a3h, a3l = _split(al * al * al)
        a2h, a2l = _split(3.0 * al * al * be)
        a1h, a1l = _split(al * (3.0 * be * be + CS))
        a0h, a0l = _split(be * (be * be + CS))
        at = _stack_rows([a3h, a3h, a3l, a2h, a2h, a2l, a1h, a1h, a1l, a0h] + _split(a0l), 16)
        for b in range(NZ):
            acol[b * 128:(b + 1) * 128, :] = jnp.concatenate(
                [at[:, b * 128:(b + 1) * 128], jnp.zeros((112, 128), F32)], axis=0).T
        qsteps(3)

        MARK('p_prep')

        def prep(i):
            for u in range(3):
                t = 3 * i + u
                cols[pl.ds(m128(t * 128), 128), :] = _col_bcast(rows[pl.ds(t, 1), :])
        qloop(C_N // 3, 5, prep)

        MARK('p_wq')
        qsteps(TB - LQ - pos[0])
        dma_loop(LQ, q_stream, 128 - LQ, o_stream, 0)

        MARK('p_qproj')
        scale = DH ** -0.5

        def q_cols(i, q):
            for t in range(2):
                qb[pl.ds(m128(i * 256 + t * 128), 128), :] = _col_bcast(
                    q[0:1, t * 128:(t + 1) * 128])

        def qproj(i0, s0, n, nxt, n0):
            def body(i, q_prev):
                step(o_stream, s0 + i * n, nxt, n0 + i * n)
                q_cols(jnp.maximum(i + i0 - 1, 0), q_prev)
                w = pairs(wq_v, [24 * g + i + i0 for g in range(80)]).astype(F32)
                w = jnp.concatenate([w[:, 0:8].reshape(D, 128), w[:, 8:16].reshape(D, 128)],
                                    axis=1)
                q = jnp.dot(h8, w, precision=lax.Precision.DEFAULT,
                            preferred_element_type=F32) * scale
                dma_loop(n - 1, o_stream, s0 + i * n + 1, nxt, n0 + i * n + 1)
                return q
            return body
        k0, v0 = k_stream(0, 0), v_stream(0, 0)
        q = loop(20, qproj(0, 0, 5, o_stream, LQ), jnp.zeros((8, 256), F32))
        q = loop(4, qproj(20, 100, 7, k0, 0), q)
        for c in range(LQ, NB):
            issue(k0, c)
        MARK('p_k0')
        step(k0, 0, v0, 0)
        q_cols(23, q)
        abuf[...] = jnp.zeros((DH, 128), F32)
        wo_last[...] = pairs(wo_v, [60 * (H - 1) + p for p in range(60)]).astype(F32).reshape(G * ND, 8, 128)
        dma_loop(NB - 1, k0, 1, v0, 1)

        def proj(h, a, out):
            o = jnp.sum(a, axis=1, keepdims=True)
            outs = [out, None]
            for jj in range(G // 2):
                tiles = _groups(pairs(wo_v, [60 * h + jj * ND + p for p in range(ND)]).astype(F32).reshape(16 * ND, 128))
                for e in range(2):
                    j = 2 * jj + e
                    w = jnp.concatenate(tiles[e * ND:(e + 1) * ND], axis=1)
                    t = o[j * 8:(j + 1) * 8] * w
                    outs[e] = t if outs[e] is None else outs[e] + t
            return outs[0] + outs[1]

        def phase_a(h, slot, out, cur, nxt, tps, n1):
            q = qb[pl.ds(pl.multiple_of(h * DH, 64), DH), :]

            def body(i, m):
                step(cur, i, nxt, i)
                for u in range(tps):
                    c = tps * i + u
                    s = _tree_sum(_groups(kbuf[slot, c].astype(F32) * q))
                    s = jnp.broadcast_to(jnp.sum(s, axis=0, keepdims=True), (8, 128))
                    sbuf[c] = s
                    m = jnp.maximum(m, s)
                return m
            n0 = NB // tps
            m = loop(n0, body, jnp.full((8, 128), -jnp.inf, F32))
            if n1 == 1:
                step(cur, n0, nxt, n0)
            else:
                dma_loop(n1, cur, n0, nxt, n0)
            m = jnp.max(m, axis=1, keepdims=True)
            out = proj(jnp.maximum(h - 1, 0), abuf[...], out)
            dma_loop(3, cur, n0 + n1, nxt, n0 + n1)
            p = jnp.exp(sbuf[...] - m)
            sbuf[...] = p
            l = _tree_sum([p[c] for c in range(NB)])
            inv_l = 1.0 / jnp.sum(l, axis=1, keepdims=True)
            return inv_l, out

        def pv_tile(slot, c, acc):
            p = sbuf[c]
            return acc + vbuf[slot, c].astype(F32) * jnp.concatenate([p] * G, axis=0)

        def pv_done(acc, inv_l):
            return acc * jnp.concatenate([jnp.broadcast_to(inv_l, (8, 128))] * G, axis=0)

        def head(h, out):
            slot = h & 1
            nslot = 1 - slot
            knext = k_stream(h + 1, nslot)
            inv_l, out = phase_a(h, slot, out, v_stream(h, slot), knext, 2, 1)
            dma_loop(NB - 20, v_stream(h, slot), 20, knext, 20)

            def body(c, acc):
                step(knext, c, v_stream(h + 1, nslot), c)
                return pv_tile(slot, c, acc)
            abuf[...] = pv_done(loop(NB, body, jnp.zeros((DH, 128), F32)), inv_l)
            return out

        MARK('main')
        out = loop(H - 1, head, jnp.zeros((8, D), F32))

        MARK('qk31')
        hl = H - 1
        sl = hl % 2
        vl = v_stream(hl, sl)
        slab(9, 6, wm_hbm).start(priority=LO)
        for b in GB_ORDER:
            gb_piece(b).start(priority=LO)
        inv_l, out = phase_a(hl, sl, out, vl, t8_stream, 4, 3)

        MARK('pv31')

        def pv2(i0, nxt):
            def body(i, acc):
                i = i + i0
                step(vl, 14 + i, nxt, 14 + i)
                return pv_tile(sl, 2 * i + 1, pv_tile(sl, 2 * i, acc))
            return body
        acc = loop(6, pv2(0, t8_stream), jnp.zeros((DH, 128), F32))
        acc = loop(8, pv2(6, None), acc)
        ga = mods[:, 2 * D:3 * D]
        xp = x32 + ga * jnp.sum(out, axis=0, keepdims=True)
        gl = ga * inv_l

        def body(i, acc):
            step(vl, 28 + i)
            return pv_tile(sl, 28 + i, acc)
        acc = loop(3, body, acc)
        def matvec(acc, a):
            for u in range(DB // 8):
                s = cols[pl.ds(C_SC * 128 + a * DB + u * 8, 8), :]
                t = _tile(s, 2 * ND) * wm_v[a, pl.ds(u * 8, 8), pl.ds(3 * D, 2 * D)].astype(F32)
                acc = t if acc is None else acc + t
            return acc

        slab(8, 5, wm_v).wait()
        macc = matvec(None, 8)
        MARK('wlast')
        step(vl, NB - 1)
        MARK('proj31')
        o = jnp.sum(pv_tile(sl, NB - 1, acc), axis=1, keepdims=True)
        outs = [None, None]
        for j in range(G):
            w = jnp.concatenate([wo_last[j * ND + n] for n in range(ND)], axis=1)
            t = o[j * 8:(j + 1) * 8] * w
            outs[j & 1] = t if outs[j & 1] is None else outs[j & 1] + t
        x1 = xp + gl * jnp.sum(outs[0] + outs[1], axis=0, keepdims=True)
        d1 = x1 - _tile(consts[2:3, :], ND)
        mom = _moments(d1)

        MARK('w9')
        slab(9, 6, wm_hbm).wait()
        MARK('ln2')
        mom = _lane_sums(mom)
        mod = jnp.sum(matvec(macc, 9), axis=0, keepdims=True) + mods[0:1, 3 * D:]
        scale_b = jnp.broadcast_to(1.0 + mod[:, D:], (8, D))
        shift_b = jnp.broadcast_to(mod[:, :D] - _tile(consts[3:4, :], ND), (8, D))
        d2 = _normalize(d1, *mom) * scale_b + shift_b
        hn = _normalize(d2, *_lane_sums(_moments(d2)))

        MARK('mlp')

        def tanh_rows(b, u, hn):
            w1c = cols[pl.ds((C_W1 + b - NZ) * 128 + u * 8, 8), :]
            b1c = cols[pl.ds((C_B1 + b - NZ) * 128 + u * 8, 8), :]
            v = hn * _tile(w1c, ND) + _tile(b1c, ND)
            return v, jnp.tanh(v * (v * v + CS))

        p2 = hn * hn
        sid = lax.broadcasted_iota(jnp.int32, (8, D), 0)
        phi, plo = _split(jnp.where(sid < 3, p2 * hn, jnp.where(sid < 6, p2, hn)))
        ptop = jnp.where((sid == 1) | (sid == 4) | (sid == 7), plo, phi)
        pbot = jnp.where(sid == 0, hn, jnp.where(sid < 4, 1.0, 0.0))
        pmat = jnp.concatenate([ptop, pbot], axis=0)
        r = None
        nz, nv = 0, NZ
        zs = []
        late = []
        for kind in ORDER:
            if kind == 'V':
                b = nv
                nv += 1
                ts = [tanh_rows(b, u, hn)[1] for u in range(16)]
                t = jnp.concatenate(ts, axis=0)
            elif kind == 'Z':
                zs.append(jnp.dot(acol[len(zs) * 128:(len(zs) + 1) * 128, 0:16], pmat,
                                  precision=lax.Precision.DEFAULT, preferred_element_type=F32))
                continue
            else:
                b = nz
                nz += 1
                t = jnp.tanh(zs[b])
                if kind == 'S':
                    late.append(b)
                    tbuf[len(late)] = t
                    continue
            rb = jnp.dot(lhs[:, b * 128:(b + 1) * 128], t,
                         precision=lax.Precision.DEFAULT, preferred_element_type=F32)
            r = rb if r is None else r + rb
        hl_ = hn + _tile(_tree_sum(_blocks(ts[0])) * 0.0, ND)
        for u in range(16):
            tbuf[0, u * 8:(u + 1) * 8, :] = tanh_rows(NF - 1, u, hl_)[1]

        def gate(accs, bs):
            for b in bs:
                for a in range(DA):
                    s = cols[pl.ds(C_SC * 128 + a * DB + b * 8, 8), :]
                    t = _tile(s, ND) * wm_v[a, pl.ds(b * 8, 8), pl.ds(5 * D, D)].astype(F32)
                    accs[a & 1] = t if accs[a & 1] is None else accs[a & 1] + t
            return accs

        MARK('gbw')
        for b in GB_ORDER[:-1]:
            gb_piece(b).wait()
        MARK('gb')
        for k, b in enumerate([NF - 1] + late):
            r = r + jnp.dot(lhs[:, b * 128:(b + 1) * 128], tbuf[k],
                            precision=lax.Precision.DEFAULT, preferred_element_type=F32)
        gacc = gate([None, None], GB_ORDER[:-1])
        y = (hn[0:1] * (r[0:1] + r[1:2] + _tile(consts[0:1, :], ND))
             + (r[2:3] + r[3:4] + _tile(consts[1:2, :], ND)))
        MARK('gbw3')
        gb_piece(GB_ORDER[-1]).wait()
        MARK('gb3')
        gacc = gate(gacc, GB_ORDER[-1:])
        gb = jnp.sum(gacc[0] + gacc[1], axis=0, keepdims=True)
        o_ref[0] = (x1[0:1] + gb * y).astype(o_ref.dtype)
        MARK(None)

    return kernel


@jax.jit
def pallas_adaLN_cond__sliding_block_cached__mixer_token_mlp__decode_kernel(
    A_x: jax.Array,
    A_k_cache: jax.Array,
    A_v_cache: jax.Array,
    A_wq: jax.Array,
    A_wo: jax.Array,
    B_x: jax.Array,
    B_w1: jax.Array,
    B_b1: jax.Array,
    B_w2: jax.Array,
    B_b2: jax.Array,
    c: jax.Array,
    w_mod: jax.Array,
):
    SK = A_k_cache.shape[2]
    W = min(4096, max(256, SK // 4))
    kt = jnp.swapaxes(A_k_cache, 2, 3).reshape(H * DH, SK)
    vt = jnp.swapaxes(A_v_cache, 2, 3).reshape(H * DH, SK)

    vmem = pltpu.VMEM
    dma = pltpu.SemaphoreType.DMA
    return pl.pallas_call(
        _make_kernel(SK, W),
        out_shape=jax.ShapeDtypeStruct(A_x.shape, A_x.dtype),
        in_specs=[pl.BlockSpec(memory_space=pl.ANY)] * 11,
        out_specs=pl.BlockSpec(memory_space=pltpu.VMEM),
        scratch_shapes=[
            vmem((2, W // 128, DH, 128), BF16), vmem((2, W // 128, DH, 128), BF16),
            vmem((TA, TB, 16, 128), BF16), vmem((TA, TB, 16, 128), BF16),
            vmem((DA, DB, 6 * D), BF16),
            vmem((1, 1, D), BF16), vmem((1, D), BF16),
            vmem((1, F), BF16), vmem((NF, 128), BF16), vmem((1, F), BF16),
            vmem((1,), BF16),
            vmem((H * DH, 128), F32), vmem((C_N, 128), F32), vmem((C_N * 128, 128), F32),
            vmem((8, F), F32), vmem((DH, 128), F32), vmem((W // 128, 8, 128), F32),
            vmem((4, 128), F32), vmem((8, 5 * D), F32),
            vmem((NZ * 128, 128), F32),
            vmem((G * ND, 8, 128), F32), vmem((1 + ORDER.count('S'), 128, D), F32),
            dma((2,)), dma((2,)), dma((64,)), dma((64,)), dma((10,)), dma((6,)),
        ],
        compiler_params=pltpu.CompilerParams(
            vmem_limit_bytes=64 * 1024 * 1024,
            disable_bounds_checks=True,
            disable_semaphore_checks=True,
        ),
    )(A_x, kt, vt, _pair_view(A_wq), _pair_view(A_wo), B_w1,
      B_b1.reshape(NF, 128), B_w2.reshape(1, F), B_b2, c, w_mod.reshape(DA, DB, 6 * D))
```

```python
import math

import jax
import jax.numpy as jnp
from jax import lax
import jax.experimental.pallas as pl
import jax.experimental.pallas.tpu as pltpu

F32 = jnp.float32
BF16 = jnp.bfloat16

D = 640
H = 32
DH = 192
F = 1536
EPS = 1e-5
G = DH // 8
ND = D // 128
NF = F // 128

LO, HI = 1, 0

_C0 = math.sqrt(2.0 / math.pi)
_C1 = 0.044715
KS = (_C0 * _C1) ** (1.0 / 3.0)
CS = _C0 / KS

ORDER = 'ZVZVVRZVRVZRVVS'
NZ = ORDER.count('Z')
NV = NF - NZ
C_W1, C_B1, C_SC, C_N = 0, NV, 2 * NV, 24

DA, DB = 10, 64
TA, TB = 15, 128


class _Group:
    def __init__(self, copies):
        self.copies = copies

    def start(self, priority):
        for c in self.copies:
            c.start(priority=priority)

    def wait(self):
        for c in self.copies:
            c.wait()


def _pair_view(w):
    r, c = w.shape
    t = w.reshape(r // 8, 8, c // 128, 128).transpose(0, 2, 1, 3)
    return t.reshape(TA, TB, 16, 128)


def _layernorm(x):
    m = jnp.mean(x, axis=-1, keepdims=True)
    xc = x - m
    v = jnp.mean(xc * xc, axis=-1, keepdims=True)
    return xc * lax.rsqrt(v + EPS)


def _moments(d):
    return _tree_sum(_blocks(d)), _tree_sum(_blocks(d * d))


def _lane_sums(xs):
    return [jnp.sum(x, axis=-1, keepdims=True) for x in xs]


def _normalize(d, s1, s2):
    s1 = s1 * (1.0 / D)
    var = jnp.maximum(s2 * (1.0 / D) - s1 * s1, 0.0)
    return (d - s1) * lax.rsqrt(var + EPS)


def _col_bcast(row128):
    return jnp.broadcast_to(row128, (128, 128)).T


def _tile(x, n):
    return jnp.concatenate([x] * n, axis=1)


def _tree_sum(parts):
    while len(parts) > 1:
        nxt = [parts[2 * i] + parts[2 * i + 1] for i in range(len(parts) // 2)]
        if len(parts) % 2:
            nxt.append(parts[-1])
        parts = nxt
    return parts[0]


def _split(a):
    hi = a.astype(BF16).astype(F32)
    return [hi, a - hi]


def _stack_rows(xs, n):
    rid = lax.broadcasted_iota(jnp.int32, (n, xs[0].shape[1]), 0)
    out = jnp.zeros(rid.shape, F32)
    for k, x in enumerate(xs):
        out = jnp.where(rid == k, x, out)
    return out


def _blocks(x):
    return [x[:, j * 128:(j + 1) * 128] for j in range(x.shape[1] // 128)]


def _groups(x):
    return [x[j * 8:(j + 1) * 8, :] for j in range(x.shape[0] // 8)]


def _make_kernel(SK, W):
    LH = 12
    KV_HI = 32
    KV_LO = DH - KV_HI
    W0 = SK - W
    NB = W // 128

    def kernel(x_hbm, k_hbm, v_hbm, wq_hbm, wo_hbm, w1_hbm, b1_hbm, w2_hbm, b2_hbm,
               c_hbm, wm_hbm, o_ref,
               kbuf, vbuf, wq_v, wo_v, wm_v, x_v, c_v, w1_v, b1_v, w2_v, b2_v,
               qb, rows, cols, lhs, abuf, sbuf, consts, mods, acol, wo_last, tbuf,
               klo, khi, vlo, vhi, wsem, ssem):
        cp = pltpu.make_async_copy
        m8 = lambda i: pl.multiple_of(i, 8)
        m128 = lambda i: pl.multiple_of(i, 128)
        MARK = lambda name: None

        def kv_stream(src, buf, lo_sem, hi_sem, h, slot, sem_of):
            def piece(c, r0, n, sem):
                return cp(src.at[pl.ds(m8(h * DH + r0), n), pl.ds(m128(W0 + c * 128), 128)],
                          buf.at[slot, c, pl.ds(r0, n), :], sem.at[sem_of(c)])
            return (lambda c: piece(c, 0, KV_LO, lo_sem),
                    lambda c: piece(c, KV_LO, KV_HI, hi_sem))

        k_stream = lambda h, slot: kv_stream(k_hbm, kbuf, klo, khi, h, slot, lambda c: slot)
        v_stream = lambda h, slot: kv_stream(v_hbm, vbuf, vlo, vhi, h, slot,
                                             lambda c: slot * NB + c)

        def w_piece(src, dst, a0, na, b, c0, n, sem):
            idx = (pl.ds(a0, na), pl.ds(m8(b * 8), 8), pl.ds(m128(c0), n))
            return cp(src.at[idx], dst.at[idx], sem)

        def m_piece(b, u, part):
            na, c0, n = (DA, u * 384, 384) if u < 5 else (DA - 1, (u - 2) * D, D)
            a0, na = {'all': (0, na), 'lo': (0, na - 1), 'hi': (na - 1, 1)}[part]
            return w_piece(wm_hbm, wm_v, a0, na, b, c0, n, wsem.at[5 if part == 'hi' else 0])

        def pair_stream(src, dst, s):

            def piece(i, a0, na, r0, nr, sem):
                idx = (pl.ds(a0, na), i, pl.ds(r0, nr))
                return cp(src.at[idx], dst.at[idx], sem)
            return (lambda i: _Group([piece(i, 0, TA, 0, 8, wsem.at[s]),
                                      piece(i, 0, TA - 3, 8, 8, wsem.at[s])]),
                    lambda i: piece(i, TA - 3, 3, 8, 8, wsem.at[s + 1]))
        q_stream = pair_stream(wq_hbm, wq_v, 1)
        o_stream = pair_stream(wo_hbm, wo_v, 3)

        idx9 = (DA - 1, slice(None), pl.ds(3 * D, 2 * D))
        slab9 = cp(wm_hbm.at[idx9], wm_v.at[idx9], wsem.at[6])

        GB_ORDER = (0, 4, 2, 6, 1, 5, 3, 7)
        gb_piece = lambda b: w_piece(wm_hbm, wm_v, 0, DA, b, 5 * D, D,
                                     wsem.at[8 if b == GB_ORDER[-1] else 7])

        class Phase:
            def __init__(self, cur, n, ll, nxt):
                self.cur, self.n, self.ll, self.nxt = cur, n, ll, nxt

            def stepper(self, a, b):
                starts = []
                for k, ahead, prio in ((0, self.ll, LO), (1, LH, HI)):
                    edge = self.n - ahead
                    assert b <= edge or a >= edge, (a, b, edge)
                    if b <= edge:
                        starts.append((self.cur[k], ahead, prio))
                    elif self.nxt is not None:
                        starts.append((self.nxt[k], -edge, prio))

                def step(i):
                    self.cur[0](i).wait()
                    for piece, off, prio in starts:
                        piece(i + off).start(priority=prio)
                    self.cur[1](i).wait()
                return step

            def run(self, a, b, fn=None, init=0):
                cuts = sorted({a, b} | {e for e in (self.n - self.ll, self.n - LH) if a < e < b})
                for lo, hi in zip(cuts[:-1], cuts[1:]):
                    step = self.stepper(lo, hi)

                    def body(i, c):
                        step(i)
                        return c if fn is None else fn(i, c)
                    init = body(lo, init) if hi - lo == 1 else lax.fori_loop(lo, hi, body, init)
                return init

            def every(self, a, n, k, fn, init=0):
                step = self.stepper(a, a + n * k)

                def body(j, c):
                    step(a + k * j)
                    c = fn(j, c)

                    def rest(u, z):
                        step(a + k * j + u)
                        return z
                    lax.fori_loop(1, k, rest, 0)
                    return c
                return lax.fori_loop(0, n, body, init)

        def pairs(ref, ps):
            return jnp.stack([ref[p >> 7, p & 127] for p in ps])

        def loop(n, body, init=0):
            return lax.fori_loop(0, n, body, init)

        MARK('p_issue')
        for u in range(7):
            m_piece(0, u, 'all').start(priority=LO)
        smalls = [cp(s, d, ssem.at[n]) for n, (s, d) in enumerate(
            [(c_hbm, c_v), (x_hbm, x_v), (w1_hbm, w1_v), (b1_hbm, b1_v), (w2_hbm, w2_v),
             (b2_hbm, b2_v)])]
        for s in smalls:
            s.start(priority=HI)

        for b in range(1, 4):
            for u in range(7):
                m_piece(b, u, 'all' if b == 1 else 'lo').start(priority=LO)

        MARK('p_ma')

        def m_sets(b0, lo_next, hi_next):
            def body(b, c):
                for u in range(7):
                    m_piece(b, u, 'all' if b0 == 0 else 'lo').wait()
                    lo_next(b, u).start(priority=LO)
                    hi = hi_next(b, u)
                    if hi is not None:
                        hi.start(priority=HI)
                    if b0:
                        m_piece(b, u, 'hi').wait()
                return c
            lax.fori_loop(b0, b0 + 2, body, 0)
        m_lo = lambda b, u: m_piece(b + 4, u, 'lo')
        m_hi = lambda b, u: m_piece(b + 2, u, 'hi')
        q_lo = lambda b, u: q_stream[0](7 * (b - 4) + u)
        m_sets(0, m_lo, m_hi)
        m_sets(2, m_lo, m_hi)
        m_sets(4, q_lo, m_hi)
        m_sets(6, q_lo, lambda b, u: q_stream[1](6 * (b - 6) + u) if u < 6 else None)
        for s in smalls:
            s.wait()

        MARK('p_moda')
        k0, v0 = k_stream(0, 0), v_stream(0, 0)
        LW = 28
        ph_q = Phase(q_stream, TB, LW, o_stream)
        ph_o = Phase(o_stream, TB, LW, k0)
        pos = [0]

        def qsteps(n):
            ph_q.run(pos[0], pos[0] + n)
            pos[0] += n

        def qloop(n, k, fn):
            def body(j, c):
                fn(j)
                return c
            ph_q.every(pos[0], n, k, body)
            pos[0] += n * k

        c32 = c_v[...].astype(F32)
        sc = (c32 * jax.nn.sigmoid(c32)).astype(BF16)
        sc16 = jnp.broadcast_to(sc, (16, D))
        w2h = w2_v[...].astype(F32) * 0.5
        w1f = w1_v[...].astype(F32)
        b1f = b1_v[...].astype(F32)
        scf = sc.astype(F32)
        for i in range(NV):
            rows[C_W1 + i:C_W1 + i + 1, :] = w1f[:, (NZ + i) * 128:(NZ + i + 1) * 128] * KS
        rows[C_B1:C_B1 + NV, :] = b1f[NZ:] * KS
        rows[C_SC + ND:C_N, :] = jnp.zeros((C_N - C_SC - ND, 128), F32)
        for i in range(ND):
            rows[C_SC + i:C_SC + i + 1, :] = scf[:, i * 128:(i + 1) * 128]

        def mod_a(i):
            c = pl.ds(m128(i * 384), 384)
            mods[:, c] = jnp.dot(sc16, wm_v[:, :, c].reshape(D, 384),
                                 preferred_element_type=F32)[0:8]
        qloop(5, 4, mod_a)

        def mod_b(i):
            c = pl.ds(m128(3 * D + i * 256), 256)
            mods[:, c] = jnp.dot(sc16[:, :D - DB], wm_v[0:DA - 1, :, c].reshape(D - DB, 256),
                                 preferred_element_type=F32)[0:8]
        qloop(5, 3, mod_b)

        x32 = x_v[0].astype(F32)
        h8 = (_layernorm(x32) * (1.0 + mods[:, D:2 * D]) + mods[:, :D]).astype(BF16).astype(F32)
        consts[2:3, :] = jnp.broadcast_to(jnp.mean(x32, axis=1, keepdims=True), (1, 128))
        consts[3:4, :] = jnp.broadcast_to(
            jnp.mean(mods[0:1, 3 * D:4 * D], axis=1, keepdims=True), (1, 128))
        qsteps(4)

        b1row = jnp.concatenate([b1f[i:i + 1, :] for i in range(NF)], axis=1)
        pw = w1f * w2h
        pb = b1row * w2h
        lhs[...] = _stack_rows(_split(pw) + _split(pb), 8)
        sum_w = jnp.sum(pw, axis=1, keepdims=True)
        sum_b = jnp.sum(pb, axis=1, keepdims=True) + b2_v[...].astype(F32).reshape(1, 1)
        consts[0:1, :] = jnp.broadcast_to(sum_w, (1, 128))
        consts[1:2, :] = jnp.broadcast_to(sum_b, (1, 128))
        qsteps(4)

        al = w1f[:, :NZ * 128] * KS
        be = b1row[:, :NZ * 128] * KS
        a3h, a3l = _split(al * al * al)
        a2h, a2l = _split(3.0 * al * al * be)
        a1h, a1l = _split(al * (3.0 * be * be + CS))
        a0h, a0l = _split(be * (be * be + CS))
        at = _stack_rows([a3h, a3h, a3l, a2h, a2h, a2l, a1h, a1h, a1l, a0h] + _split(a0l), 16)
        for b in range(NZ):
            acol[b * 128:(b + 1) * 128, :] = jnp.concatenate(
                [at[:, b * 128:(b + 1) * 128], jnp.zeros((112, 128), F32)], axis=0).T
        qsteps(3)

        MARK('p_prep')

        def prep(i):
            for u in range(3):
                t = 3 * i + u
                cols[pl.ds(m128(t * 128), 128), :] = _col_bcast(rows[pl.ds(t, 1), :])
        qloop(C_N // 3, 5, prep)

        MARK('p_wq')
        qsteps(TB - pos[0])

        MARK('p_qproj')
        scale = DH ** -0.5

        def q_cols(i, q):
            for t in range(2):
                qb[pl.ds(m128(i * 256 + t * 128), 128), :] = _col_bcast(
                    q[0:1, t * 128:(t + 1) * 128])

        def qproj(i0):
            def fn(i, q_prev):
                q_cols(jnp.maximum(i + i0 - 1, 0), q_prev)
                w = pairs(wq_v, [24 * g + i + i0 for g in range(D // 8)]).astype(F32)
                w = jnp.concatenate([w[:, 0:8].reshape(D, 128), w[:, 8:16].reshape(D, 128)],
                                    axis=1)
                return jnp.dot(h8, w, precision=lax.Precision.DEFAULT,
                               preferred_element_type=F32) * scale
            return fn
        q = ph_o.every(0, 20, 5, qproj(0), jnp.zeros((8, 256), F32))
        q = ph_o.every(100, 4, 4, qproj(20), q)
        ph_o.run(116, 117)
        q_cols(23, q)
        ph_o.run(117, TB)
        for c in range(LW, NB):
            k0[0](c).start(priority=LO)
        MARK('p_k0')
        ph = Phase(k0, NB, NB, v0)
        ph.run(0, 1)
        abuf[...] = jnp.zeros((DH, 128), F32)
        wo_last[...] = pairs(wo_v, [60 * (H - 1) + p for p in range(60)]).astype(F32).reshape(
            G * ND, 8, 128)
        ph.run(1, NB)

        def proj(h, a, out):
            o = jnp.sum(a, axis=1, keepdims=True)
            outs = [out, None]
            for jj in range(G // 2):
                tiles = _groups(pairs(wo_v, [60 * h + jj * ND + p for p in range(ND)]).astype(F32).reshape(16 * ND, 128))
                for e in range(2):
                    j = 2 * jj + e
                    w = jnp.concatenate(tiles[e * ND:(e + 1) * ND], axis=1)
                    t = o[j * 8:(j + 1) * 8] * w
                    outs[e] = t if outs[e] is None else outs[e] + t
            return outs[0] + outs[1]

        def phase_a(h, slot, out, ph, tps, n1):
            q = qb[pl.ds(pl.multiple_of(h * DH, 64), DH), :]

            def body(i, m):
                for u in range(tps):
                    c = tps * i + u
                    s = _tree_sum(_groups(kbuf[slot, c].astype(F32) * q))
                    s = jnp.broadcast_to(jnp.sum(s, axis=0, keepdims=True), (8, 128))
                    sbuf[c] = s
                    m = jnp.maximum(m, s)
                return m
            n0 = NB // tps
            m = ph.run(0, n0, body, jnp.full((8, 128), -jnp.inf, F32))
            ph.run(n0, n0 + n1)
            m = jnp.max(m, axis=1, keepdims=True)
            out = proj(jnp.maximum(h - 1, 0), abuf[...], out)
            ph.run(n0 + n1, n0 + n1 + 3)
            p = jnp.exp(sbuf[...] - m)
            sbuf[...] = p
            l = _tree_sum([p[c] for c in range(NB)])
            inv_l = 1.0 / jnp.sum(l, axis=1, keepdims=True)
            return inv_l, out

        def pv_tile(slot, c, acc):
            p = sbuf[c]
            return acc + vbuf[slot, c].astype(F32) * jnp.concatenate([p] * G, axis=0)

        def pv_done(acc, inv_l):
            return acc * jnp.concatenate([jnp.broadcast_to(inv_l, (8, 128))] * G, axis=0)

        def head(h, out):
            slot = h & 1
            nslot = 1 - slot
            knext = k_stream(h + 1, nslot)
            ph = Phase(v_stream(h, slot), NB, NB, knext)
            inv_l, out = phase_a(h, slot, out, ph, 2, 1)
            ph.run(20, NB)
            ph = Phase(knext, NB, NB, v_stream(h + 1, nslot))
            acc = ph.run(0, NB, lambda c, acc: pv_tile(slot, c, acc), jnp.zeros((DH, 128), F32))
            abuf[...] = pv_done(acc, inv_l)
            return out

        MARK('main')
        out = loop(H - 1, head, jnp.zeros((8, D), F32))

        MARK('qk31')
        hl = H - 1
        sl = hl % 2
        slab9.start(priority=LO)
        for b in GB_ORDER:
            gb_piece(b).start(priority=LO)
        ph = Phase(v_stream(hl, sl), NB, NB, None)
        inv_l, out = phase_a(hl, sl, out, ph, 4, 3)

        MARK('pv31')
        acc = ph.run(14, 28, lambda i, acc: pv_tile(sl, 2 * i - 27, pv_tile(sl, 2 * i - 28, acc)),
                     jnp.zeros((DH, 128), F32))
        ga = mods[:, 2 * D:3 * D]
        xp = x32 + ga * jnp.sum(out, axis=0, keepdims=True)
        gl = ga * inv_l
        acc = ph.run(28, NB - 1, lambda c, acc: pv_tile(sl, c, acc), acc)
        MARK('wlast')
        ph.run(NB - 1, NB)
        MARK('proj31')
        o = jnp.sum(pv_tile(sl, NB - 1, acc), axis=1, keepdims=True)
        outs = [None, None]
        for j in range(G):
            w = jnp.concatenate([wo_last[j * ND + n] for n in range(ND)], axis=1)
            t = o[j * 8:(j + 1) * 8] * w
            outs[j & 1] = t if outs[j & 1] is None else outs[j & 1] + t
        x1 = xp + gl * jnp.sum(outs[0] + outs[1], axis=0, keepdims=True)
        d1 = x1 - _tile(consts[2:3, :], ND)
        mom = _moments(d1)

        MARK('w9')
        slab9.wait()
        MARK('ln2')
        mom = _lane_sums(mom)
        macc = None
        for u in range(DB // 8):
            s = cols[pl.ds(C_SC * 128 + D - DB + u * 8, 8), :]
            t = _tile(s, 2 * ND) * wm_v[DA - 1, pl.ds(u * 8, 8), pl.ds(3 * D, 2 * D)].astype(F32)
            macc = t if macc is None else macc + t
        mod = jnp.sum(macc, axis=0, keepdims=True) + mods[0:1, 3 * D:]
        scale_b = jnp.broadcast_to(1.0 + mod[:, D:], (8, D))
        shift_b = jnp.broadcast_to(mod[:, :D] - _tile(consts[3:4, :], ND), (8, D))
        d2 = _normalize(d1, *mom) * scale_b + shift_b
        hn = _normalize(d2, *_lane_sums(_moments(d2)))

        MARK('mlp')

        def tanh_rows(b, u, hn):
            w1c = cols[pl.ds((C_W1 + b - NZ) * 128 + u * 8, 8), :]
            b1c = cols[pl.ds((C_B1 + b - NZ) * 128 + u * 8, 8), :]
            v = hn * _tile(w1c, ND) + _tile(b1c, ND)
            return v, jnp.tanh(v * (v * v + CS))

        p2 = hn * hn
        sid = lax.broadcasted_iota(jnp.int32, (8, D), 0)
        phi, plo = _split(jnp.where(sid < 3, p2 * hn, jnp.where(sid < 6, p2, hn)))
        ptop = jnp.where((sid == 1) | (sid == 4) | (sid == 7), plo, phi)
        pbot = jnp.where(sid == 0, hn, jnp.where(sid < 4, 1.0, 0.0))
        pmat = jnp.concatenate([ptop, pbot], axis=0)
        r = None
        nz, nv = 0, NZ
        zs = []
        late = []
        for kind in ORDER:
            if kind == 'V':
                b = nv
                nv += 1
                ts = [tanh_rows(b, u, hn)[1] for u in range(16)]
                t = jnp.concatenate(ts, axis=0)
            elif kind == 'Z':
                zs.append(jnp.dot(acol[len(zs) * 128:(len(zs) + 1) * 128, 0:16], pmat,
                                  precision=lax.Precision.DEFAULT, preferred_element_type=F32))
                continue
            else:
                b = nz
                nz += 1
                t = jnp.tanh(zs[b])
                if kind == 'S':
                    late.append(b)
                    tbuf[len(late)] = t
                    continue
            rb = jnp.dot(lhs[:, b * 128:(b + 1) * 128], t,
                         precision=lax.Precision.DEFAULT, preferred_element_type=F32)
            r = rb if r is None else r + rb
        hl_ = hn + _tile(_tree_sum(_blocks(ts[0])) * 0.0, ND)
        for u in range(16):
            tbuf[0, u * 8:(u + 1) * 8, :] = tanh_rows(NF - 1, u, hl_)[1]

        def gate(accs, bs):
            for b in bs:
                for a in range(DA):
                    s = cols[pl.ds(C_SC * 128 + a * DB + b * 8, 8), :]
                    t = _tile(s, ND) * wm_v[a, pl.ds(b * 8, 8), pl.ds(5 * D, D)].astype(F32)
                    accs[a & 1] = t if accs[a & 1] is None else accs[a & 1] + t
            return accs

        MARK('gbw')
        for b in GB_ORDER[:-1]:
            gb_piece(b).wait()
        MARK('gb')
        for k, b in enumerate([NF - 1] + late):
            r = r + jnp.dot(lhs[:, b * 128:(b + 1) * 128], tbuf[k],
                            precision=lax.Precision.DEFAULT, preferred_element_type=F32)
        gacc = gate([None, None], GB_ORDER[:-1])
        y = (hn[0:1] * (r[0:1] + r[1:2] + _tile(consts[0:1, :], ND))
             + (r[2:3] + r[3:4] + _tile(consts[1:2, :], ND)))
        MARK('gbw3')
        gb_piece(GB_ORDER[-1]).wait()
        MARK('gb3')
        gacc = gate(gacc, GB_ORDER[-1:])
        gb = jnp.sum(gacc[0] + gacc[1], axis=0, keepdims=True)
        o_ref[0] = (x1[0:1] + gb * y).astype(o_ref.dtype)
        MARK(None)

    return kernel


@jax.jit
def pallas_adaLN_cond__sliding_block_cached__mixer_token_mlp__decode_kernel(
    A_x: jax.Array,
    A_k_cache: jax.Array,
    A_v_cache: jax.Array,
    A_wq: jax.Array,
    A_wo: jax.Array,
    B_x: jax.Array,
    B_w1: jax.Array,
    B_b1: jax.Array,
    B_w2: jax.Array,
    B_b2: jax.Array,
    c: jax.Array,
    w_mod: jax.Array,
):
    SK = A_k_cache.shape[2]
    W = min(4096, max(256, SK // 4))
    kt = jnp.swapaxes(A_k_cache, 2, 3).reshape(H * DH, SK)
    vt = jnp.swapaxes(A_v_cache, 2, 3).reshape(H * DH, SK)

    vmem = pltpu.VMEM
    dma = pltpu.SemaphoreType.DMA
    return pl.pallas_call(
        _make_kernel(SK, W),
        out_shape=jax.ShapeDtypeStruct(A_x.shape, A_x.dtype),
        in_specs=[pl.BlockSpec(memory_space=pl.ANY)] * 11,
        out_specs=pl.BlockSpec(memory_space=pltpu.VMEM),
        scratch_shapes=[
            vmem((2, W // 128, DH, 128), BF16), vmem((2, W // 128, DH, 128), BF16),
            vmem((TA, TB, 16, 128), BF16), vmem((TA, TB, 16, 128), BF16),
            vmem((DA, DB, 6 * D), BF16),
            vmem((1, 1, D), BF16), vmem((1, D), BF16),
            vmem((1, F), BF16), vmem((NF, 128), BF16), vmem((1, F), BF16),
            vmem((1,), BF16),
            vmem((H * DH, 128), F32), vmem((C_N, 128), F32), vmem((C_N * 128, 128), F32),
            vmem((8, F), F32), vmem((DH, 128), F32), vmem((W // 128, 8, 128), F32),
            vmem((4, 128), F32), vmem((8, 5 * D), F32),
            vmem((NZ * 128, 128), F32),
            vmem((G * ND, 8, 128), F32), vmem((1 + ORDER.count('S'), 128, D), F32),
            dma((2,)), dma((2,)), dma((64,)), dma((64,)), dma((9,)), dma((6,)),
        ],
        compiler_params=pltpu.CompilerParams(
            vmem_limit_bytes=64 * 1024 * 1024,
            disable_bounds_checks=True,
            disable_semaphore_checks=True,
        ),
    )(A_x, kt, vt, _pair_view(A_wq), _pair_view(A_wo), B_w1,
      B_b1.reshape(NF, 128), B_w2.reshape(1, F), B_b2, c, w_mod.reshape(DA, DB, 6 * D))
```

```python
import math

import jax
import jax.numpy as jnp
from jax import lax
import jax.experimental.pallas as pl
import jax.experimental.pallas.tpu as pltpu

F32 = jnp.float32
BF16 = jnp.bfloat16

D = 640
H = 32
DH = 192
F = 1536
EPS = 1e-5
G = DH // 8
ND = D // 128
NF = F // 128

LO, HI = 1, 0

_C0 = math.sqrt(2.0 / math.pi)
_C1 = 0.044715
KS = (_C0 * _C1) ** (1.0 / 3.0)
CS = _C0 / KS

ORDER = 'ZVZVVRZVRVZRVVS'
NZ = ORDER.count('Z')
NV = NF - NZ
C_W1, C_B1, C_SC, C_N = 0, NV, 2 * NV, 24

DA, DB = 10, 64
TA, TB = 15, 128


class _Group:
    def __init__(self, copies):
        self.copies = copies

    def start(self, priority):
        for c in self.copies:
            c.start(priority=priority)

    def wait(self):
        for c in self.copies:
            c.wait()


def _pair_view(w):
    r, c = w.shape
    t = w.reshape(r // 8, 8, c // 128, 128).transpose(0, 2, 1, 3)
    return t.reshape(TA, TB, 16, 128)


def _layernorm(x):
    m = jnp.mean(x, axis=-1, keepdims=True)
    xc = x - m
    v = jnp.mean(xc * xc, axis=-1, keepdims=True)
    return xc * lax.rsqrt(v + EPS)


def _moments(d):
    return _tree_sum(_blocks(d)), _tree_sum(_blocks(d * d))


def _lane_sums(xs):
    return [jnp.sum(x, axis=-1, keepdims=True) for x in xs]


def _normalize(d, s1, s2):
    s1 = s1 * (1.0 / D)
    var = jnp.maximum(s2 * (1.0 / D) - s1 * s1, 0.0)
    return (d - s1) * lax.rsqrt(var + EPS)


def _col_bcast(row128):
    return jnp.broadcast_to(row128, (128, 128)).T


def _tile(x, n):
    return jnp.concatenate([x] * n, axis=1)


def _tree_sum(parts):
    while len(parts) > 1:
        nxt = [parts[2 * i] + parts[2 * i + 1] for i in range(len(parts) // 2)]
        if len(parts) % 2:
            nxt.append(parts[-1])
        parts = nxt
    return parts[0]


def _split(a):
    hi = a.astype(BF16).astype(F32)
    return [hi, a - hi]


def _stack_rows(xs, n):
    rid = lax.broadcasted_iota(jnp.int32, (n, xs[0].shape[1]), 0)
    out = jnp.zeros(rid.shape, F32)
    for k, x in enumerate(xs):
        out = jnp.where(rid == k, x, out)
    return out


def _blocks(x):
    return [x[:, j * 128:(j + 1) * 128] for j in range(x.shape[1] // 128)]


def _groups(x):
    return [x[j * 8:(j + 1) * 8, :] for j in range(x.shape[0] // 8)]


def _make_kernel(SK, W):
    LH = 14
    KV_HI = 16
    KV_LO = DH - KV_HI
    W0 = SK - W
    NB = W // 128

    def kernel(x_hbm, k_hbm, v_hbm, wq_hbm, wo_hbm, w1_hbm, b1_hbm, w2_hbm, b2_hbm,
               c_hbm, wm_hbm, o_ref,
               kbuf, vbuf, wq_v, wo_v, wm_v, x_v, c_v, w1_v, b1_v, w2_v, b2_v,
               qb, rows, cols, lhs, abuf, sbuf, consts, mods, acol, wo_last, tbuf,
               klo, khi, vlo, vhi, wsem, ssem):
        cp = pltpu.make_async_copy
        m8 = lambda i: pl.multiple_of(i, 8)
        m128 = lambda i: pl.multiple_of(i, 128)
        MARK = lambda name: None

        def kv_stream(src, buf, lo_sem, hi_sem, h, slot, sem_of):
            def piece(c, r0, n, sem):
                return cp(src.at[pl.ds(m8(h * DH + r0), n), pl.ds(m128(W0 + c * 128), 128)],
                          buf.at[slot, c, pl.ds(r0, n), :], sem.at[sem_of(c)])
            return (lambda c: piece(c, 0, KV_LO, lo_sem),
                    lambda c: piece(c, KV_LO, KV_HI, hi_sem))

        k_stream = lambda h, slot: kv_stream(k_hbm, kbuf, klo, khi, h, slot, lambda c: slot)
        v_stream = lambda h, slot: kv_stream(v_hbm, vbuf, vlo, vhi, h, slot,
                                             lambda c: slot * NB + c)

        def w_piece(src, dst, a0, na, b, c0, n, sem):
            idx = (pl.ds(a0, na), pl.ds(m8(b * 8), 8), pl.ds(m128(c0), n))
            return cp(src.at[idx], dst.at[idx], sem)

        def m_piece(b, u, part):
            na, c0, n = (DA, u * 384, 384) if u < 5 else (DA - 1, (u - 2) * D, D)
            a0, na = {'all': (0, na), 'lo': (0, na - 1), 'hi': (na - 1, 1)}[part]
            return w_piece(wm_hbm, wm_v, a0, na, b, c0, n, wsem.at[5 if part == 'hi' else 0])

        def pair_stream(src, dst, s):

            def piece(i, a0, na, r0, nr, sem):
                idx = (pl.ds(a0, na), i, pl.ds(r0, nr))
                return cp(src.at[idx], dst.at[idx], sem)
            return (lambda i: _Group([piece(i, 0, TA, 0, 8, wsem.at[s]),
                                      piece(i, 0, TA - 3, 8, 8, wsem.at[s])]),
                    lambda i: piece(i, TA - 3, 3, 8, 8, wsem.at[s + 1]))
        q_stream = pair_stream(wq_hbm, wq_v, 1)
        o_stream = pair_stream(wo_hbm, wo_v, 3)

        idx9 = (DA - 1, slice(None), pl.ds(3 * D, 2 * D))
        slab9 = cp(wm_hbm.at[idx9], wm_v.at[idx9], wsem.at[6])

        GB_ORDER = (0, 4, 2, 6, 1, 5, 3, 7)
        gb_piece = lambda b: w_piece(wm_hbm, wm_v, 0, DA, b, 5 * D, D,
                                     wsem.at[8 if b == GB_ORDER[-1] else 7])

        class Phase:
            def __init__(self, cur, n, ll, nxt):
                self.cur, self.n, self.nxt = cur, n, nxt
                self.ahead = (ll, LH)
                self.edges = {n - ll, n - LH}

            def stepper(self, a, b):
                starts = []
                assert not any(a < e < b for e in self.edges), (a, b)
                for k, prio in ((0, LO), (1, HI)):
                    ahead = self.ahead[k]
                    if b <= self.n - ahead:
                        starts.append((self.cur[k], ahead, prio))
                    elif self.nxt is not None:
                        starts.append((self.nxt[k], ahead - self.n, prio))

                def step(i):
                    self.cur[0](i).wait()
                    for piece, off, prio in starts:
                        piece(i + off).start(priority=prio)
                    self.cur[1](i).wait()
                return step

            def run(self, a, b, fn=None, init=0):
                cuts = sorted({a, b} | {e for e in self.edges if a < e < b})
                for lo, hi in zip(cuts[:-1], cuts[1:]):
                    step = self.stepper(lo, hi)

                    def body(i, c):
                        step(i)
                        return c if fn is None else fn(i, c)
                    init = body(lo, init) if hi - lo == 1 else lax.fori_loop(lo, hi, body, init)
                return init

            def every(self, a, n, k, fn, init=0):
                step = self.stepper(a, a + n * k)

                def body(j, c):
                    step(a + k * j)
                    c = fn(j, c)

                    def rest(u, z):
                        step(a + k * j + u)
                        return z
                    lax.fori_loop(1, k, rest, 0)
                    return c
                return lax.fori_loop(0, n, body, init)

        def pairs(ref, ps):
            return jnp.stack([ref[p >> 7, p & 127] for p in ps])

        def loop(n, body, init=0):
            return lax.fori_loop(0, n, body, init)

        MARK('p_issue')
        for u in range(7):
            m_piece(0, u, 'all').start(priority=LO)
        smalls = [cp(s, d, ssem.at[n]) for n, (s, d) in enumerate(
            [(c_hbm, c_v), (x_hbm, x_v), (w1_hbm, w1_v), (b1_hbm, b1_v), (w2_hbm, w2_v),
             (b2_hbm, b2_v)])]
        for s in smalls:
            s.start(priority=HI)

        for b in range(1, 4):
            for u in range(7):
                m_piece(b, u, 'all' if b < 2 else 'lo').start(priority=LO)

        MARK('p_ma')
        for b0 in range(0, 8, 2):
            def body(b, c):
                for u in range(7):
                    m_piece(b, u, 'lo' if b0 else 'all').wait()
                    lo = m_piece(b + 4, u, 'lo') if b0 < 4 else q_stream[0](7 * (b - 4) + u)
                    hi = m_piece(b + 2, u, 'hi') if b0 < 6 else q_stream[1](7 * (b - 6) + u)
                    lo.start(priority=LO)
                    hi.start(priority=HI)
                    if b0:
                        m_piece(b, u, 'hi').wait()
                return c
            lax.fori_loop(b0, b0 + 2, body, 0)
        for s in smalls:
            s.wait()

        MARK('p_moda')
        k0, v0 = k_stream(0, 0), v_stream(0, 0)
        LW = 28
        ph_q = Phase(q_stream, TB, LW, o_stream)
        ph_o = Phase(o_stream, TB, LW, k0)
        pos = [0]

        def qsteps(n):
            ph_q.run(pos[0], pos[0] + n)
            pos[0] += n

        def qloop(n, k, fn):
            def body(j, c):
                fn(j)
                return c
            ph_q.every(pos[0], n, k, body)
            pos[0] += n * k

        c32 = c_v[...].astype(F32)
        sc = (c32 * jax.nn.sigmoid(c32)).astype(BF16)
        sc16 = jnp.broadcast_to(sc, (16, D))
        w2h = w2_v[...].astype(F32) * 0.5
        w1f = w1_v[...].astype(F32)
        b1f = b1_v[...].astype(F32)
        scf = sc.astype(F32)
        for i in range(NV):
            rows[C_W1 + i:C_W1 + i + 1, :] = w1f[:, (NZ + i) * 128:(NZ + i + 1) * 128] * KS
        rows[C_B1:C_B1 + NV, :] = b1f[NZ:] * KS
        rows[C_SC + ND:C_N, :] = jnp.zeros((C_N - C_SC - ND, 128), F32)
        for i in range(ND):
            rows[C_SC + i:C_SC + i + 1, :] = scf[:, i * 128:(i + 1) * 128]

        def mod_a(i):
            c = pl.ds(m128(i * 384), 384)
            mods[:, c] = jnp.dot(sc16, wm_v[:, :, c].reshape(D, 384),
                                 preferred_element_type=F32)[0:8]
        qloop(5, 4, mod_a)

        def mod_b(i):
            c = pl.ds(m128(3 * D + i * 256), 256)
            mods[:, c] = jnp.dot(sc16[:, :D - DB], wm_v[0:DA - 1, :, c].reshape(D - DB, 256),
                                 preferred_element_type=F32)[0:8]
        qloop(5, 3, mod_b)

        x32 = x_v[0].astype(F32)
        h8 = (_layernorm(x32) * (1.0 + mods[:, D:2 * D]) + mods[:, :D]).astype(BF16).astype(F32)
        consts[2:3, :] = jnp.broadcast_to(jnp.mean(x32, axis=1, keepdims=True), (1, 128))
        consts[3:4, :] = jnp.broadcast_to(
            jnp.mean(mods[0:1, 3 * D:4 * D], axis=1, keepdims=True), (1, 128))
        qsteps(4)

        b1row = jnp.concatenate([b1f[i:i + 1, :] for i in range(NF)], axis=1)
        pw = w1f * w2h
        pb = b1row * w2h
        lhs[...] = _stack_rows(_split(pw) + _split(pb), 8)
        sum_w = jnp.sum(pw, axis=1, keepdims=True)
        sum_b = jnp.sum(pb, axis=1, keepdims=True) + b2_v[...].astype(F32).reshape(1, 1)
        consts[0:1, :] = jnp.broadcast_to(sum_w, (1, 128))
        consts[1:2, :] = jnp.broadcast_to(sum_b, (1, 128))
        qsteps(4)

        al = w1f[:, :NZ * 128] * KS
        be = b1row[:, :NZ * 128] * KS
        a3h, a3l = _split(al * al * al)
        a2h, a2l = _split(3.0 * al * al * be)
        a1h, a1l = _split(al * (3.0 * be * be + CS))
        a0h, a0l = _split(be * (be * be + CS))
        at = _stack_rows([a3h, a3h, a3l, a2h, a2h, a2l, a1h, a1h, a1l, a0h] + _split(a0l), 16)
        for b in range(NZ):
            acol[b * 128:(b + 1) * 128, :] = jnp.concatenate(
                [at[:, b * 128:(b + 1) * 128], jnp.zeros((112, 128), F32)], axis=0).T
        qsteps(3)

        MARK('p_prep')

        def prep(i):
            for u in range(3):
                t = 3 * i + u
                cols[pl.ds(m128(t * 128), 128), :] = _col_bcast(rows[pl.ds(t, 1), :])
        qloop(C_N // 3, 5, prep)

        MARK('p_wq')
        qsteps(TB - pos[0])

        MARK('p_qproj')
        scale = DH ** -0.5

        def q_cols(i, q):
            for t in range(2):
                qb[pl.ds(m128(i * 256 + t * 128), 128), :] = _col_bcast(
                    q[0:1, t * 128:(t + 1) * 128])

        def qproj(i0):
            def fn(i, q_prev):
                q_cols(jnp.maximum(i + i0 - 1, 0), q_prev)
                w = pairs(wq_v, [24 * g + i + i0 for g in range(D // 8)]).astype(F32)
                w = jnp.concatenate([w[:, 0:8].reshape(D, 128), w[:, 8:16].reshape(D, 128)],
                                    axis=1)
                return jnp.dot(h8, w, precision=lax.Precision.DEFAULT,
                               preferred_element_type=F32) * scale
            return fn
        q = ph_o.every(0, 20, 5, qproj(0), jnp.zeros((8, 256), F32))
        q = ph_o.every(100, 2, 7, qproj(20), q)
        q = ph_o.every(114, 2, 7, qproj(22), q)
        for c in range(LW, NB):
            k0[0](c).start(priority=LO)
        MARK('p_k0')
        ph = Phase(k0, NB, NB, v0)
        ph.run(0, 1)
        q_cols(23, q)
        abuf[...] = jnp.zeros((DH, 128), F32)
        wo_last[...] = pairs(wo_v, [60 * (H - 1) + p for p in range(60)]).astype(F32).reshape(
            G * ND, 8, 128)
        ph.run(1, NB)

        def proj(h, a, out):
            o = jnp.sum(a, axis=1, keepdims=True)
            outs = [out, None]
            for jj in range(G // 2):
                tiles = _groups(pairs(wo_v, [60 * h + jj * ND + p for p in range(ND)]).astype(F32).reshape(16 * ND, 128))
                for e in range(2):
                    j = 2 * jj + e
                    w = jnp.concatenate(tiles[e * ND:(e + 1) * ND], axis=1)
                    t = o[j * 8:(j + 1) * 8] * w
                    outs[e] = t if outs[e] is None else outs[e] + t
            return outs[0] + outs[1]

        def phase_a(h, slot, out, ph, tps, n1):
            q = qb[pl.ds(pl.multiple_of(h * DH, 64), DH), :]

            def body(i, m):
                for u in range(tps):
                    c = tps * i + u
                    s = _tree_sum(_groups(kbuf[slot, c].astype(F32) * q))
                    s = jnp.broadcast_to(jnp.sum(s, axis=0, keepdims=True), (8, 128))
                    sbuf[c] = s
                    m = jnp.maximum(m, s)
                return m
            n0 = NB // tps
            m = ph.run(0, n0, body, jnp.full((8, 128), -jnp.inf, F32))
            ph.run(n0, n0 + n1)
            m = jnp.max(m, axis=1, keepdims=True)
            out = proj(jnp.maximum(h - 1, 0), abuf[...], out)
            ph.run(n0 + n1, n0 + n1 + 3)
            p = jnp.exp(sbuf[...] - m)
            sbuf[...] = p
            l = _tree_sum([p[c] for c in range(NB)])
            inv_l = 1.0 / jnp.sum(l, axis=1, keepdims=True)
            return inv_l, out

        def pv_tile(slot, c, acc):
            p = sbuf[c]
            return acc + vbuf[slot, c].astype(F32) * jnp.concatenate([p] * G, axis=0)

        def pv_done(acc, inv_l):
            return acc * jnp.concatenate([jnp.broadcast_to(inv_l, (8, 128))] * G, axis=0)

        def head(h, out):
            slot = h & 1
            nslot = 1 - slot
            knext = k_stream(h + 1, nslot)
            ph = Phase(v_stream(h, slot), NB, NB, knext)
            inv_l, out = phase_a(h, slot, out, ph, 2, 1)
            ph.run(20, NB)
            ph = Phase(knext, NB, NB, v_stream(h + 1, nslot))
            acc = ph.run(0, NB, lambda c, acc: pv_tile(slot, c, acc), jnp.zeros((DH, 128), F32))
            abuf[...] = pv_done(acc, inv_l)
            return out

        MARK('main')
        out = loop(H - 1, head, jnp.zeros((8, D), F32))

        MARK('qk31')
        hl = H - 1
        sl = hl % 2
        slab9.start(priority=LO)
        for b in GB_ORDER:
            gb_piece(b).start(priority=LO)
        ph = Phase(v_stream(hl, sl), NB, NB, None)
        inv_l, out = phase_a(hl, sl, out, ph, 4, 3)

        MARK('pv31')
        acc = ph.run(14, 28, lambda i, acc: pv_tile(sl, 2 * i - 27, pv_tile(sl, 2 * i - 28, acc)),
                     jnp.zeros((DH, 128), F32))
        ga = mods[:, 2 * D:3 * D]
        xp = x32 + ga * jnp.sum(out, axis=0, keepdims=True)
        gl = ga * inv_l
        acc = ph.run(28, NB - 1, lambda c, acc: pv_tile(sl, c, acc), acc)
        MARK('wlast')
        ph.run(NB - 1, NB)
        MARK('proj31')
        o = jnp.sum(pv_tile(sl, NB - 1, acc), axis=1, keepdims=True)
        outs = [None, None]
        for j in range(G):
            w = jnp.concatenate([wo_last[j * ND + n] for n in range(ND)], axis=1)
            t = o[j * 8:(j + 1) * 8] * w
            outs[j & 1] = t if outs[j & 1] is None else outs[j & 1] + t
        x1 = xp + gl * jnp.sum(outs[0] + outs[1], axis=0, keepdims=True)
        d1 = x1 - _tile(consts[2:3, :], ND)
        mom = _moments(d1)

        MARK('w9')
        slab9.wait()
        MARK('ln2')
        mom = _lane_sums(mom)
        macc = None
        for u in range(DB // 8):
            s = cols[pl.ds(C_SC * 128 + D - DB + u * 8, 8), :]
            t = _tile(s, 2 * ND) * wm_v[DA - 1, pl.ds(u * 8, 8), pl.ds(3 * D, 2 * D)].astype(F32)
            macc = t if macc is None else macc + t
        mod = jnp.sum(macc, axis=0, keepdims=True) + mods[0:1, 3 * D:]
        scale_b = jnp.broadcast_to(1.0 + mod[:, D:], (8, D))
        shift_b = jnp.broadcast_to(mod[:, :D] - _tile(consts[3:4, :], ND), (8, D))
        d2 = _normalize(d1, *mom) * scale_b + shift_b
        hn = _normalize(d2, *_lane_sums(_moments(d2)))

        MARK('mlp')

        def tanh_rows(b, u, hn):
            w1c = cols[pl.ds((C_W1 + b - NZ) * 128 + u * 8, 8), :]
            b1c = cols[pl.ds((C_B1 + b - NZ) * 128 + u * 8, 8), :]
            v = hn * _tile(w1c, ND) + _tile(b1c, ND)
            return v, jnp.tanh(v * (v * v + CS))

        p2 = hn * hn
        sid = lax.broadcasted_iota(jnp.int32, (8, D), 0)
        phi, plo = _split(jnp.where(sid < 3, p2 * hn, jnp.where(sid < 6, p2, hn)))
        ptop = jnp.where((sid == 1) | (sid == 4) | (sid == 7), plo, phi)
        pbot = jnp.where(sid == 0, hn, jnp.where(sid < 4, 1.0, 0.0))
        pmat = jnp.concatenate([ptop, pbot], axis=0)
        r = None
        nz, nv = 0, NZ
        zs = []
        late = []
        for kind in ORDER:
            if kind == 'V':
                b = nv
                nv += 1
                ts = [tanh_rows(b, u, hn)[1] for u in range(16)]
                t = jnp.concatenate(ts, axis=0)
            elif kind == 'Z':
                zs.append(jnp.dot(acol[len(zs) * 128:(len(zs) + 1) * 128, 0:16], pmat,
                                  precision=lax.Precision.DEFAULT, preferred_element_type=F32))
                continue
            else:
                b = nz
                nz += 1
                t = jnp.tanh(zs[b])
                if kind == 'S':
                    late.append(b)
                    tbuf[len(late)] = t
                    continue
            rb = jnp.dot(lhs[:, b * 128:(b + 1) * 128], t,
                         precision=lax.Precision.DEFAULT, preferred_element_type=F32)
            r = rb if r is None else r + rb
        hl_ = hn + _tile(_tree_sum(_blocks(ts[0])) * 0.0, ND)
        for u in range(16):
            tbuf[0, u * 8:(u + 1) * 8, :] = tanh_rows(NF - 1, u, hl_)[1]

        def gate(accs, bs):
            for b in bs:
                for a in range(DA):
                    s = cols[pl.ds(C_SC * 128 + a * DB + b * 8, 8), :]
                    t = _tile(s, ND) * wm_v[a, pl.ds(b * 8, 8), pl.ds(5 * D, D)].astype(F32)
                    accs[a & 1] = t if accs[a & 1] is None else accs[a & 1] + t
            return accs

        MARK('gbw')
        for b in GB_ORDER[:-1]:
            gb_piece(b).wait()
        MARK('gb')
        for k, b in enumerate([NF - 1] + late):
            r = r + jnp.dot(lhs[:, b * 128:(b + 1) * 128], tbuf[k],
                            precision=lax.Precision.DEFAULT, preferred_element_type=F32)
        gacc = gate([None, None], GB_ORDER[:-1])
        y = (hn[0:1] * (r[0:1] + r[1:2] + _tile(consts[0:1, :], ND))
             + (r[2:3] + r[3:4] + _tile(consts[1:2, :], ND)))
        MARK('gbw3')
        gb_piece(GB_ORDER[-1]).wait()
        MARK('gb3')
        gacc = gate(gacc, GB_ORDER[-1:])
        gb = jnp.sum(gacc[0] + gacc[1], axis=0, keepdims=True)
        o_ref[0] = (x1[0:1] + gb * y).astype(o_ref.dtype)
        MARK(None)

    return kernel


@jax.jit
def pallas_adaLN_cond__sliding_block_cached__mixer_token_mlp__decode_kernel(
    A_x: jax.Array,
    A_k_cache: jax.Array,
    A_v_cache: jax.Array,
    A_wq: jax.Array,
    A_wo: jax.Array,
    B_x: jax.Array,
    B_w1: jax.Array,
    B_b1: jax.Array,
    B_w2: jax.Array,
    B_b2: jax.Array,
    c: jax.Array,
    w_mod: jax.Array,
):
    SK = A_k_cache.shape[2]
    W = min(4096, max(256, SK // 4))
    kt = jnp.swapaxes(A_k_cache, 2, 3).reshape(H * DH, SK)
    vt = jnp.swapaxes(A_v_cache, 2, 3).reshape(H * DH, SK)

    vmem = pltpu.VMEM
    dma = pltpu.SemaphoreType.DMA
    return pl.pallas_call(
        _make_kernel(SK, W),
        out_shape=jax.ShapeDtypeStruct(A_x.shape, A_x.dtype),
        in_specs=[pl.BlockSpec(memory_space=pl.ANY)] * 11,
        out_specs=pl.BlockSpec(memory_space=pltpu.VMEM),
        scratch_shapes=[
            vmem((2, W // 128, DH, 128), BF16), vmem((2, W // 128, DH, 128), BF16),
            vmem((TA, TB, 16, 128), BF16), vmem((TA, TB, 16, 128), BF16),
            vmem((DA, DB, 6 * D), BF16),
            vmem((1, 1, D), BF16), vmem((1, D), BF16),
            vmem((1, F), BF16), vmem((NF, 128), BF16), vmem((1, F), BF16),
            vmem((1,), BF16),
            vmem((H * DH, 128), F32), vmem((C_N, 128), F32), vmem((C_N * 128, 128), F32),
            vmem((8, F), F32), vmem((DH, 128), F32), vmem((W // 128, 8, 128), F32),
            vmem((4, 128), F32), vmem((8, 5 * D), F32),
            vmem((NZ * 128, 128), F32),
            vmem((G * ND, 8, 128), F32), vmem((1 + ORDER.count('S'), 128, D), F32),
            dma((2,)), dma((2,)), dma((64,)), dma((64,)), dma((9,)), dma((6,)),
        ],
        compiler_params=pltpu.CompilerParams(
            vmem_limit_bytes=64 * 1024 * 1024,
            disable_bounds_checks=True,
            disable_semaphore_checks=True,
        ),
    )(A_x, kt, vt, _pair_view(A_wq), _pair_view(A_wo), B_w1,
      B_b1.reshape(NF, 128), B_w2.reshape(1, F), B_b2, c, w_mod.reshape(DA, DB, 6 * D))
```

```python
import math

import jax
import jax.numpy as jnp
from jax import lax
import jax.experimental.pallas as pl
import jax.experimental.pallas.tpu as pltpu

F32 = jnp.float32
BF16 = jnp.bfloat16

D = 640
H = 32
DH = 192
F = 1536
EPS = 1e-5
G = DH // 8
ND = D // 128
NF = F // 128

LO, HI = 1, 0

_C0 = math.sqrt(2.0 / math.pi)
_C1 = 0.044715
KS = (_C0 * _C1) ** (1.0 / 3.0)
CS = _C0 / KS

ORDER = 'ZVZVVRZVRVZRVVS'
NZ = ORDER.count('Z')
NV = NF - NZ
C_W1, C_B1, C_SC, C_N = 0, NV, 2 * NV, 24

DA, DB = 10, 64
TA, TB = 15, 128


class _Group:
    def __init__(self, copies):
        self.copies = copies

    def start(self, priority):
        for c in self.copies:
            c.start(priority=priority)

    def wait(self):
        for c in self.copies:
            c.wait()


def _pair_view(w):
    r, c = w.shape
    t = w.reshape(r // 8, 8, c // 128, 128).transpose(0, 2, 1, 3)
    return t.reshape(TA, TB, 16, 128)


def _layernorm(x):
    m = jnp.mean(x, axis=-1, keepdims=True)
    xc = x - m
    v = jnp.mean(xc * xc, axis=-1, keepdims=True)
    return xc * lax.rsqrt(v + EPS)


def _moments(d):
    return _tree_sum(_blocks(d)), _tree_sum(_blocks(d * d))


def _lane_sums(xs):
    return [jnp.sum(x, axis=-1, keepdims=True) for x in xs]


def _normalize(d, s1, s2):
    s1 = s1 * (1.0 / D)
    var = jnp.maximum(s2 * (1.0 / D) - s1 * s1, 0.0)
    return (d - s1) * lax.rsqrt(var + EPS)


def _col_bcast(row128):
    return jnp.broadcast_to(row128, (128, 128)).T


def _tile(x, n):
    return jnp.concatenate([x] * n, axis=1)


def _tree_sum(parts):
    while len(parts) > 1:
        nxt = [parts[2 * i] + parts[2 * i + 1] for i in range(len(parts) // 2)]
        if len(parts) % 2:
            nxt.append(parts[-1])
        parts = nxt
    return parts[0]


def _split(a):
    hi = a.astype(BF16).astype(F32)
    return [hi, a - hi]


def _stack_rows(xs, n):
    rid = lax.broadcasted_iota(jnp.int32, (n, xs[0].shape[1]), 0)
    out = jnp.zeros(rid.shape, F32)
    for k, x in enumerate(xs):
        out = jnp.where(rid == k, x, out)
    return out


def _blocks(x):
    return [x[:, j * 128:(j + 1) * 128] for j in range(x.shape[1] // 128)]


def _groups(x):
    return [x[j * 8:(j + 1) * 8, :] for j in range(x.shape[0] // 8)]


def _make_kernel(SK, W):
    LH = 14
    KV_HI = 16
    KV_LO = DH - KV_HI
    W0 = SK - W
    NB = W // 128

    def kernel(x_hbm, k_hbm, v_hbm, wq_hbm, wo_hbm, w1_hbm, b1_hbm, w2_hbm, b2_hbm,
               c_hbm, wm_hbm, o_ref,
               kbuf, vbuf, wq_v, wo_v, wm_v, x_v, c_v, w1_v, b1_v, w2_v, b2_v,
               qb, rows, cols, lhs, abuf, sbuf, consts, mods, acol, wo_last, tbuf,
               klo, khi, vlo, vhi, wsem, ssem):
        cp = pltpu.make_async_copy
        m8 = lambda i: pl.multiple_of(i, 8)
        m128 = lambda i: pl.multiple_of(i, 128)
        MARK = lambda name: None

        def kv_stream(src, buf, lo_sem, hi_sem, h, slot, sem_of):
            def piece(c, r0, n, sem):
                return cp(src.at[pl.ds(m8(h * DH + r0), n), pl.ds(m128(W0 + c * 128), 128)],
                          buf.at[slot, c, pl.ds(r0, n), :], sem.at[sem_of(c)])
            return (lambda c: piece(c, 0, KV_LO, lo_sem),
                    lambda c: piece(c, KV_LO, KV_HI, hi_sem))

        k_stream = lambda h, slot: kv_stream(k_hbm, kbuf, klo, khi, h, slot, lambda c: slot)
        v_stream = lambda h, slot: kv_stream(v_hbm, vbuf, vlo, vhi, h, slot,
                                             lambda c: slot * NB + c)

        def w_piece(src, dst, a0, na, b, c0, n, sem):
            idx = (pl.ds(a0, na), pl.ds(m8(b * 8), 8), pl.ds(m128(c0), n))
            return cp(src.at[idx], dst.at[idx], sem)

        def m_piece(b, u, part, kind=None):
            kind = u if kind is None else kind
            na, c0, n = (DA, u * 384, 384) if kind < 5 else (DA - 1, (u - 2) * D, D)
            a0, na = {'all': (0, na), 'lo': (0, na - 1), 'hi': (na - 1, 1)}[part]
            return w_piece(wm_hbm, wm_v, a0, na, b, c0, n, wsem.at[5 if part == 'hi' else 0])

        def pair_stream(src, dst, s):

            def piece(i, a0, na, r0, nr, sem):
                idx = (pl.ds(a0, na), i, pl.ds(r0, nr))
                return cp(src.at[idx], dst.at[idx], sem)
            return (lambda i: _Group([piece(i, 0, TA, 0, 8, wsem.at[s]),
                                      piece(i, 0, TA - 3, 8, 8, wsem.at[s])]),
                    lambda i: piece(i, TA - 3, 3, 8, 8, wsem.at[s + 1]))
        q_stream = pair_stream(wq_hbm, wq_v, 1)
        o_stream = pair_stream(wo_hbm, wo_v, 3)

        idx9 = (DA - 1, slice(None), pl.ds(3 * D, 2 * D))
        slab9 = cp(wm_hbm.at[idx9], wm_v.at[idx9], wsem.at[6])

        GB_ORDER = (0, 4, 2, 6, 1, 5, 3, 7)
        gb_piece = lambda b: w_piece(wm_hbm, wm_v, 0, DA, b, 5 * D, D,
                                     wsem.at[8 if b in GB_ORDER[-2:] else 7])

        class Phase:
            def __init__(self, cur, n, ll, nxt):
                self.cur, self.n, self.nxt = cur, n, nxt
                self.ahead = (ll, LH)
                self.edges = {n - ll, n - LH}

            def stepper(self, a, b):
                starts = []
                assert not any(a < e < b for e in self.edges), (a, b)
                for k, prio in ((0, LO), (1, HI)):
                    ahead = self.ahead[k]
                    if b <= self.n - ahead:
                        starts.append((self.cur[k], ahead, prio))
                    elif self.nxt is not None:
                        starts.append((self.nxt[k], ahead - self.n, prio))

                def step(i):
                    self.cur[0](i).wait()
                    for piece, off, prio in starts:
                        piece(i + off).start(priority=prio)
                    self.cur[1](i).wait()
                return step

            def run(self, a, b, fn=None, init=0):
                cuts = sorted({a, b} | {e for e in self.edges if a < e < b})
                for lo, hi in zip(cuts[:-1], cuts[1:]):
                    step = self.stepper(lo, hi)

                    def body(i, c):
                        step(i)
                        return c if fn is None else fn(i, c)
                    init = body(lo, init) if hi - lo == 1 else lax.fori_loop(lo, hi, body, init)
                return init

            def every(self, a, n, k, fn, init=0):
                step = self.stepper(a, a + n * k)

                def body(j, c):
                    step(a + k * j)
                    c = fn(j, c)

                    def rest(u, z):
                        step(a + k * j + u)
                        return z
                    lax.fori_loop(1, k, rest, 0)
                    return c
                return lax.fori_loop(0, n, body, init)

        def pairs(ref, ps):
            return jnp.stack([ref[p >> 7, p & 127] for p in ps])

        def loop(n, body, init=0):
            return lax.fori_loop(0, n, body, init)

        MARK('p_issue')
        for u in range(7):
            m_piece(0, u, 'all').start(priority=LO)
        smalls = [cp(s, d, ssem.at[n]) for n, (s, d) in enumerate(
            [(c_hbm, c_v), (x_hbm, x_v), (w1_hbm, w1_v), (b1_hbm, b1_v), (w2_hbm, w2_v),
             (b2_hbm, b2_v)])]
        for s in smalls:
            s.start(priority=HI)

        for b in range(1, 4):
            for u in range(7):
                m_piece(b, u, 'lo').start(priority=LO)
        for u0, u1 in ((0, 5), (5, 7)):
            def body(u, c):
                qb[pl.ds(m128(u * 768), 768), :] = jnp.zeros((768, 128), F32)
                m_piece(1, u, 'hi', u0).start(priority=HI)
                return c
            lax.fori_loop(u0, u1, body, 0)

        MARK('p_ma')
        for b0, b1 in ((0, 1), (1, 4), (4, 6), (6, 8)):
            def body(b, c):
                for u in range(7):
                    m_piece(b, u, 'lo' if b0 else 'all').wait()
                    lo = m_piece(b + 4, u, 'lo') if b0 < 4 else q_stream[0](7 * (b - 4) + u)
                    hi = m_piece(b + 2, u, 'hi') if b0 < 6 else q_stream[1](7 * (b - 6) + u)
                    lo.start(priority=LO)
                    hi.start(priority=HI)
                    if b0:
                        m_piece(b, u, 'hi').wait()
                return c
            lax.fori_loop(b0, b1, body, 0)
        for s in smalls:
            s.wait()

        MARK('p_moda')
        k0, v0 = k_stream(0, 0), v_stream(0, 0)
        LW = 28
        ph_q = Phase(q_stream, TB, LW, o_stream)
        ph_o = Phase(o_stream, TB, LW, k0)
        pos = [0]

        def qsteps(n):
            ph_q.run(pos[0], pos[0] + n)
            pos[0] += n

        def qloop(n, k, fn):
            def body(j, c):
                fn(j)
                return c
            ph_q.every(pos[0], n, k, body)
            pos[0] += n * k

        c32 = c_v[...].astype(F32)
        sc = (c32 * jax.nn.sigmoid(c32)).astype(BF16)
        sc16 = jnp.broadcast_to(sc, (16, D))
        w2h = w2_v[...].astype(F32) * 0.5
        w1f = w1_v[...].astype(F32)
        b1f = b1_v[...].astype(F32)
        scf = sc.astype(F32)
        for i in range(NV):
            rows[C_W1 + i:C_W1 + i + 1, :] = w1f[:, (NZ + i) * 128:(NZ + i + 1) * 128] * KS
        rows[C_B1:C_B1 + NV, :] = b1f[NZ:] * KS
        rows[C_SC + ND:C_N, :] = jnp.zeros((C_N - C_SC - ND, 128), F32)
        for i in range(ND):
            rows[C_SC + i:C_SC + i + 1, :] = scf[:, i * 128:(i + 1) * 128]

        def mod_a(i):
            c = pl.ds(m128(i * 384), 384)
            mods[:, c] = jnp.dot(sc16, wm_v[:, :, c].reshape(D, 384),
                                 preferred_element_type=F32)[0:8]
        qloop(5, 4, mod_a)

        def mod_b(i):
            c = pl.ds(m128(3 * D + i * 256), 256)
            mods[:, c] = jnp.dot(sc16[:, :D - DB], wm_v[0:DA - 1, :, c].reshape(D - DB, 256),
                                 preferred_element_type=F32)[0:8]
        qloop(5, 3, mod_b)

        x32 = x_v[0].astype(F32)
        h8 = (_layernorm(x32) * (1.0 + mods[:, D:2 * D]) + mods[:, :D]).astype(BF16).astype(F32)
        consts[2:3, :] = jnp.broadcast_to(jnp.mean(x32, axis=1, keepdims=True), (1, 128))
        consts[3:4, :] = jnp.broadcast_to(
            jnp.mean(mods[0:1, 3 * D:4 * D], axis=1, keepdims=True), (1, 128))
        qsteps(4)

        b1row = jnp.concatenate([b1f[i:i + 1, :] for i in range(NF)], axis=1)
        pw = w1f * w2h
        pb = b1row * w2h
        lhs[...] = _stack_rows(_split(pw) + _split(pb), 8)
        sum_w = jnp.sum(pw, axis=1, keepdims=True)
        sum_b = jnp.sum(pb, axis=1, keepdims=True) + b2_v[...].astype(F32).reshape(1, 1)
        consts[0:1, :] = jnp.broadcast_to(sum_w, (1, 128))
        consts[1:2, :] = jnp.broadcast_to(sum_b, (1, 128))
        qsteps(4)

        al = w1f[:, :NZ * 128] * KS
        be = b1row[:, :NZ * 128] * KS
        a3h, a3l = _split(al * al * al)
        a2h, a2l = _split(3.0 * al * al * be)
        a1h, a1l = _split(al * (3.0 * be * be + CS))
        a0h, a0l = _split(be * (be * be + CS))
        at = _stack_rows([a3h, a3h, a3l, a2h, a2h, a2l, a1h, a1h, a1l, a0h] + _split(a0l), 16)
        for b in range(NZ):
            acol[b * 128:(b + 1) * 128, :] = jnp.concatenate(
                [at[:, b * 128:(b + 1) * 128], jnp.zeros((112, 128), F32)], axis=0).T
        qsteps(3)

        MARK('p_prep')

        def prep(i):
            for u in range(3):
                t = 3 * i + u
                cols[pl.ds(m128(t * 128), 128), :] = _col_bcast(rows[pl.ds(t, 1), :])
        qloop(C_N // 3, 5, prep)

        MARK('p_wq')
        qsteps(TB - pos[0])

        MARK('p_qproj')
        scale = DH ** -0.5

        def q_cols(i, q):
            for t in range(2):
                qb[pl.ds(m128(i * 256 + t * 128), 128), :] = _col_bcast(
                    q[0:1, t * 128:(t + 1) * 128])

        def qproj(i0):
            def fn(i, q_prev):
                q_cols(jnp.maximum(i + i0 - 1, 0), q_prev)
                w = pairs(wq_v, [24 * g + i + i0 for g in range(D // 8)]).astype(F32)
                w = jnp.concatenate([w[:, 0:8].reshape(D, 128), w[:, 8:16].reshape(D, 128)],
                                    axis=1)
                return jnp.dot(h8, w, precision=lax.Precision.DEFAULT,
                               preferred_element_type=F32) * scale
            return fn
        q = ph_o.every(0, 20, 5, qproj(0), jnp.zeros((8, 256), F32))
        q = ph_o.every(100, 2, 7, qproj(20), q)
        q = ph_o.every(114, 2, 7, qproj(22), q)
        for c in range(LW, NB):
            k0[0](c).start(priority=LO)
        MARK('p_k0')
        ph = Phase(k0, NB, NB, v0)
        ph.run(0, 1)
        q_cols(23, q)
        abuf[...] = jnp.zeros((DH, 128), F32)
        wo_last[...] = pairs(wo_v, [60 * (H - 1) + p for p in range(60)]).astype(F32).reshape(
            G * ND, 8, 128)
        ph.run(1, NB)

        def proj(h, a, out):
            o = jnp.sum(a, axis=1, keepdims=True)
            outs = [out, None]
            for jj in range(G // 2):
                tiles = _groups(pairs(wo_v, [60 * h + jj * ND + p for p in range(ND)]).astype(F32).reshape(16 * ND, 128))
                for e in range(2):
                    j = 2 * jj + e
                    w = jnp.concatenate(tiles[e * ND:(e + 1) * ND], axis=1)
                    t = o[j * 8:(j + 1) * 8] * w
                    outs[e] = t if outs[e] is None else outs[e] + t
            return outs[0] + outs[1]

        def phase_a(h, slot, out, ph, tps, n1):
            q = qb[pl.ds(pl.multiple_of(h * DH, 64), DH), :]

            def body(i, m):
                for u in range(tps):
                    c = tps * i + u
                    s = _tree_sum(_groups(kbuf[slot, c].astype(F32) * q))
                    s = jnp.broadcast_to(jnp.sum(s, axis=0, keepdims=True), (8, 128))
                    sbuf[c] = s
                    m = jnp.maximum(m, s)
                return m
            n0 = NB // tps
            m = ph.run(0, n0, body, jnp.full((8, 128), -jnp.inf, F32))
            ph.run(n0, n0 + n1)
            m = jnp.max(m, axis=1, keepdims=True)
            out = proj(jnp.maximum(h - 1, 0), abuf[...], out)
            ph.run(n0 + n1, n0 + n1 + 3)
            p = jnp.exp(sbuf[...] - m)
            sbuf[...] = p
            l = _tree_sum([p[c] for c in range(NB)])
            inv_l = 1.0 / jnp.sum(l, axis=1, keepdims=True)
            return inv_l, out

        def pv_tile(slot, c, acc):
            p = sbuf[c]
            return acc + vbuf[slot, c].astype(F32) * jnp.concatenate([p] * G, axis=0)

        def pv_done(acc, inv_l):
            return acc * jnp.concatenate([jnp.broadcast_to(inv_l, (8, 128))] * G, axis=0)

        def head(h, out):
            slot = h & 1
            nslot = 1 - slot
            knext = k_stream(h + 1, nslot)
            ph = Phase(v_stream(h, slot), NB, NB, knext)
            inv_l, out = phase_a(h, slot, out, ph, 2, 1)
            ph.run(20, NB)
            ph = Phase(knext, NB, NB, v_stream(h + 1, nslot))
            acc = ph.run(0, NB, lambda c, acc: pv_tile(slot, c, acc), jnp.zeros((DH, 128), F32))
            abuf[...] = pv_done(acc, inv_l)
            return out

        MARK('main')
        out = loop(H - 1, head, jnp.zeros((8, D), F32))

        MARK('qk31')
        hl = H - 1
        sl = hl % 2
        slab9.start(priority=LO)
        for b in GB_ORDER:
            gb_piece(b).start(priority=LO)
        ph = Phase(v_stream(hl, sl), NB, NB, None)
        inv_l, out = phase_a(hl, sl, out, ph, 4, 3)

        MARK('pv31')
        acc = ph.run(14, 28, lambda i, acc: pv_tile(sl, 2 * i - 27, pv_tile(sl, 2 * i - 28, acc)),
                     jnp.zeros((DH, 128), F32))
        ga = mods[:, 2 * D:3 * D]
        xp = x32 + ga * jnp.sum(out, axis=0, keepdims=True)
        gl = ga * inv_l
        acc = ph.run(28, NB - 1, lambda c, acc: pv_tile(sl, c, acc), acc)
        MARK('wlast')
        ph.run(NB - 1, NB)
        MARK('proj31')
        o = jnp.sum(pv_tile(sl, NB - 1, acc), axis=1, keepdims=True)
        outs = [None, None]
        for j in range(G):
            w = jnp.concatenate([wo_last[j * ND + n] for n in range(ND)], axis=1)
            t = o[j * 8:(j + 1) * 8] * w
            outs[j & 1] = t if outs[j & 1] is None else outs[j & 1] + t
        x1 = xp + gl * jnp.sum(outs[0] + outs[1], axis=0, keepdims=True)
        d1 = x1 - _tile(consts[2:3, :], ND)
        mom = _moments(d1)

        MARK('w9')
        slab9.wait()
        MARK('ln2')
        mom = _lane_sums(mom)
        macc = None
        for u in range(DB // 8):
            s = cols[pl.ds(C_SC * 128 + D - DB + u * 8, 8), :]
            t = _tile(s, 2 * ND) * wm_v[DA - 1, pl.ds(u * 8, 8), pl.ds(3 * D, 2 * D)].astype(F32)
            macc = t if macc is None else macc + t
        mod = jnp.sum(macc, axis=0, keepdims=True) + mods[0:1, 3 * D:]
        scale_b = jnp.broadcast_to(1.0 + mod[:, D:], (8, D))
        shift_b = jnp.broadcast_to(mod[:, :D] - _tile(consts[3:4, :], ND), (8, D))
        d2 = _normalize(d1, *mom) * scale_b + shift_b
        hn = _normalize(d2, *_lane_sums(_moments(d2)))

        MARK('mlp')

        def tanh_rows(b, u, hn):
            w1c = cols[pl.ds((C_W1 + b - NZ) * 128 + u * 8, 8), :]
            b1c = cols[pl.ds((C_B1 + b - NZ) * 128 + u * 8, 8), :]
            v = hn * _tile(w1c, ND) + _tile(b1c, ND)
            return v, jnp.tanh(v * (v * v + CS))

        p2 = hn * hn
        sid = lax.broadcasted_iota(jnp.int32, (8, D), 0)
        phi, plo = _split(jnp.where(sid < 3, p2 * hn, jnp.where(sid < 6, p2, hn)))
        ptop = jnp.where((sid == 1) | (sid == 4) | (sid == 7), plo, phi)
        pbot = jnp.where(sid == 0, hn, jnp.where(sid < 4, 1.0, 0.0))
        pmat = jnp.concatenate([ptop, pbot], axis=0)
        r = None
        nz, nv = 0, NZ
        zs = []
        late = []
        for kind in ORDER:
            if kind == 'V':
                b = nv
                nv += 1
                ts = [tanh_rows(b, u, hn)[1] for u in range(16)]
                t = jnp.concatenate(ts, axis=0)
            elif kind == 'Z':
                zs.append(jnp.dot(acol[len(zs) * 128:(len(zs) + 1) * 128, 0:16], pmat,
                                  precision=lax.Precision.DEFAULT, preferred_element_type=F32))
                continue
            else:
                b = nz
                nz += 1
                t = jnp.tanh(zs[b])
                if kind == 'S':
                    late.append(b)
                    tbuf[len(late)] = t
                    continue
            rb = jnp.dot(lhs[:, b * 128:(b + 1) * 128], t,
                         precision=lax.Precision.DEFAULT, preferred_element_type=F32)
            r = rb if r is None else r + rb
        hl_ = hn + _tile(_tree_sum(_blocks(ts[0])) * 0.0, ND)
        for u in range(16):
            tbuf[0, u * 8:(u + 1) * 8, :] = tanh_rows(NF - 1, u, hl_)[1]

        def gate(accs, bs):
            for b in bs:
                for a in range(DA):
                    s = cols[pl.ds(C_SC * 128 + a * DB + b * 8, 8), :]
                    t = _tile(s, ND) * wm_v[a, pl.ds(b * 8, 8), pl.ds(5 * D, D)].astype(F32)
                    accs[a & 1] = t if accs[a & 1] is None else accs[a & 1] + t
            return accs

        MARK('gbw')
        for b in GB_ORDER[:-2]:
            gb_piece(b).wait()
        MARK('gb')
        for k, b in enumerate([NF - 1] + late):
            r = r + jnp.dot(lhs[:, b * 128:(b + 1) * 128], tbuf[k],
                            precision=lax.Precision.DEFAULT, preferred_element_type=F32)
        gacc = gate([None, None], GB_ORDER[:-2])
        y = (hn[0:1] * (r[0:1] + r[1:2] + _tile(consts[0:1, :], ND))
             + (r[2:3] + r[3:4] + _tile(consts[1:2, :], ND)))
        MARK('gbw3')
        for b in GB_ORDER[-2:]:
            gb_piece(b).wait()
        MARK('gb3')
        gacc = gate(gacc, GB_ORDER[-2:])
        gb = jnp.sum(gacc[0] + gacc[1], axis=0, keepdims=True)
        o_ref[0] = (x1[0:1] + gb * y).astype(o_ref.dtype)
        MARK(None)

    return kernel


@jax.jit
def pallas_adaLN_cond__sliding_block_cached__mixer_token_mlp__decode_kernel(
    A_x: jax.Array,
    A_k_cache: jax.Array,
    A_v_cache: jax.Array,
    A_wq: jax.Array,
    A_wo: jax.Array,
    B_x: jax.Array,
    B_w1: jax.Array,
    B_b1: jax.Array,
    B_w2: jax.Array,
    B_b2: jax.Array,
    c: jax.Array,
    w_mod: jax.Array,
):
    SK = A_k_cache.shape[2]
    W = min(4096, max(256, SK // 4))
    kt = jnp.swapaxes(A_k_cache, 2, 3).reshape(H * DH, SK)
    vt = jnp.swapaxes(A_v_cache, 2, 3).reshape(H * DH, SK)

    vmem = pltpu.VMEM
    dma = pltpu.SemaphoreType.DMA
    return pl.pallas_call(
        _make_kernel(SK, W),
        out_shape=jax.ShapeDtypeStruct(A_x.shape, A_x.dtype),
        in_specs=[pl.BlockSpec(memory_space=pl.ANY)] * 11,
        out_specs=pl.BlockSpec(memory_space=pltpu.VMEM),
        scratch_shapes=[
            vmem((2, W // 128, DH, 128), BF16), vmem((2, W // 128, DH, 128), BF16),
            vmem((TA, TB, 16, 128), BF16), vmem((TA, TB, 16, 128), BF16),
            vmem((DA, DB, 6 * D), BF16),
            vmem((1, 1, D), BF16), vmem((1, D), BF16),
            vmem((1, F), BF16), vmem((NF, 128), BF16), vmem((1, F), BF16),
            vmem((1,), BF16),
            vmem((H * DH, 128), F32), vmem((C_N, 128), F32), vmem((C_N * 128, 128), F32),
            vmem((8, F), F32), vmem((DH, 128), F32), vmem((W // 128, 8, 128), F32),
            vmem((4, 128), F32), vmem((8, 5 * D), F32),
            vmem((NZ * 128, 128), F32),
            vmem((G * ND, 8, 128), F32), vmem((1 + ORDER.count('S'), 128, D), F32),
            dma((2,)), dma((2,)), dma((64,)), dma((64,)), dma((9,)), dma((6,)),
        ],
        compiler_params=pltpu.CompilerParams(
            vmem_limit_bytes=64 * 1024 * 1024,
            disable_bounds_checks=True,
            disable_semaphore_checks=True,
        ),
    )(A_x, kt, vt, _pair_view(A_wq), _pair_view(A_wo), B_w1,
      B_b1.reshape(NF, 128), B_w2.reshape(1, F), B_b2, c, w_mod.reshape(DA, DB, 6 * D))
```

```python
import math

import jax
import jax.numpy as jnp
from jax import lax
import jax.experimental.pallas as pl
import jax.experimental.pallas.tpu as pltpu

F32 = jnp.float32
BF16 = jnp.bfloat16

D = 640
H = 32
DH = 192
F = 1536
EPS = 1e-5
G = DH // 8
ND = D // 128
NF = F // 128

LO, HI = 1, 0

_C0 = math.sqrt(2.0 / math.pi)
_C1 = 0.044715
KS = (_C0 * _C1) ** (1.0 / 3.0)
CS = _C0 / KS

ORDER = 'ZVZVVRZVRVZRVVS'
NZ = ORDER.count('Z')
NV = NF - NZ
C_W1, C_B1, C_SC, C_N = 0, NV, 2 * NV, 2 * NV + ND
assert C_N % 3 == 0

DA, DB = 10, 64
TA, TB = 15, 128


class _Group:
    def __init__(self, copies):
        self.copies = copies

    def start(self, priority):
        for c in self.copies:
            c.start(priority=priority)

    def wait(self):
        for c in self.copies:
            c.wait()


def _pair_view(w):
    r, c = w.shape
    t = w.reshape(r // 8, 8, c // 128, 128).transpose(0, 2, 1, 3)
    return t.reshape(TA, TB, 16, 128)


def _layernorm(x):
    m = jnp.mean(x, axis=-1, keepdims=True)
    xc = x - m
    v = jnp.mean(xc * xc, axis=-1, keepdims=True)
    return xc * lax.rsqrt(v + EPS)


def _moments(d):
    return _tree_sum(_blocks(d)), _tree_sum(_blocks(d * d))


def _lane_sums(xs):
    return [jnp.sum(x, axis=-1, keepdims=True) for x in xs]


def _normalize(d, s1, s2):
    s1 = s1 * (1.0 / D)
    var = jnp.maximum(s2 * (1.0 / D) - s1 * s1, 0.0)
    return (d - s1) * lax.rsqrt(var + EPS)


def _col_bcast(row128):
    return jnp.broadcast_to(row128, (128, 128)).T


def _tile(x, n):
    return jnp.concatenate([x] * n, axis=1)


def _tree_sum(parts):
    while len(parts) > 1:
        nxt = [parts[2 * i] + parts[2 * i + 1] for i in range(len(parts) // 2)]
        if len(parts) % 2:
            nxt.append(parts[-1])
        parts = nxt
    return parts[0]


def _split(a):
    hi = a.astype(BF16).astype(F32)
    return [hi, a - hi]


def _stack_rows(xs, n):
    rid = lax.broadcasted_iota(jnp.int32, (n, xs[0].shape[1]), 0)
    out = jnp.zeros(rid.shape, F32)
    for k, x in enumerate(xs):
        out = jnp.where(rid == k, x, out)
    return out


def _blocks(x):
    return [x[:, j * 128:(j + 1) * 128] for j in range(x.shape[1] // 128)]


def _groups(x):
    return [x[j * 8:(j + 1) * 8, :] for j in range(x.shape[0] // 8)]


def _make_kernel(SK, W):
    LH = 14
    KV_HI = 16
    KV_LO = DH - KV_HI
    W0 = SK - W
    NB = W // 128
    assert NB == 32

    def kernel(x_hbm, k_hbm, v_hbm, wq_hbm, wo_hbm, w1_hbm, b1_hbm, w2_hbm, b2_hbm,
               c_hbm, wm_hbm, o_ref,
               kbuf, vbuf, wq_v, wo_v, wm_v, x_v, c_v, w1_v, b1_v, w2_v, b2_v,
               qb, rows, cols, lhs, abuf, sbuf, consts, mods, acol, wo_last, tbuf,
               klo, khi, vlo, vhi, wsem, ssem):
        cp = pltpu.make_async_copy
        m8 = lambda i: pl.multiple_of(i, 8)
        m128 = lambda i: pl.multiple_of(i, 128)
        MARK = lambda name: None

        def kv_stream(src, buf, lo_sem, hi_sem, h, slot, sem_of):
            def piece(c, r0, n, sem):
                return cp(src.at[pl.ds(m8(h * DH + r0), n), pl.ds(m128(W0 + c * 128), 128)],
                          buf.at[slot, c, pl.ds(r0, n), :], sem.at[sem_of(c)])
            return (lambda c: piece(c, 0, KV_LO, lo_sem),
                    lambda c: piece(c, KV_LO, KV_HI, hi_sem))

        k_stream = lambda h, slot: kv_stream(k_hbm, kbuf, klo, khi, h, slot, lambda c: slot)
        v_stream = lambda h, slot: kv_stream(v_hbm, vbuf, vlo, vhi, h, slot,
                                             lambda c: slot * NB + c)

        def w_piece(src, dst, a0, na, b, c0, n, sem):
            idx = (pl.ds(a0, na), pl.ds(m8(b * 8), 8), pl.ds(m128(c0), n))
            return cp(src.at[idx], dst.at[idx], sem)

        def m_piece(b, u, part, kind=None):
            kind = u if kind is None else kind
            na, c0, n = (DA, u * 384, 384) if kind < 5 else (DA - 1, (u - 2) * D, D)
            a0, na = {'all': (0, na), 'lo': (0, na - 1), 'hi': (na - 1, 1)}[part]
            return w_piece(wm_hbm, wm_v, a0, na, b, c0, n, wsem.at[5 if part == 'hi' else 0])

        def pair_stream(src, dst, s):
            def piece(i, a0, na, r0, nr, sem):
                idx = (pl.ds(a0, na), i, pl.ds(r0, nr))
                return cp(src.at[idx], dst.at[idx], sem)
            return (lambda i: _Group([piece(i, 0, TA, 0, 8, wsem.at[s]),
                                      piece(i, 0, TA - 3, 8, 8, wsem.at[s])]),
                    lambda i: piece(i, TA - 3, 3, 8, 8, wsem.at[s + 1]))
        q_stream = pair_stream(wq_hbm, wq_v, 1)
        o_stream = pair_stream(wo_hbm, wo_v, 3)

        idx9 = (DA - 1, slice(None), pl.ds(3 * D, 2 * D))
        slab9 = cp(wm_hbm.at[idx9], wm_v.at[idx9], wsem.at[6])

        GB_ORDER = (0, 4, 2, 6, 1, 5, 3, 7)
        gb_piece = lambda b: w_piece(wm_hbm, wm_v, 0, DA, b, 5 * D, D,
                                     wsem.at[8 if b in GB_ORDER[-2:] else 7])

        class Phase:
            def __init__(self, cur, n, ll, nxt):
                self.cur, self.n, self.nxt = cur, n, nxt
                self.ahead = (ll, LH)
                self.edges = {n - ll, n - LH}

            def stepper(self, a, b):
                starts = []
                assert not any(a < e < b for e in self.edges), (a, b)
                for k, prio in ((0, LO), (1, HI)):
                    ahead = self.ahead[k]
                    if b <= self.n - ahead:
                        starts.append((self.cur[k], ahead, prio))
                    elif self.nxt is not None:
                        starts.append((self.nxt[k], ahead - self.n, prio))

                def step(i):
                    self.cur[0](i).wait()
                    for piece, off, prio in starts:
                        piece(i + off).start(priority=prio)
                    self.cur[1](i).wait()
                return step

            def run(self, a, b, fn=None, init=0):
                cuts = sorted({a, b} | {e for e in self.edges if a < e < b})
                for lo, hi in zip(cuts[:-1], cuts[1:]):
                    step = self.stepper(lo, hi)

                    def body(i, c):
                        step(i)
                        return c if fn is None else fn(i, c)
                    init = body(lo, init) if hi - lo == 1 else lax.fori_loop(lo, hi, body, init)
                return init

            def every(self, a, n, k, fn, init=0):
                step = self.stepper(a, a + n * k)

                def body(j, c):
                    step(a + k * j)
                    c = fn(j, c)

                    def rest(u, z):
                        step(a + k * j + u)
                        return z
                    lax.fori_loop(1, k, rest, 0)
                    return c
                return lax.fori_loop(0, n, body, init)

        def pairs(ref, ps):
            return jnp.stack([ref[p >> 7, p & 127] for p in ps])

        MARK('p_issue')
        for u in range(7):
            m_piece(0, u, 'all').start(priority=LO)
        smalls = [cp(s, d, ssem.at[n]) for n, (s, d) in enumerate(
            [(c_hbm, c_v), (x_hbm, x_v), (w1_hbm, w1_v), (b1_hbm, b1_v), (w2_hbm, w2_v),
             (b2_hbm, b2_v)])]
        for s in smalls:
            s.start(priority=HI)

        for b in range(1, 4):
            for u in range(7):
                m_piece(b, u, 'lo').start(priority=LO)
        for u0, u1 in ((0, 5), (5, 7)):
            def body(u, c):
                qb[pl.ds(m128(u * 768), 768), :] = jnp.zeros((768, 128), F32)
                m_piece(1, u, 'hi', u0).start(priority=HI)
                return c
            lax.fori_loop(u0, u1, body, 0)

        MARK('p_ma')
        for b0, b1 in ((0, 1), (1, 4), (4, 6), (6, 8)):
            def body(b, c):
                for u in range(7):
                    m_piece(b, u, 'lo' if b0 else 'all').wait()
                    lo = m_piece(b + 4, u, 'lo') if b0 < 4 else q_stream[0](7 * (b - 4) + u)
                    hi = m_piece(b + 2, u, 'hi') if b0 < 6 else q_stream[1](7 * (b - 6) + u)
                    lo.start(priority=LO)
                    hi.start(priority=HI)
                    if b0:
                        m_piece(b, u, 'hi').wait()
                return c
            lax.fori_loop(b0, b1, body, 0)
        for s in smalls:
            s.wait()

        MARK('p_moda')
        k0, v0 = k_stream(0, 0), v_stream(0, 0)
        LW = 28
        ph_q = Phase(q_stream, TB, LW, o_stream)
        ph_o = Phase(o_stream, TB, LW, k0)
        pos = [0]

        def qsteps(n):
            ph_q.run(pos[0], pos[0] + n)
            pos[0] += n

        def qloop(n, k, fn):
            def body(j, c):
                fn(j)
                return c
            ph_q.every(pos[0], n, k, body)
            pos[0] += n * k

        c32 = c_v[...].astype(F32)
        sc = (c32 * jax.nn.sigmoid(c32)).astype(BF16)
        sc16 = jnp.broadcast_to(sc, (16, D))
        w2h = w2_v[...].astype(F32) * 0.5
        w1f = w1_v[...].astype(F32)
        b1f = b1_v[...].astype(F32)
        scf = sc.astype(F32)
        for i in range(NV):
            rows[C_W1 + i:C_W1 + i + 1, :] = w1f[:, (NZ + i) * 128:(NZ + i + 1) * 128] * KS
        rows[C_B1:C_B1 + NV, :] = b1f[NZ:] * KS
        for i in range(ND):
            rows[C_SC + i:C_SC + i + 1, :] = scf[:, i * 128:(i + 1) * 128]

        def mod_a(i):
            c = pl.ds(m128(i * 384), 384)
            mods[:, c] = jnp.dot(sc16, wm_v[:, :, c].reshape(D, 384),
                                 preferred_element_type=F32)[0:8]
        qloop(5, 4, mod_a)

        def mod_b(i):
            c = pl.ds(m128(3 * D + i * 256), 256)
            mods[:, c] = jnp.dot(sc16[:, :D - DB], wm_v[0:DA - 1, :, c].reshape(D - DB, 256),
                                 preferred_element_type=F32)[0:8]
        qloop(5, 3, mod_b)

        x32 = x_v[0].astype(F32)
        h8 = (_layernorm(x32) * (1.0 + mods[:, D:2 * D]) + mods[:, :D]).astype(BF16).astype(F32)
        consts[2:3, :] = jnp.broadcast_to(jnp.mean(x32, axis=1, keepdims=True), (1, 128))
        consts[3:4, :] = jnp.broadcast_to(
            jnp.mean(mods[0:1, 3 * D:4 * D], axis=1, keepdims=True), (1, 128))
        qsteps(4)

        b1row = jnp.concatenate([b1f[i:i + 1, :] for i in range(NF)], axis=1)
        pw = w1f * w2h
        pb = b1row * w2h
        lhs[...] = _stack_rows(_split(pw) + _split(pb), 8)
        sum_w = jnp.sum(pw, axis=1, keepdims=True)
        sum_b = jnp.sum(pb, axis=1, keepdims=True) + b2_v[...].astype(F32).reshape(1, 1)
        consts[0:1, :] = jnp.broadcast_to(sum_w, (1, 128))
        consts[1:2, :] = jnp.broadcast_to(sum_b, (1, 128))
        qsteps(4)

        al = w1f[:, :NZ * 128] * KS
        be = b1row[:, :NZ * 128] * KS
        a3h, a3l = _split(al * al * al)
        a2h, a2l = _split(3.0 * al * al * be)
        a1h, a1l = _split(al * (3.0 * be * be + CS))
        a0h, a0l = _split(be * (be * be + CS))
        at = _stack_rows([a3h, a3h, a3l, a2h, a2h, a2l, a1h, a1h, a1l, a0h] + _split(a0l), 16)
        for b in range(NZ):
            acol[b * 128:(b + 1) * 128, :] = jnp.concatenate(
                [at[:, b * 128:(b + 1) * 128], jnp.zeros((112, 128), F32)], axis=0).T
        qsteps(3)

        MARK('p_prep')

        def prep(i):
            for u in range(3):
                t = 3 * i + u
                cols[pl.ds(m128(t * 128), 128), :] = _col_bcast(rows[pl.ds(t, 1), :])
        qloop(C_N // 3, 5, prep)

        MARK('p_wq')
        qsteps(TB - pos[0])

        MARK('p_qproj')
        scale = DH ** -0.5

        def q_cols(i, q):
            for t in range(2):
                qb[pl.ds(m128(i * 256 + t * 128), 128), :] = _col_bcast(
                    q[0:1, t * 128:(t + 1) * 128])

        def qproj(i0):
            def fn(i, q_prev):
                q_cols(jnp.maximum(i + i0 - 1, 0), q_prev)
                w = pairs(wq_v, [24 * g + i + i0 for g in range(D // 8)]).astype(F32)
                w = jnp.concatenate([w[:, 0:8].reshape(D, 128), w[:, 8:16].reshape(D, 128)],
                                    axis=1)
                return jnp.dot(h8, w, precision=lax.Precision.DEFAULT,
                               preferred_element_type=F32) * scale
            return fn
        q = ph_o.every(0, 20, 5, qproj(0), jnp.zeros((8, 256), F32))
        q = ph_o.every(100, 2, 7, qproj(20), q)
        q = ph_o.every(114, 2, 7, qproj(22), q)
        for c in range(LW, NB):
            k0[0](c).start(priority=LO)
        MARK('p_k0')
        ph = Phase(k0, NB, NB, v0)
        ph.run(0, 1)
        q_cols(23, q)
        abuf[...] = jnp.zeros((DH, 128), F32)
        wo_last[...] = pairs(wo_v, [60 * (H - 1) + p for p in range(60)]).astype(F32).reshape(
            G * ND, 8, 128)
        ph.run(1, NB)

        def proj(h, a, out):
            o = jnp.sum(a, axis=1, keepdims=True)
            outs = [out, None]
            for jj in range(G // 2):
                w = pairs(wo_v, [60 * h + jj * ND + p for p in range(ND)]).astype(F32)
                tiles = _groups(w.reshape(16 * ND, 128))
                for e in range(2):
                    j = 2 * jj + e
                    w = jnp.concatenate(tiles[e * ND:(e + 1) * ND], axis=1)
                    t = o[j * 8:(j + 1) * 8] * w
                    outs[e] = t if outs[e] is None else outs[e] + t
            return outs[0] + outs[1]

        def phase_a(h, slot, out, ph, tps, n1):
            q = qb[pl.ds(pl.multiple_of(h * DH, 64), DH), :]

            def body(i, m):
                for u in range(tps):
                    c = tps * i + u
                    s = _tree_sum(_groups(kbuf[slot, c].astype(F32) * q))
                    s = jnp.broadcast_to(jnp.sum(s, axis=0, keepdims=True), (8, 128))
                    sbuf[c] = s
                    m = jnp.maximum(m, s)
                return m
            n0 = NB // tps
            m = ph.run(0, n0, body, jnp.full((8, 128), -jnp.inf, F32))
            ph.run(n0, n0 + n1)
            m = jnp.max(m, axis=1, keepdims=True)
            out = proj(jnp.maximum(h - 1, 0), abuf[...], out)
            ph.run(n0 + n1, n0 + n1 + 3)
            p = jnp.exp(sbuf[...] - m)
            sbuf[...] = p
            l = _tree_sum([p[c] for c in range(NB)])
            inv_l = 1.0 / jnp.sum(l, axis=1, keepdims=True)
            return inv_l, out

        def pv_tile(slot, c, acc):
            p = sbuf[c]
            return acc + vbuf[slot, c].astype(F32) * jnp.concatenate([p] * G, axis=0)

        def pv_done(acc, inv_l):
            return acc * jnp.concatenate([jnp.broadcast_to(inv_l, (8, 128))] * G, axis=0)

        def head(h, out):
            slot = h & 1
            nslot = 1 - slot
            knext = k_stream(h + 1, nslot)
            ph = Phase(v_stream(h, slot), NB, NB, knext)
            inv_l, out = phase_a(h, slot, out, ph, 2, 1)
            ph.run(20, NB)
            ph = Phase(knext, NB, NB, v_stream(h + 1, nslot))
            acc = ph.run(0, NB, lambda c, acc: pv_tile(slot, c, acc), jnp.zeros((DH, 128), F32))
            abuf[...] = pv_done(acc, inv_l)
            return out

        MARK('main')
        out = lax.fori_loop(0, H - 1, head, jnp.zeros((8, D), F32))

        MARK('qk31')
        hl = H - 1
        sl = hl % 2
        slab9.start(priority=LO)
        for b in GB_ORDER:
            gb_piece(b).start(priority=LO)
        ph = Phase(v_stream(hl, sl), NB, NB, None)
        inv_l, out = phase_a(hl, sl, out, ph, 4, 3)

        MARK('pv31')
        acc = ph.run(14, 28, lambda i, acc: pv_tile(sl, 2 * i - 27, pv_tile(sl, 2 * i - 28, acc)),
                     jnp.zeros((DH, 128), F32))
        ga = mods[:, 2 * D:3 * D]
        xp = x32 + ga * jnp.sum(out, axis=0, keepdims=True)
        gl = ga * inv_l
        acc = ph.run(28, NB - 1, lambda c, acc: pv_tile(sl, c, acc), acc)
        MARK('wlast')
        ph.run(NB - 1, NB)
        MARK('proj31')
        o = jnp.sum(pv_tile(sl, NB - 1, acc), axis=1, keepdims=True)
        outs = [None, None]
        for j in range(G):
            w = jnp.concatenate([wo_last[j * ND + n] for n in range(ND)], axis=1)
            t = o[j * 8:(j + 1) * 8] * w
            outs[j & 1] = t if outs[j & 1] is None else outs[j & 1] + t
        x1 = xp + gl * jnp.sum(outs[0] + outs[1], axis=0, keepdims=True)
        d1 = x1 - _tile(consts[2:3, :], ND)
        mom = _moments(d1)

        MARK('w9')
        slab9.wait()
        MARK('ln2')
        mom = _lane_sums(mom)
        macc = None
        for u in range(DB // 8):
            s = cols[pl.ds(C_SC * 128 + D - DB + u * 8, 8), :]
            t = _tile(s, 2 * ND) * wm_v[DA - 1, pl.ds(u * 8, 8), pl.ds(3 * D, 2 * D)].astype(F32)
            macc = t if macc is None else macc + t
        mod = jnp.sum(macc, axis=0, keepdims=True) + mods[0:1, 3 * D:]
        scale_b = jnp.broadcast_to(1.0 + mod[:, D:], (8, D))
        shift_b = jnp.broadcast_to(mod[:, :D] - _tile(consts[3:4, :], ND), (8, D))
        d2 = _normalize(d1, *mom) * scale_b + shift_b
        hn = _normalize(d2, *_lane_sums(_moments(d2)))

        MARK('mlp')

        def tanh_rows(b, u, hn):
            w1c = cols[pl.ds((C_W1 + b - NZ) * 128 + u * 8, 8), :]
            b1c = cols[pl.ds((C_B1 + b - NZ) * 128 + u * 8, 8), :]
            v = hn * _tile(w1c, ND) + _tile(b1c, ND)
            return jnp.tanh(v * (v * v + CS))

        p2 = hn * hn
        sid = lax.broadcasted_iota(jnp.int32, (8, D), 0)
        phi, plo = _split(jnp.where(sid < 3, p2 * hn, jnp.where(sid < 6, p2, hn)))
        ptop = jnp.where((sid == 1) | (sid == 4) | (sid == 7), plo, phi)
        pbot = jnp.where(sid == 0, hn, jnp.where(sid < 4, 1.0, 0.0))
        pmat = jnp.concatenate([ptop, pbot], axis=0)
        r = None
        nz, nv = 0, NZ
        zs = []
        late = []
        for kind in ORDER:
            if kind == 'V':
                b = nv
                nv += 1
                ts = [tanh_rows(b, u, hn) for u in range(16)]
                t = jnp.concatenate(ts, axis=0)
            elif kind == 'Z':
                zs.append(jnp.dot(acol[len(zs) * 128:(len(zs) + 1) * 128, 0:16], pmat,
                                  precision=lax.Precision.DEFAULT, preferred_element_type=F32))
                continue
            else:
                b = nz
                nz += 1
                t = jnp.tanh(zs[b])
                if kind == 'S':
                    late.append(b)
                    tbuf[len(late)] = t
                    continue
            rb = jnp.dot(lhs[:, b * 128:(b + 1) * 128], t,
                         precision=lax.Precision.DEFAULT, preferred_element_type=F32)
            r = rb if r is None else r + rb
        hl_ = hn + _tile(_tree_sum(_blocks(ts[0])) * 0.0, ND)
        for u in range(16):
            tbuf[0, u * 8:(u + 1) * 8, :] = tanh_rows(NF - 1, u, hl_)

        def gate(accs, bs):
            for b in bs:
                for a in range(DA):
                    s = cols[pl.ds(C_SC * 128 + a * DB + b * 8, 8), :]
                    t = _tile(s, ND) * wm_v[a, pl.ds(b * 8, 8), pl.ds(5 * D, D)].astype(F32)
                    accs[a & 1] = t if accs[a & 1] is None else accs[a & 1] + t
            return accs

        MARK('gbw')
        for b in GB_ORDER[:-2]:
            gb_piece(b).wait()
        MARK('gb')
        for k, b in enumerate([NF - 1] + late):
            r = r + jnp.dot(lhs[:, b * 128:(b + 1) * 128], tbuf[k],
                            precision=lax.Precision.DEFAULT, preferred_element_type=F32)
        gacc = gate([None, None], GB_ORDER[:-2])
        y = (hn[0:1] * (r[0:1] + r[1:2] + _tile(consts[0:1, :], ND))
             + (r[2:3] + r[3:4] + _tile(consts[1:2, :], ND)))
        MARK('gbw3')
        for b in GB_ORDER[-2:]:
            gb_piece(b).wait()
        MARK('gb3')
        gacc = gate(gacc, GB_ORDER[-2:])
        gb = jnp.sum(gacc[0] + gacc[1], axis=0, keepdims=True)
        o_ref[0] = (x1[0:1] + gb * y).astype(o_ref.dtype)
        MARK(None)

    return kernel


@jax.jit
def pallas_adaLN_cond__sliding_block_cached__mixer_token_mlp__decode_kernel(
    A_x: jax.Array,
    A_k_cache: jax.Array,
    A_v_cache: jax.Array,
    A_wq: jax.Array,
    A_wo: jax.Array,
    B_x: jax.Array,
    B_w1: jax.Array,
    B_b1: jax.Array,
    B_w2: jax.Array,
    B_b2: jax.Array,
    c: jax.Array,
    w_mod: jax.Array,
):
    SK = A_k_cache.shape[2]
    W = min(4096, max(256, SK // 4))
    kt = jnp.swapaxes(A_k_cache, 2, 3).reshape(H * DH, SK)
    vt = jnp.swapaxes(A_v_cache, 2, 3).reshape(H * DH, SK)

    vmem = pltpu.VMEM
    dma = pltpu.SemaphoreType.DMA
    return pl.pallas_call(
        _make_kernel(SK, W),
        out_shape=jax.ShapeDtypeStruct(A_x.shape, A_x.dtype),
        in_specs=[pl.BlockSpec(memory_space=pl.ANY)] * 11,
        out_specs=pl.BlockSpec(memory_space=pltpu.VMEM),
        scratch_shapes=[
            vmem((2, W // 128, DH, 128), BF16), vmem((2, W // 128, DH, 128), BF16),
            vmem((TA, TB, 16, 128), BF16), vmem((TA, TB, 16, 128), BF16),
            vmem((DA, DB, 6 * D), BF16),
            vmem((1, 1, D), BF16), vmem((1, D), BF16),
            vmem((1, F), BF16), vmem((NF, 128), BF16), vmem((1, F), BF16),
            vmem((1,), BF16),
            vmem((H * DH, 128), F32), vmem((C_N, 128), F32), vmem((C_N * 128, 128), F32),
            vmem((8, F), F32), vmem((DH, 128), F32), vmem((W // 128, 8, 128), F32),
            vmem((4, 128), F32), vmem((8, 5 * D), F32),
            vmem((NZ * 128, 128), F32),
            vmem((G * ND, 8, 128), F32), vmem((1 + ORDER.count('S'), 128, D), F32),
            dma((2,)), dma((2,)), dma((64,)), dma((64,)), dma((9,)), dma((6,)),
        ],
        compiler_params=pltpu.CompilerParams(
            vmem_limit_bytes=64 * 1024 * 1024,
            disable_bounds_checks=True,
            disable_semaphore_checks=True,
        ),
    )(A_x, kt, vt, _pair_view(A_wq), _pair_view(A_wo), B_w1,
      B_b1.reshape(NF, 128), B_w2.reshape(1, F), B_b2, c, w_mod.reshape(DA, DB, 6 * D))
```

```python
import math

import jax
import jax.numpy as jnp
from jax import lax
import jax.experimental.pallas as pl
import jax.experimental.pallas.tpu as pltpu

F32 = jnp.float32
BF16 = jnp.bfloat16

D = 640
H = 32
DH = 192
F = 1536
EPS = 1e-5
G = DH // 8
ND = D // 128
NF = F // 128

LO, HI = 1, 0

_C0 = math.sqrt(2.0 / math.pi)
_C1 = 0.044715
KS = (_C0 * _C1) ** (1.0 / 3.0)
CS = _C0 / KS

ORDER = 'ZVZVVRZVRVZRVVS'
NZ = ORDER.count('Z')
NV = NF - NZ
C_W1, C_B1, C_SC, C_N = 0, NV, 2 * NV, 2 * NV + ND
assert C_N % 3 == 0

DA, DB = 10, 64
TA, TB = 15, 128


class _Group:
    def __init__(self, copies):
        self.copies = copies

    def start(self, priority):
        for c in self.copies:
            c.start(priority=priority)

    def wait(self):
        for c in self.copies:
            c.wait()


def _pair_view(w):
    r, c = w.shape
    t = w.reshape(r // 8, 8, c // 128, 128).transpose(0, 2, 1, 3)
    return t.reshape(TA, TB, 16, 128)


def _layernorm(x):
    m = jnp.mean(x, axis=-1, keepdims=True)
    xc = x - m
    v = jnp.mean(xc * xc, axis=-1, keepdims=True)
    return xc * lax.rsqrt(v + EPS)


def _moments(d):
    return _tree_sum(_blocks(d)), _tree_sum(_blocks(d * d))


def _lane_sums(xs):
    return [jnp.sum(x, axis=-1, keepdims=True) for x in xs]


def _normalize(d, s1, s2):
    s1 = s1 * (1.0 / D)
    var = jnp.maximum(s2 * (1.0 / D) - s1 * s1, 0.0)
    return (d - s1) * lax.rsqrt(var + EPS)


def _col_bcast(row128):
    return jnp.broadcast_to(row128, (128, 128)).T


def _tile(x, n):
    return jnp.concatenate([x] * n, axis=1)


def _tree_sum(parts):
    while len(parts) > 1:
        nxt = [parts[2 * i] + parts[2 * i + 1] for i in range(len(parts) // 2)]
        if len(parts) % 2:
            nxt.append(parts[-1])
        parts = nxt
    return parts[0]


def _split(a):
    hi = a.astype(BF16).astype(F32)
    return [hi, a - hi]


def _stack_rows(xs, n):
    rid = lax.broadcasted_iota(jnp.int32, (n, xs[0].shape[1]), 0)
    out = jnp.zeros(rid.shape, F32)
    for k, x in enumerate(xs):
        out = jnp.where(rid == k, x, out)
    return out


def _blocks(x):
    return [x[:, j * 128:(j + 1) * 128] for j in range(x.shape[1] // 128)]


def _groups(x):
    return [x[j * 8:(j + 1) * 8, :] for j in range(x.shape[0] // 8)]


def _make_kernel(SK, W):
    LH = 14
    KV_HI = 16
    KV_LO = DH - KV_HI
    W0 = SK - W
    NB = W // 128
    assert NB == 32

    def kernel(x_hbm, k_hbm, v_hbm, wq_hbm, wo_hbm, w1_hbm, b1_hbm, w2_hbm, b2_hbm,
               c_hbm, wm_hbm, o_ref,
               kbuf, vbuf, wq_v, wo_v, wm_v, x_v, c_v, w1_v, b1_v, w2_v, b2_v,
               qb, rows, cols, lhs, abuf, sbuf, consts, mods, acol, wo_last, tbuf,
               klo, khi, vlo, vhi, wsem, ssem):
        cp = pltpu.make_async_copy
        m8 = lambda i: pl.multiple_of(i, 8)
        m128 = lambda i: pl.multiple_of(i, 128)
        MARK = lambda name: None

        def kv_stream(src, buf, lo_sem, hi_sem, h, slot, sem_of):
            def piece(c, r0, n, sem):
                return cp(src.at[pl.ds(m8(h * DH + r0), n), pl.ds(m128(W0 + c * 128), 128)],
                          buf.at[slot, c, pl.ds(r0, n), :], sem.at[sem_of(c)])
            return (lambda c: piece(c, 0, KV_LO, lo_sem),
                    lambda c: piece(c, KV_LO, KV_HI, hi_sem))

        k_stream = lambda h, slot: kv_stream(k_hbm, kbuf, klo, khi, h, slot, lambda c: slot)
        v_stream = lambda h, slot: kv_stream(v_hbm, vbuf, vlo, vhi, h, slot,
                                             lambda c: slot * NB + c)

        def w_piece(src, dst, a0, na, b, c0, n, sem):
            idx = (pl.ds(a0, na), pl.ds(m8(b * 8), 8), pl.ds(m128(c0), n))
            return cp(src.at[idx], dst.at[idx], sem)

        def m_piece(b, u, part, kind=None):
            kind = u if kind is None else kind
            na, c0, n = (DA, u * 384, 384) if kind < 5 else (DA - 1, (u - 2) * D, D)
            a0, na = {'all': (0, na), 'lo': (0, na - 1), 'hi': (na - 1, 1)}[part]
            return w_piece(wm_hbm, wm_v, a0, na, b, c0, n, wsem.at[5 if part == 'hi' else 0])

        def pair_stream(src, dst, s):
            def piece(i, a0, na, r0, nr, sem):
                idx = (pl.ds(a0, na), i, pl.ds(r0, nr))
                return cp(src.at[idx], dst.at[idx], sem)
            return (lambda i: _Group([piece(i, 0, TA, 0, 8, wsem.at[s]),
                                      piece(i, 0, TA - 3, 8, 8, wsem.at[s])]),
                    lambda i: piece(i, TA - 3, 3, 8, 8, wsem.at[s + 1]))
        q_stream = pair_stream(wq_hbm, wq_v, 1)
        o_stream = pair_stream(wo_hbm, wo_v, 3)

        N9 = 5

        def slab9(k):
            r = pl.ds(8 * N9, DB - 8 * N9) if k else pl.ds(0, 8 * N9)
            idx = (DA - 1, r, pl.ds(3 * D, 2 * D))
            return cp(wm_hbm.at[idx], wm_v.at[idx], wsem.at[9 if k else 6])

        GB_ORDER = (0, 4, 2, 6, 1, 5, 3, 7)
        gb_piece = lambda b: w_piece(wm_hbm, wm_v, 0, DA, b, 5 * D, D,
                                     wsem.at[8 if b in GB_ORDER[-2:] else 7])

        class Phase:
            def __init__(self, cur, n, ll, nxt):
                self.cur, self.n, self.nxt = cur, n, nxt
                self.ahead = (ll, LH)
                self.edges = {n - ll, n - LH}

            def stepper(self, a, b):
                starts = []
                assert not any(a < e < b for e in self.edges), (a, b)
                for k, prio in ((0, LO), (1, HI)):
                    ahead = self.ahead[k]
                    if b <= self.n - ahead:
                        starts.append((self.cur[k], ahead, prio))
                    elif self.nxt is not None:
                        starts.append((self.nxt[k], ahead - self.n, prio))

                def step(i):
                    self.cur[0](i).wait()
                    for piece, off, prio in starts:
                        piece(i + off).start(priority=prio)
                    self.cur[1](i).wait()
                return step

            def run(self, a, b, fn=None, init=0):
                cuts = sorted({a, b} | {e for e in self.edges if a < e < b})
                for lo, hi in zip(cuts[:-1], cuts[1:]):
                    step = self.stepper(lo, hi)

                    def body(i, c):
                        step(i)
                        return c if fn is None else fn(i, c)
                    init = body(lo, init) if hi - lo == 1 else lax.fori_loop(lo, hi, body, init)
                return init

            def every(self, a, n, k, fn, init=0):
                step = self.stepper(a, a + n * k)

                def body(j, c):
                    step(a + k * j)
                    c = fn(j, c)

                    def rest(u, z):
                        step(a + k * j + u)
                        return z
                    lax.fori_loop(1, k, rest, 0)
                    return c
                return lax.fori_loop(0, n, body, init)

        def pairs(ref, ps):
            return jnp.stack([ref[p >> 7, p & 127] for p in ps])

        MARK('p_issue')
        for u in range(7):
            m_piece(0, u, 'all').start(priority=LO)
        smalls = [cp(s, d, ssem.at[n]) for n, (s, d) in enumerate(
            [(c_hbm, c_v), (x_hbm, x_v), (w1_hbm, w1_v), (b1_hbm, b1_v), (w2_hbm, w2_v),
             (b2_hbm, b2_v)])]
        for s in smalls:
            s.start(priority=HI)

        for b in range(1, 4):
            for u in range(7):
                m_piece(b, u, 'lo').start(priority=LO)
        for u0, u1 in ((0, 5), (5, 7)):
            def body(u, c):
                qb[pl.ds(m128(u * 768), 768), :] = jnp.zeros((768, 128), F32)
                m_piece(1, u, 'hi', u0).start(priority=HI)
                return c
            lax.fori_loop(u0, u1, body, 0)

        MARK('p_ma')
        for b0, b1 in ((0, 1), (1, 4), (4, 6), (6, 8)):
            def body(b, c):
                for u in range(7):
                    m_piece(b, u, 'lo' if b0 else 'all').wait()
                    lo = m_piece(b + 4, u, 'lo') if b0 < 4 else q_stream[0](7 * (b - 4) + u)
                    hi = m_piece(b + 2, u, 'hi') if b0 < 6 else q_stream[1](7 * (b - 6) + u)
                    lo.start(priority=LO)
                    hi.start(priority=HI)
                    if b0:
                        m_piece(b, u, 'hi').wait()
                return c
            lax.fori_loop(b0, b1, body, 0)
        for s in smalls:
            s.wait()

        MARK('p_moda')
        k0, v0 = k_stream(0, 0), v_stream(0, 0)
        LW = 28
        ph_q = Phase(q_stream, TB, LW, o_stream)
        ph_o = Phase(o_stream, TB, LW, k0)
        pos = [0]

        def qsteps(n):
            ph_q.run(pos[0], pos[0] + n)
            pos[0] += n

        def qloop(n, k, fn):
            def body(j, c):
                fn(j)
                return c
            ph_q.every(pos[0], n, k, body)
            pos[0] += n * k

        c32 = c_v[...].astype(F32)
        sc = (c32 * jax.nn.sigmoid(c32)).astype(BF16)
        sc16 = jnp.broadcast_to(sc, (16, D))
        w2h = w2_v[...].astype(F32) * 0.5
        w1f = w1_v[...].astype(F32)
        b1f = b1_v[...].astype(F32)
        scf = sc.astype(F32)
        for i in range(NV):
            rows[C_W1 + i:C_W1 + i + 1, :] = w1f[:, (NZ + i) * 128:(NZ + i + 1) * 128] * KS
        rows[C_B1:C_B1 + NV, :] = b1f[NZ:] * KS
        for i in range(ND):
            rows[C_SC + i:C_SC + i + 1, :] = scf[:, i * 128:(i + 1) * 128]

        def mod_a(i):
            c = pl.ds(m128(i * 384), 384)
            mods[:, c] = jnp.dot(sc16, wm_v[:, :, c].reshape(D, 384),
                                 preferred_element_type=F32)[0:8]
        qloop(5, 4, mod_a)

        def mod_b(i):
            c = pl.ds(m128(3 * D + i * 256), 256)
            mods[:, c] = jnp.dot(sc16[:, :D - DB], wm_v[0:DA - 1, :, c].reshape(D - DB, 256),
                                 preferred_element_type=F32)[0:8]
        qloop(5, 3, mod_b)

        x32 = x_v[0].astype(F32)
        h8 = (_layernorm(x32) * (1.0 + mods[:, D:2 * D]) + mods[:, :D]).astype(BF16).astype(F32)
        consts[2:3, :] = jnp.broadcast_to(jnp.mean(x32, axis=1, keepdims=True), (1, 128))
        consts[3:4, :] = jnp.broadcast_to(
            jnp.mean(mods[0:1, 3 * D:4 * D], axis=1, keepdims=True), (1, 128))
        qsteps(4)

        b1row = jnp.concatenate([b1f[i:i + 1, :] for i in range(NF)], axis=1)
        pw = w1f * w2h
        pb = b1row * w2h
        lhs[...] = _stack_rows(_split(pw) + _split(pb), 8)
        sum_w = jnp.sum(pw, axis=1, keepdims=True)
        sum_b = jnp.sum(pb, axis=1, keepdims=True) + b2_v[...].astype(F32).reshape(1, 1)
        consts[0:1, :] = jnp.broadcast_to(sum_w, (1, 128))
        consts[1:2, :] = jnp.broadcast_to(sum_b, (1, 128))
        qsteps(4)

        al = w1f[:, :NZ * 128] * KS
        be = b1row[:, :NZ * 128] * KS
        a3h, a3l = _split(al * al * al)
        a2h, a2l = _split(3.0 * al * al * be)
        a1h, a1l = _split(al * (3.0 * be * be + CS))
        a0h, a0l = _split(be * (be * be + CS))
        at = _stack_rows([a3h, a3h, a3l, a2h, a2h, a2l, a1h, a1h, a1l, a0h] + _split(a0l), 16)
        for b in range(NZ):
            acol[b * 128:(b + 1) * 128, :] = jnp.concatenate(
                [at[:, b * 128:(b + 1) * 128], jnp.zeros((112, 128), F32)], axis=0).T
        qsteps(3)

        MARK('p_prep')

        def prep(i):
            for u in range(3):
                t = 3 * i + u
                cols[pl.ds(m128(t * 128), 128), :] = _col_bcast(rows[pl.ds(t, 1), :])
        qloop(C_N // 3, 5, prep)

        MARK('p_wq')
        qsteps(TB - pos[0])

        MARK('p_qproj')
        scale = DH ** -0.5

        def q_cols(i, q):
            for t in range(2):
                qb[pl.ds(m128(i * 256 + t * 128), 128), :] = _col_bcast(
                    q[0:1, t * 128:(t + 1) * 128])

        def qproj(i0):
            def fn(i, q_prev):
                q_cols(jnp.maximum(i + i0 - 1, 0), q_prev)
                w = pairs(wq_v, [24 * g + i + i0 for g in range(D // 8)]).astype(F32)
                w = jnp.concatenate([w[:, 0:8].reshape(D, 128), w[:, 8:16].reshape(D, 128)],
                                    axis=1)
                return jnp.dot(h8, w, precision=lax.Precision.DEFAULT,
                               preferred_element_type=F32) * scale
            return fn
        q = ph_o.every(0, 20, 5, qproj(0), jnp.zeros((8, 256), F32))
        q = ph_o.every(100, 2, 7, qproj(20), q)
        q = ph_o.every(114, 2, 7, qproj(22), q)
        for c in range(LW, NB):
            k0[0](c).start(priority=LO)
        MARK('p_k0')
        ph = Phase(k0, NB, NB, v0)
        ph.run(0, 1)
        q_cols(23, q)
        abuf[...] = jnp.zeros((DH, 128), F32)
        wo_last[...] = pairs(wo_v, [60 * (H - 1) + p for p in range(60)]).astype(F32).reshape(
            G * ND, 8, 128)
        ph.run(1, NB)

        def proj(h, a, out):
            o = jnp.sum(a, axis=1, keepdims=True)
            outs = [out, None]
            for jj in range(G // 2):
                w = pairs(wo_v, [60 * h + jj * ND + p for p in range(ND)]).astype(F32)
                tiles = _groups(w.reshape(16 * ND, 128))
                for e in range(2):
                    j = 2 * jj + e
                    w = jnp.concatenate(tiles[e * ND:(e + 1) * ND], axis=1)
                    t = o[j * 8:(j + 1) * 8] * w
                    outs[e] = t if outs[e] is None else outs[e] + t
            return outs[0] + outs[1]

        def phase_a(h, slot, out, ph, tps, n1):
            q = qb[pl.ds(pl.multiple_of(h * DH, 64), DH), :]

            def body(i, m):
                for u in range(tps):
                    c = tps * i + u
                    s = _tree_sum(_groups(kbuf[slot, c].astype(F32) * q))
                    s = jnp.broadcast_to(jnp.sum(s, axis=0, keepdims=True), (8, 128))
                    sbuf[c] = s
                    m = jnp.maximum(m, s)
                return m
            n0 = NB // tps
            m = ph.run(0, n0, body, jnp.full((8, 128), -jnp.inf, F32))
            ph.run(n0, n0 + n1)
            m = jnp.max(m, axis=1, keepdims=True)
            out = proj(jnp.maximum(h - 1, 0), abuf[...], out)
            ph.run(n0 + n1, n0 + n1 + 3)
            p = jnp.exp(sbuf[...] - m)
            sbuf[...] = p
            l = _tree_sum([p[c] for c in range(NB)])
            inv_l = 1.0 / jnp.sum(l, axis=1, keepdims=True)
            return inv_l, out

        def pv_tile(slot, c, acc):
            p = sbuf[c]
            return acc + vbuf[slot, c].astype(F32) * jnp.concatenate([p] * G, axis=0)

        def pv_done(acc, inv_l):
            return acc * jnp.concatenate([jnp.broadcast_to(inv_l, (8, 128))] * G, axis=0)

        def head(h, out):
            slot = h & 1
            nslot = 1 - slot
            knext = k_stream(h + 1, nslot)
            ph = Phase(v_stream(h, slot), NB, NB, knext)
            inv_l, out = phase_a(h, slot, out, ph, 2, 1)
            ph.run(20, NB)
            ph = Phase(knext, NB, NB, v_stream(h + 1, nslot))
            acc = ph.run(0, NB, lambda c, acc: pv_tile(slot, c, acc), jnp.zeros((DH, 128), F32))
            abuf[...] = pv_done(acc, inv_l)
            return out

        MARK('main')
        out = lax.fori_loop(0, H - 1, head, jnp.zeros((8, D), F32))

        MARK('qk31')
        hl = H - 1
        sl = hl % 2
        slab9(0).start(priority=LO)
        slab9(1).start(priority=LO)
        for b in GB_ORDER:
            gb_piece(b).start(priority=LO)
        ph = Phase(v_stream(hl, sl), NB, NB, None)
        inv_l, out = phase_a(hl, sl, out, ph, 4, 3)

        MARK('pv31')
        acc = ph.run(14, 28, lambda i, acc: pv_tile(sl, 2 * i - 27, pv_tile(sl, 2 * i - 28, acc)),
                     jnp.zeros((DH, 128), F32))
        ga = mods[:, 2 * D:3 * D]
        xp = x32 + ga * jnp.sum(out, axis=0, keepdims=True)
        gl = ga * inv_l
        acc = ph.run(28, NB - 1, lambda c, acc: pv_tile(sl, c, acc), acc)
        MARK('wlast')
        ph.run(NB - 1, NB)
        MARK('proj31')
        o = jnp.sum(pv_tile(sl, NB - 1, acc), axis=1, keepdims=True)
        outs = [None, None]
        for j in range(G):
            w = jnp.concatenate([wo_last[j * ND + n] for n in range(ND)], axis=1)
            t = o[j * 8:(j + 1) * 8] * w
            outs[j & 1] = t if outs[j & 1] is None else outs[j & 1] + t
        x1 = xp + gl * jnp.sum(outs[0] + outs[1], axis=0, keepdims=True)
        d1 = x1 - _tile(consts[2:3, :], ND)
        mom = _moments(d1)

        MARK('w9')
        slab9(0).wait()
        MARK('ln2')
        mom = _lane_sums(mom)
        macc = None
        for u in range(DB // 8):
            if u == N9:
                MARK('w9b')
                slab9(1).wait()
                MARK('ln2b')
            s = cols[pl.ds(C_SC * 128 + D - DB + u * 8, 8), :]
            t = _tile(s, 2 * ND) * wm_v[DA - 1, pl.ds(u * 8, 8), pl.ds(3 * D, 2 * D)].astype(F32)
            macc = t if macc is None else macc + t
        mod = jnp.sum(macc, axis=0, keepdims=True) + mods[0:1, 3 * D:]
        scale_b = jnp.broadcast_to(1.0 + mod[:, D:], (8, D))
        shift_b = jnp.broadcast_to(mod[:, :D] - _tile(consts[3:4, :], ND), (8, D))
        d2 = _normalize(d1, *mom) * scale_b + shift_b
        hn = _normalize(d2, *_lane_sums(_moments(d2)))

        MARK('mlp')

        def tanh_rows(b, u, hn):
            w1c = cols[pl.ds((C_W1 + b - NZ) * 128 + u * 8, 8), :]
            b1c = cols[pl.ds((C_B1 + b - NZ) * 128 + u * 8, 8), :]
            v = hn * _tile(w1c, ND) + _tile(b1c, ND)
            return jnp.tanh(v * (v * v + CS))

        p2 = hn * hn
        sid = lax.broadcasted_iota(jnp.int32, (8, D), 0)
        phi, plo = _split(jnp.where(sid < 3, p2 * hn, jnp.where(sid < 6, p2, hn)))
        ptop = jnp.where((sid == 1) | (sid == 4) | (sid == 7), plo, phi)
        pbot = jnp.where(sid == 0, hn, jnp.where(sid < 4, 1.0, 0.0))
        pmat = jnp.concatenate([ptop, pbot], axis=0)
        r = None
        nz, nv = 0, NZ
        zs = []
        late = []
        for kind in ORDER:
            if kind == 'V':
                b = nv
                nv += 1
                ts = [tanh_rows(b, u, hn) for u in range(16)]
                t = jnp.concatenate(ts, axis=0)
            elif kind == 'Z':
                zs.append(jnp.dot(acol[len(zs) * 128:(len(zs) + 1) * 128, 0:16], pmat,
                                  precision=lax.Precision.DEFAULT, preferred_element_type=F32))
                continue
            else:
                b = nz
                nz += 1
                t = jnp.tanh(zs[b])
                if kind == 'S':
                    late.append(b)
                    tbuf[len(late)] = t
                    continue
            rb = jnp.dot(lhs[:, b * 128:(b + 1) * 128], t,
                         precision=lax.Precision.DEFAULT, preferred_element_type=F32)
            r = rb if r is None else r + rb
        hl_ = hn + _tile(_tree_sum(_blocks(ts[0])) * 0.0, ND)
        for u in range(16):
            tbuf[0, u * 8:(u + 1) * 8, :] = tanh_rows(NF - 1, u, hl_)

        def gate(accs, bs):
            for b in bs:
                for a in range(DA):
                    s = cols[pl.ds(C_SC * 128 + a * DB + b * 8, 8), :]
                    t = _tile(s, ND) * wm_v[a, pl.ds(b * 8, 8), pl.ds(5 * D, D)].astype(F32)
                    accs[a & 1] = t if accs[a & 1] is None else accs[a & 1] + t
            return accs

        MARK('gbw')
        for b in GB_ORDER[:-2]:
            gb_piece(b).wait()
        MARK('gb')
        for k, b in enumerate([NF - 1] + late):
            r = r + jnp.dot(lhs[:, b * 128:(b + 1) * 128], tbuf[k],
                            precision=lax.Precision.DEFAULT, preferred_element_type=F32)
        gacc = gate([None, None], GB_ORDER[:-2])
        y = (hn[0:1] * (r[0:1] + r[1:2] + _tile(consts[0:1, :], ND))
             + (r[2:3] + r[3:4] + _tile(consts[1:2, :], ND)))
        MARK('gbw3')
        for b in GB_ORDER[-2:]:
            gb_piece(b).wait()
        MARK('gb3')
        gacc = gate(gacc, GB_ORDER[-2:])
        gb = jnp.sum(gacc[0] + gacc[1], axis=0, keepdims=True)
        o_ref[0] = (x1[0:1] + gb * y).astype(o_ref.dtype)
        MARK(None)

    return kernel


@jax.jit
def pallas_adaLN_cond__sliding_block_cached__mixer_token_mlp__decode_kernel(
    A_x: jax.Array,
    A_k_cache: jax.Array,
    A_v_cache: jax.Array,
    A_wq: jax.Array,
    A_wo: jax.Array,
    B_x: jax.Array,
    B_w1: jax.Array,
    B_b1: jax.Array,
    B_w2: jax.Array,
    B_b2: jax.Array,
    c: jax.Array,
    w_mod: jax.Array,
):
    SK = A_k_cache.shape[2]
    W = min(4096, max(256, SK // 4))
    kt = jnp.swapaxes(A_k_cache, 2, 3).reshape(H * DH, SK)
    vt = jnp.swapaxes(A_v_cache, 2, 3).reshape(H * DH, SK)

    vmem = pltpu.VMEM
    dma = pltpu.SemaphoreType.DMA
    return pl.pallas_call(
        _make_kernel(SK, W),
        out_shape=jax.ShapeDtypeStruct(A_x.shape, A_x.dtype),
        in_specs=[pl.BlockSpec(memory_space=pl.ANY)] * 11,
        out_specs=pl.BlockSpec(memory_space=pltpu.VMEM),
        scratch_shapes=[
            vmem((2, W // 128, DH, 128), BF16), vmem((2, W // 128, DH, 128), BF16),
            vmem((TA, TB, 16, 128), BF16), vmem((TA, TB, 16, 128), BF16),
            vmem((DA, DB, 6 * D), BF16),
            vmem((1, 1, D), BF16), vmem((1, D), BF16),
            vmem((1, F), BF16), vmem((NF, 128), BF16), vmem((1, F), BF16),
            vmem((1,), BF16),
            vmem((H * DH, 128), F32), vmem((C_N, 128), F32), vmem((C_N * 128, 128), F32),
            vmem((8, F), F32), vmem((DH, 128), F32), vmem((W // 128, 8, 128), F32),
            vmem((4, 128), F32), vmem((8, 5 * D), F32),
            vmem((NZ * 128, 128), F32),
            vmem((G * ND, 8, 128), F32), vmem((1 + ORDER.count('S'), 128, D), F32),
            dma((2,)), dma((2,)), dma((64,)), dma((64,)), dma((10,)), dma((6,)),
        ],
        compiler_params=pltpu.CompilerParams(
            vmem_limit_bytes=64 * 1024 * 1024,
            disable_bounds_checks=True,
            disable_semaphore_checks=True,
        ),
    )(A_x, kt, vt, _pair_view(A_wq), _pair_view(A_wo), B_w1,
      B_b1.reshape(NF, 128), B_w2.reshape(1, F), B_b2, c, w_mod.reshape(DA, DB, 6 * D))
```

```python
import math

import jax
import jax.numpy as jnp
from jax import lax
import jax.experimental.pallas as pl
import jax.experimental.pallas.tpu as pltpu

F32 = jnp.float32
BF16 = jnp.bfloat16

D = 640
H = 32
DH = 192
F = 1536
EPS = 1e-5
G = DH // 8
ND = D // 128
NF = F // 128

LO, HI = 1, 0

_C0 = math.sqrt(2.0 / math.pi)
_C1 = 0.044715
KS = (_C0 * _C1) ** (1.0 / 3.0)
CS = _C0 / KS

ORDER = 'ZVZVVRZVRVZRVVS'
NZ = ORDER.count('Z')
NV = NF - NZ
C_W1, C_B1, C_SC, C_N = 0, NV, 2 * NV, 2 * NV + ND
assert C_N % 3 == 0

DA, DB = 10, 64
TA, TB = 15, 128


class _Group:
    def __init__(self, copies):
        self.copies = copies

    def start(self, priority):
        for c in self.copies:
            c.start(priority=priority)

    def wait(self):
        for c in self.copies:
            c.wait()


def _pair_view(w):
    r, c = w.shape
    t = w.reshape(r // 8, 8, c // 128, 128).transpose(0, 2, 1, 3)
    return t.reshape(TA, TB, 16, 128)


def _layernorm(x):
    m = jnp.mean(x, axis=-1, keepdims=True)
    xc = x - m
    v = jnp.mean(xc * xc, axis=-1, keepdims=True)
    return xc * lax.rsqrt(v + EPS)


def _moments(d):
    return _tree_sum(_blocks(d)), _tree_sum(_blocks(d * d))


def _lane_sums(xs):
    return [jnp.sum(x, axis=-1, keepdims=True) for x in xs]


def _normalize(d, s1, s2):
    s1 = s1 * (1.0 / D)
    var = jnp.maximum(s2 * (1.0 / D) - s1 * s1, 0.0)
    return (d - s1) * lax.rsqrt(var + EPS)


def _col_bcast(row128):
    return jnp.broadcast_to(row128, (128, 128)).T


def _tile(x, n):
    return jnp.concatenate([x] * n, axis=1)


def _tree_sum(parts):
    while len(parts) > 1:
        nxt = [parts[2 * i] + parts[2 * i + 1] for i in range(len(parts) // 2)]
        if len(parts) % 2:
            nxt.append(parts[-1])
        parts = nxt
    return parts[0]


def _split(a):
    hi = a.astype(BF16).astype(F32)
    return [hi, a - hi]


def _stack_rows(xs, n):
    rid = lax.broadcasted_iota(jnp.int32, (n, xs[0].shape[1]), 0)
    out = jnp.zeros(rid.shape, F32)
    for k, x in enumerate(xs):
        out = jnp.where(rid == k, x, out)
    return out


def _blocks(x):
    return [x[:, j * 128:(j + 1) * 128] for j in range(x.shape[1] // 128)]


def _groups(x):
    return [x[j * 8:(j + 1) * 8, :] for j in range(x.shape[0] // 8)]


def _make_kernel(SK, W):
    LH = 14
    KV_HI = 16
    KV_LO = DH - KV_HI
    W0 = SK - W
    NB = W // 128
    assert NB == 32

    def kernel(x_hbm, k_hbm, v_hbm, wq_hbm, wo_hbm, w1_hbm, b1_hbm, w2_hbm, b2_hbm,
               c_hbm, wm_hbm, o_ref,
               kbuf, vbuf, wq_v, wo_v, wm_v, x_v, c_v, w1_v, b1_v, w2_v, b2_v,
               qb, rows, cols, lhs, abuf, sbuf, consts, mods, acol, wo_last, tbuf,
               klo, khi, vlo, vhi, wsem, ssem):
        cp = pltpu.make_async_copy
        m8 = lambda i: pl.multiple_of(i, 8)
        m128 = lambda i: pl.multiple_of(i, 128)
        MARK = lambda name: None

        def kv_stream(src, buf, lo_sem, hi_sem, h, slot, sem_of):
            def piece(c, r0, n, sem):
                return cp(src.at[pl.ds(m8(h * DH + r0), n), pl.ds(m128(W0 + c * 128), 128)],
                          buf.at[slot, c, pl.ds(r0, n), :], sem.at[sem_of(c)])
            return (lambda c: piece(c, 0, KV_LO, lo_sem),
                    lambda c: piece(c, KV_LO, KV_HI, hi_sem))

        k_stream = lambda h, slot: kv_stream(k_hbm, kbuf, klo, khi, h, slot, lambda c: slot)
        v_stream = lambda h, slot: kv_stream(v_hbm, vbuf, vlo, vhi, h, slot,
                                             lambda c: slot * NB + c)

        def w_piece(src, dst, a0, na, b, c0, n, sem):
            idx = (pl.ds(a0, na), pl.ds(m8(b * 8), 8), pl.ds(m128(c0), n))
            return cp(src.at[idx], dst.at[idx], sem)

        def m_piece(b, u, part, kind=None):
            kind = u if kind is None else kind
            na, c0, n = (DA, u * 384, 384) if kind < 5 else (DA - 1, (u - 2) * D, D)
            a0, na = {'all': (0, na), 'lo': (0, na - 1), 'hi': (na - 1, 1)}[part]
            return w_piece(wm_hbm, wm_v, a0, na, b, c0, n, wsem.at[5 if part == 'hi' else 0])

        def pair_stream(src, dst, s):
            def piece(i, a0, na, r0, nr, sem):
                idx = (pl.ds(a0, na), i, pl.ds(r0, nr))
                return cp(src.at[idx], dst.at[idx], sem)
            return (lambda i: _Group([piece(i, 0, TA, 0, 8, wsem.at[s]),
                                      piece(i, 0, TA - 3, 8, 8, wsem.at[s])]),
                    lambda i: piece(i, TA - 3, 3, 8, 8, wsem.at[s + 1]))
        q_stream = pair_stream(wq_hbm, wq_v, 1)
        o_stream = pair_stream(wo_hbm, wo_v, 3)

        N9 = 6

        def slab9(k):
            r = pl.ds(8 * N9, DB - 8 * N9) if k else pl.ds(0, 8 * N9)
            idx = (DA - 1, r, pl.ds(3 * D, 2 * D))
            return cp(wm_hbm.at[idx], wm_v.at[idx], wsem.at[9 if k else 6])

        NG1 = 6
        gb_piece = lambda b: w_piece(wm_hbm, wm_v, 0, DA, b, 5 * D, D,
                                     wsem.at[7 if b < NG1 else 8])

        class Phase:
            def __init__(self, cur, n, ll, nxt):
                self.cur, self.n, self.nxt = cur, n, nxt
                self.ahead = (ll, LH)
                self.edges = {n - ll, n - LH}

            def stepper(self, a, b):
                starts = []
                assert not any(a < e < b for e in self.edges), (a, b)
                for k, prio in ((0, LO), (1, HI)):
                    ahead = self.ahead[k]
                    if b <= self.n - ahead:
                        starts.append((self.cur[k], ahead, prio))
                    elif self.nxt is not None:
                        starts.append((self.nxt[k], ahead - self.n, prio))

                def step(i):
                    self.cur[0](i).wait()
                    for piece, off, prio in starts:
                        piece(i + off).start(priority=prio)
                    self.cur[1](i).wait()
                return step

            def run(self, a, b, fn=None, init=0):
                cuts = sorted({a, b} | {e for e in self.edges if a < e < b})
                for lo, hi in zip(cuts[:-1], cuts[1:]):
                    step = self.stepper(lo, hi)

                    def body(i, c):
                        step(i)
                        return c if fn is None else fn(i, c)
                    init = body(lo, init) if hi - lo == 1 else lax.fori_loop(lo, hi, body, init)
                return init

            def every(self, a, n, k, fn, init=0):
                step = self.stepper(a, a + n * k)

                def body(j, c):
                    step(a + k * j)
                    c = fn(j, c)

                    def rest(u, z):
                        step(a + k * j + u)
                        return z
                    lax.fori_loop(1, k, rest, 0)
                    return c
                return lax.fori_loop(0, n, body, init)

        def pairs(ref, ps):
            return jnp.stack([ref[p >> 7, p & 127] for p in ps])

        MARK('p_issue')
        for u in range(7):
            m_piece(0, u, 'all').start(priority=LO)
        smalls = [cp(s, d, ssem.at[n]) for n, (s, d) in enumerate(
            [(c_hbm, c_v), (x_hbm, x_v), (w1_hbm, w1_v), (b1_hbm, b1_v), (w2_hbm, w2_v),
             (b2_hbm, b2_v)])]
        for s in smalls:
            s.start(priority=HI)

        for b in range(1, 4):
            for u in range(7):
                m_piece(b, u, 'lo').start(priority=LO)
        for u0, u1 in ((0, 5), (5, 7)):
            def body(u, c):
                qb[pl.ds(m128(u * 768), 768), :] = jnp.zeros((768, 128), F32)
                m_piece(1, u, 'hi', u0).start(priority=HI)
                return c
            lax.fori_loop(u0, u1, body, 0)

        MARK('p_ma')
        for b0, b1 in ((0, 1), (1, 4), (4, 6), (6, 8)):
            def body(b, c):
                for u in range(7):
                    m_piece(b, u, 'lo' if b0 else 'all').wait()
                    lo = m_piece(b + 4, u, 'lo') if b0 < 4 else q_stream[0](7 * (b - 4) + u)
                    hi = m_piece(b + 2, u, 'hi') if b0 < 6 else q_stream[1](7 * (b - 6) + u)
                    lo.start(priority=LO)
                    hi.start(priority=HI)
                    if b0:
                        m_piece(b, u, 'hi').wait()
                return c
            lax.fori_loop(b0, b1, body, 0)
        for s in smalls:
            s.wait()

        MARK('p_moda')
        k0, v0 = k_stream(0, 0), v_stream(0, 0)
        LW = 28
        ph_q = Phase(q_stream, TB, LW, o_stream)
        ph_o = Phase(o_stream, TB, LW, k0)
        pos = [0]

        def qsteps(n):
            ph_q.run(pos[0], pos[0] + n)
            pos[0] += n

        def qloop(n, k, fn):
            def body(j, c):
                fn(j)
                return c
            ph_q.every(pos[0], n, k, body)
            pos[0] += n * k

        c32 = c_v[...].astype(F32)
        sc = (c32 * jax.nn.sigmoid(c32)).astype(BF16)
        sc16 = jnp.broadcast_to(sc, (16, D))
        w2h = w2_v[...].astype(F32) * 0.5
        w1f = w1_v[...].astype(F32)
        b1f = b1_v[...].astype(F32)
        scf = sc.astype(F32)
        for i in range(NV):
            rows[C_W1 + i:C_W1 + i + 1, :] = w1f[:, (NZ + i) * 128:(NZ + i + 1) * 128] * KS
        rows[C_B1:C_B1 + NV, :] = b1f[NZ:] * KS
        for i in range(ND):
            rows[C_SC + i:C_SC + i + 1, :] = scf[:, i * 128:(i + 1) * 128]

        def mod_a(i):
            c = pl.ds(m128(i * 384), 384)
            mods[:, c] = jnp.dot(sc16, wm_v[:, :, c].reshape(D, 384),
                                 preferred_element_type=F32)[0:8]
        qloop(5, 4, mod_a)

        def mod_b(i):
            c = pl.ds(m128(3 * D + i * 256), 256)
            mods[:, c] = jnp.dot(sc16[:, :D - DB], wm_v[0:DA - 1, :, c].reshape(D - DB, 256),
                                 preferred_element_type=F32)[0:8]
        qloop(5, 3, mod_b)

        x32 = x_v[0].astype(F32)
        h8 = (_layernorm(x32) * (1.0 + mods[:, D:2 * D]) + mods[:, :D]).astype(BF16).astype(F32)
        consts[2:3, :] = jnp.broadcast_to(jnp.mean(x32, axis=1, keepdims=True), (1, 128))
        consts[3:4, :] = jnp.broadcast_to(
            jnp.mean(mods[0:1, 3 * D:4 * D], axis=1, keepdims=True), (1, 128))
        qsteps(4)

        b1row = jnp.concatenate([b1f[i:i + 1, :] for i in range(NF)], axis=1)
        pw = w1f * w2h
        pb = b1row * w2h
        lhs[...] = _stack_rows(_split(pw) + _split(pb), 8)
        sum_w = jnp.sum(pw, axis=1, keepdims=True)
        sum_b = jnp.sum(pb, axis=1, keepdims=True) + b2_v[...].astype(F32).reshape(1, 1)
        consts[0:1, :] = jnp.broadcast_to(sum_w, (1, 128))
        consts[1:2, :] = jnp.broadcast_to(sum_b, (1, 128))
        qsteps(4)

        al = w1f[:, :NZ * 128] * KS
        be = b1row[:, :NZ * 128] * KS
        a3h, a3l = _split(al * al * al)
        a2h, a2l = _split(3.0 * al * al * be)
        a1h, a1l = _split(al * (3.0 * be * be + CS))
        a0h, a0l = _split(be * (be * be + CS))
        at = _stack_rows([a3h, a3h, a3l, a2h, a2h, a2l, a1h, a1h, a1l, a0h] + _split(a0l), 16)
        for b in range(NZ):
            acol[b * 128:(b + 1) * 128, :] = jnp.concatenate(
                [at[:, b * 128:(b + 1) * 128], jnp.zeros((112, 128), F32)], axis=0).T
        qsteps(3)

        MARK('p_prep')

        def prep(i):
            for u in range(3):
                t = 3 * i + u
                cols[pl.ds(m128(t * 128), 128), :] = _col_bcast(rows[pl.ds(t, 1), :])
        qloop(C_N // 3, 5, prep)

        MARK('p_wq')
        qsteps(TB - pos[0])

        MARK('p_qproj')
        scale = DH ** -0.5

        def q_cols(i, q):
            for t in range(2):
                qb[pl.ds(m128(i * 256 + t * 128), 128), :] = _col_bcast(
                    q[0:1, t * 128:(t + 1) * 128])

        def qproj(i0):
            def fn(i, q_prev):
                q_cols(jnp.maximum(i + i0 - 1, 0), q_prev)
                w = pairs(wq_v, [24 * g + i + i0 for g in range(D // 8)]).astype(F32)
                w = jnp.concatenate([w[:, 0:8].reshape(D, 128), w[:, 8:16].reshape(D, 128)],
                                    axis=1)
                return jnp.dot(h8, w, precision=lax.Precision.DEFAULT,
                               preferred_element_type=F32) * scale
            return fn
        q = ph_o.every(0, 20, 5, qproj(0), jnp.zeros((8, 256), F32))
        q = ph_o.every(100, 2, 7, qproj(20), q)
        q = ph_o.every(114, 2, 7, qproj(22), q)
        for c in range(LW, NB):
            k0[0](c).start(priority=LO)
        MARK('p_k0')
        ph = Phase(k0, NB, NB, v0)
        ph.run(0, 1)
        q_cols(23, q)
        abuf[...] = jnp.zeros((DH, 128), F32)
        wo_last[...] = pairs(wo_v, [60 * (H - 1) + p for p in range(60)]).astype(F32).reshape(
            G * ND, 8, 128)
        ph.run(1, NB)

        def proj(h, a, out):
            o = jnp.sum(a, axis=1, keepdims=True)
            outs = [out, None]
            for jj in range(G // 2):
                w = pairs(wo_v, [60 * h + jj * ND + p for p in range(ND)]).astype(F32)
                tiles = _groups(w.reshape(16 * ND, 128))
                for e in range(2):
                    j = 2 * jj + e
                    w = jnp.concatenate(tiles[e * ND:(e + 1) * ND], axis=1)
                    t = o[j * 8:(j + 1) * 8] * w
                    outs[e] = t if outs[e] is None else outs[e] + t
            return outs[0] + outs[1]

        def phase_a(h, slot, out, ph, tps, n1):
            q = qb[pl.ds(pl.multiple_of(h * DH, 64), DH), :]

            def body(i, m):
                for u in range(tps):
                    c = tps * i + u
                    s = _tree_sum(_groups(kbuf[slot, c].astype(F32) * q))
                    s = jnp.broadcast_to(jnp.sum(s, axis=0, keepdims=True), (8, 128))
                    sbuf[c] = s
                    m = jnp.maximum(m, s)
                return m
            n0 = NB // tps
            m = ph.run(0, n0, body, jnp.full((8, 128), -jnp.inf, F32))
            ph.run(n0, n0 + n1)
            m = jnp.max(m, axis=1, keepdims=True)
            out = proj(jnp.maximum(h - 1, 0), abuf[...], out)
            ph.run(n0 + n1, n0 + n1 + 3)
            p = jnp.exp(sbuf[...] - m)
            sbuf[...] = p
            l = _tree_sum([p[c] for c in range(NB)])
            inv_l = 1.0 / jnp.sum(l, axis=1, keepdims=True)
            return inv_l, out

        def pv_tile(slot, c, acc):
            p = sbuf[c]
            return acc + vbuf[slot, c].astype(F32) * jnp.concatenate([p] * G, axis=0)

        def pv_done(acc, inv_l):
            return acc * jnp.concatenate([jnp.broadcast_to(inv_l, (8, 128))] * G, axis=0)

        def head(h, out):
            slot = h & 1
            nslot = 1 - slot
            knext = k_stream(h + 1, nslot)
            ph = Phase(v_stream(h, slot), NB, NB, knext)
            inv_l, out = phase_a(h, slot, out, ph, 2, 1)
            ph.run(20, NB)
            ph = Phase(knext, NB, NB, v_stream(h + 1, nslot))
            acc = ph.run(0, NB, lambda c, acc: pv_tile(slot, c, acc), jnp.zeros((DH, 128), F32))
            abuf[...] = pv_done(acc, inv_l)
            return out

        MARK('main')
        out = lax.fori_loop(0, H - 1, head, jnp.zeros((8, D), F32))

        MARK('qk31')
        hl = H - 1
        sl = hl % 2
        slab9(0).start(priority=LO)
        slab9(1).start(priority=LO)
        for b in range(8):
            gb_piece(b).start(priority=LO)
        ph = Phase(v_stream(hl, sl), NB, NB, None)
        inv_l, out = phase_a(hl, sl, out, ph, 4, 3)

        MARK('pv31')
        acc = ph.run(14, 28, lambda i, acc: pv_tile(sl, 2 * i - 27, pv_tile(sl, 2 * i - 28, acc)),
                     jnp.zeros((DH, 128), F32))
        ga = mods[:, 2 * D:3 * D]
        xp = x32 + ga * jnp.sum(out, axis=0, keepdims=True)
        gl = ga * inv_l
        acc = ph.run(28, NB - 1, lambda c, acc: pv_tile(sl, c, acc), acc)
        MARK('wlast')
        ph.run(NB - 1, NB)
        MARK('proj31')
        o = jnp.sum(pv_tile(sl, NB - 1, acc), axis=1, keepdims=True)
        outs = [None, None]
        for j in range(G):
            w = jnp.concatenate([wo_last[j * ND + n] for n in range(ND)], axis=1)
            t = o[j * 8:(j + 1) * 8] * w
            outs[j & 1] = t if outs[j & 1] is None else outs[j & 1] + t
        x1 = xp + gl * jnp.sum(outs[0] + outs[1], axis=0, keepdims=True)
        d1 = x1 - _tile(consts[2:3, :], ND)
        mom = _moments(d1)

        MARK('w9')
        slab9(0).wait()
        MARK('ln2')
        mom = _lane_sums(mom)
        macc = None
        for u in range(DB // 8):
            if u == N9:
                MARK('w9b')
                slab9(1).wait()
                MARK('ln2b')
            s = cols[pl.ds(C_SC * 128 + D - DB + u * 8, 8), :]
            t = _tile(s, 2 * ND) * wm_v[DA - 1, pl.ds(u * 8, 8), pl.ds(3 * D, 2 * D)].astype(F32)
            macc = t if macc is None else macc + t
        mod = jnp.sum(macc, axis=0, keepdims=True) + mods[0:1, 3 * D:]
        scale_b = jnp.broadcast_to(1.0 + mod[:, D:], (8, D))
        shift_b = jnp.broadcast_to(mod[:, :D] - _tile(consts[3:4, :], ND), (8, D))
        d2 = _normalize(d1, *mom) * scale_b + shift_b
        hn = _normalize(d2, *_lane_sums(_moments(d2)))

        MARK('mlp')

        def tanh_rows(b, u, hn):
            w1c = cols[pl.ds((C_W1 + b - NZ) * 128 + u * 8, 8), :]
            b1c = cols[pl.ds((C_B1 + b - NZ) * 128 + u * 8, 8), :]
            v = hn * _tile(w1c, ND) + _tile(b1c, ND)
            return jnp.tanh(v * (v * v + CS))

        p2 = hn * hn
        sid = lax.broadcasted_iota(jnp.int32, (8, D), 0)
        phi, plo = _split(jnp.where(sid < 3, p2 * hn, jnp.where(sid < 6, p2, hn)))
        ptop = jnp.where((sid == 1) | (sid == 4) | (sid == 7), plo, phi)
        pbot = jnp.where(sid == 0, hn, jnp.where(sid < 4, 1.0, 0.0))
        pmat = jnp.concatenate([ptop, pbot], axis=0)
        r = None
        nz, nv = 0, NZ
        zs = []
        late = []
        for kind in ORDER:
            if kind == 'V':
                b = nv
                nv += 1
                ts = [tanh_rows(b, u, hn) for u in range(16)]
                t = jnp.concatenate(ts, axis=0)
            elif kind == 'Z':
                zs.append(jnp.dot(acol[len(zs) * 128:(len(zs) + 1) * 128, 0:16], pmat,
                                  precision=lax.Precision.DEFAULT, preferred_element_type=F32))
                continue
            else:
                b = nz
                nz += 1
                t = jnp.tanh(zs[b])
                if kind == 'S':
                    late.append(b)
                    tbuf[len(late)] = t
                    continue
            rb = jnp.dot(lhs[:, b * 128:(b + 1) * 128], t,
                         precision=lax.Precision.DEFAULT, preferred_element_type=F32)
            r = rb if r is None else r + rb
        hl_ = hn + _tile(_tree_sum(_blocks(ts[0])) * 0.0, ND)
        for u in range(16):
            tbuf[0, u * 8:(u + 1) * 8, :] = tanh_rows(NF - 1, u, hl_)

        def gate(accs, bs):
            for b in bs:
                for a in range(DA):
                    s = cols[pl.ds(C_SC * 128 + a * DB + b * 8, 8), :]
                    t = _tile(s, ND) * wm_v[a, pl.ds(b * 8, 8), pl.ds(5 * D, D)].astype(F32)
                    accs[a & 1] = t if accs[a & 1] is None else accs[a & 1] + t
            return accs

        MARK('gbw')
        for b in range(NG1):
            gb_piece(b).wait()
        MARK('gb')
        for k, b in enumerate([NF - 1] + late):
            r = r + jnp.dot(lhs[:, b * 128:(b + 1) * 128], tbuf[k],
                            precision=lax.Precision.DEFAULT, preferred_element_type=F32)
        gacc = gate([None, None], range(NG1))
        y = (hn[0:1] * (r[0:1] + r[1:2] + _tile(consts[0:1, :], ND))
             + (r[2:3] + r[3:4] + _tile(consts[1:2, :], ND)))
        MARK('gbw3')
        for b in range(NG1, 8):
            gb_piece(b).wait()
        MARK('gb3')
        gacc = gate(gacc, range(NG1, 8))
        gb = jnp.sum(gacc[0] + gacc[1], axis=0, keepdims=True)
        o_ref[0] = (x1[0:1] + gb * y).astype(o_ref.dtype)
        MARK(None)

    return kernel


@jax.jit
def pallas_adaLN_cond__sliding_block_cached__mixer_token_mlp__decode_kernel(
    A_x: jax.Array,
    A_k_cache: jax.Array,
    A_v_cache: jax.Array,
    A_wq: jax.Array,
    A_wo: jax.Array,
    B_x: jax.Array,
    B_w1: jax.Array,
    B_b1: jax.Array,
    B_w2: jax.Array,
    B_b2: jax.Array,
    c: jax.Array,
    w_mod: jax.Array,
):
    SK = A_k_cache.shape[2]
    W = min(4096, max(256, SK // 4))
    kt = jnp.swapaxes(A_k_cache, 2, 3).reshape(H * DH, SK)
    vt = jnp.swapaxes(A_v_cache, 2, 3).reshape(H * DH, SK)

    vmem = pltpu.VMEM
    dma = pltpu.SemaphoreType.DMA
    return pl.pallas_call(
        _make_kernel(SK, W),
        out_shape=jax.ShapeDtypeStruct(A_x.shape, A_x.dtype),
        in_specs=[pl.BlockSpec(memory_space=pl.ANY)] * 11,
        out_specs=pl.BlockSpec(memory_space=pltpu.VMEM),
        scratch_shapes=[
            vmem((2, W // 128, DH, 128), BF16), vmem((2, W // 128, DH, 128), BF16),
            vmem((TA, TB, 16, 128), BF16), vmem((TA, TB, 16, 128), BF16),
            vmem((DA, DB, 6 * D), BF16),
            vmem((1, 1, D), BF16), vmem((1, D), BF16),
            vmem((1, F), BF16), vmem((NF, 128), BF16), vmem((1, F), BF16),
            vmem((1,), BF16),
            vmem((H * DH, 128), F32), vmem((C_N, 128), F32), vmem((C_N * 128, 128), F32),
            vmem((8, F), F32), vmem((DH, 128), F32), vmem((W // 128, 8, 128), F32),
            vmem((4, 128), F32), vmem((8, 5 * D), F32),
            vmem((NZ * 128, 128), F32),
            vmem((G * ND, 8, 128), F32), vmem((1 + ORDER.count('S'), 128, D), F32),
            dma((2,)), dma((2,)), dma((64,)), dma((64,)), dma((10,)), dma((6,)),
        ],
        compiler_params=pltpu.CompilerParams(
            vmem_limit_bytes=64 * 1024 * 1024,
            disable_bounds_checks=True,
            disable_semaphore_checks=True,
        ),
    )(A_x, kt, vt, _pair_view(A_wq), _pair_view(A_wo), B_w1,
      B_b1.reshape(NF, 128), B_w2.reshape(1, F), B_b2, c, w_mod.reshape(DA, DB, 6 * D))
```

```python
import math

import jax
import jax.numpy as jnp
from jax import lax
import jax.experimental.pallas as pl
import jax.experimental.pallas.tpu as pltpu

F32 = jnp.float32
BF16 = jnp.bfloat16

D = 640
H = 32
DH = 192
F = 1536
EPS = 1e-5
G = DH // 8
ND = D // 128
NF = F // 128

LO, HI = 1, 0

_C0 = math.sqrt(2.0 / math.pi)
_C1 = 0.044715
KS = (_C0 * _C1) ** (1.0 / 3.0)
CS = _C0 / KS

ORDER = 'ZVZVVRZVRVZRVVS'
NZ = ORDER.count('Z')
NV = NF - NZ
C_W1, C_B1, C_SC, C_N = 0, NV, 2 * NV, 2 * NV + ND
assert C_N % 3 == 0

DA, DB = 10, 64
TA, TB = 15, 128


class _Group:
    def __init__(self, copies):
        self.copies = copies

    def start(self, priority):
        for c in self.copies:
            c.start(priority=priority)

    def wait(self):
        for c in self.copies:
            c.wait()


def _pair_view(w):
    r, c = w.shape
    t = w.reshape(r // 8, 8, c // 128, 128).transpose(0, 2, 1, 3)
    return t.reshape(TA, TB, 16, 128)


def _layernorm(x):
    m = jnp.mean(x, axis=-1, keepdims=True)
    xc = x - m
    v = jnp.mean(xc * xc, axis=-1, keepdims=True)
    return xc * lax.rsqrt(v + EPS)


def _moments(d):
    low = lax.broadcasted_iota(jnp.int32, d.shape, 0) < 4
    return _tree_sum(_blocks(d * jnp.where(low, 1.0, d)))


def _lane_sum(x):
    return jnp.broadcast_to(jnp.sum(x, axis=-1, keepdims=True), x.shape)


def _stats(s):
    s = s * (1.0 / D)
    m1, m2 = jnp.broadcast_to(s[0:1], s.shape), jnp.broadcast_to(s[4:5], s.shape)
    return _tile(m1, ND), _tile(lax.rsqrt(jnp.maximum(m2 - m1 * m1, 0.0) + EPS), ND)


def _col_bcast(row128):
    return jnp.broadcast_to(row128, (128, 128)).T


def _tile(x, n):
    return jnp.concatenate([x] * n, axis=1)


def _tree_sum(parts):
    while len(parts) > 1:
        nxt = [parts[2 * i] + parts[2 * i + 1] for i in range(len(parts) // 2)]
        if len(parts) % 2:
            nxt.append(parts[-1])
        parts = nxt
    return parts[0]


def _split(a):
    hi = a.astype(BF16).astype(F32)
    return [hi, a - hi]


def _stack_rows(xs, n):
    rid = lax.broadcasted_iota(jnp.int32, (n, xs[0].shape[1]), 0)
    out = jnp.zeros(rid.shape, F32)
    for k, x in enumerate(xs):
        out = jnp.where(rid == k, x, out)
    return out


def _blocks(x):
    return [x[:, j * 128:(j + 1) * 128] for j in range(x.shape[1] // 128)]


def _groups(x):
    return [x[j * 8:(j + 1) * 8, :] for j in range(x.shape[0] // 8)]


def _make_kernel(SK, W):
    LH = 14
    KV_HI = 16
    KV_LO = DH - KV_HI
    W0 = SK - W
    NB = W // 128
    assert NB == 32

    def kernel(x_hbm, k_hbm, v_hbm, wq_hbm, wo_hbm, w1_hbm, b1_hbm, w2_hbm, b2_hbm,
               c_hbm, wm_hbm, o_ref,
               kbuf, vbuf, wq_v, wo_v, wm_v, x_v, c_v, w1_v, b1_v, w2_v, b2_v,
               qb, rows, cols, lhs, abuf, sbuf, consts, mods, acol, wo_last, tbuf,
               klo, khi, vlo, vhi, wsem, ssem):
        cp = pltpu.make_async_copy
        m8 = lambda i: pl.multiple_of(i, 8)
        m128 = lambda i: pl.multiple_of(i, 128)
        MARK = lambda name: None

        def kv_stream(src, buf, lo_sem, hi_sem, h, slot, sem_of):
            def piece(c, r0, n, sem):
                return cp(src.at[pl.ds(m8(h * DH + r0), n), pl.ds(m128(W0 + c * 128), 128)],
                          buf.at[slot, c, pl.ds(r0, n), :], sem.at[sem_of(c)])
            return (lambda c: piece(c, 0, KV_LO, lo_sem),
                    lambda c: piece(c, KV_LO, KV_HI, hi_sem))

        k_stream = lambda h, slot: kv_stream(k_hbm, kbuf, klo, khi, h, slot, lambda c: slot)
        v_stream = lambda h, slot: kv_stream(v_hbm, vbuf, vlo, vhi, h, slot,
                                             lambda c: slot * NB + c)

        def w_piece(src, dst, a0, na, b, c0, n, sem):
            idx = (pl.ds(a0, na), pl.ds(m8(b * 8), 8), pl.ds(m128(c0), n))
            return cp(src.at[idx], dst.at[idx], sem)

        def m_piece(b, u, part, kind=None):
            kind = u if kind is None else kind
            na, c0, n = (DA, u * 384, 384) if kind < 5 else (DA - 1, (u - 2) * D, D)
            a0, na = {'all': (0, na), 'lo': (0, na - 1), 'hi': (na - 1, 1)}[part]
            return w_piece(wm_hbm, wm_v, a0, na, b, c0, n, wsem.at[5 if part == 'hi' else 0])

        def pair_stream(src, dst, s):
            def piece(i, a0, na, r0, nr, sem):
                idx = (pl.ds(a0, na), i, pl.ds(r0, nr))
                return cp(src.at[idx], dst.at[idx], sem)
            return (lambda i: _Group([piece(i, 0, TA, 0, 8, wsem.at[s]),
                                      piece(i, 0, TA - 3, 8, 8, wsem.at[s])]),
                    lambda i: piece(i, TA - 3, 3, 8, 8, wsem.at[s + 1]))
        q_stream = pair_stream(wq_hbm, wq_v, 1)
        o_stream = pair_stream(wo_hbm, wo_v, 3)

        N9 = 6

        def slab9(k):
            r = pl.ds(8 * N9, DB - 8 * N9) if k else pl.ds(0, 8 * N9)
            idx = (DA - 1, r, pl.ds(3 * D, 2 * D))
            return cp(wm_hbm.at[idx], wm_v.at[idx], wsem.at[9 if k else 6])

        NG1 = 6
        gb_piece = lambda b: w_piece(wm_hbm, wm_v, 0, DA, b, 5 * D, D,
                                     wsem.at[7 if b < NG1 else 8])

        class Phase:
            def __init__(self, cur, n, ll, nxt):
                self.cur, self.n, self.nxt = cur, n, nxt
                self.ahead = (ll, LH)
                self.edges = {n - ll, n - LH}

            def stepper(self, a, b):
                starts = []
                assert not any(a < e < b for e in self.edges), (a, b)
                for k, prio in ((0, LO), (1, HI)):
                    ahead = self.ahead[k]
                    if b <= self.n - ahead:
                        starts.append((self.cur[k], ahead, prio))
                    elif self.nxt is not None:
                        starts.append((self.nxt[k], ahead - self.n, prio))

                def step(i):
                    self.cur[0](i).wait()
                    for piece, off, prio in starts:
                        piece(i + off).start(priority=prio)
                    self.cur[1](i).wait()
                return step

            def run(self, a, b, fn=None, init=0):
                cuts = sorted({a, b} | {e for e in self.edges if a < e < b})
                for lo, hi in zip(cuts[:-1], cuts[1:]):
                    step = self.stepper(lo, hi)

                    def body(i, c):
                        step(i)
                        return c if fn is None else fn(i, c)
                    init = body(lo, init) if hi - lo == 1 else lax.fori_loop(lo, hi, body, init)
                return init

            def every(self, a, n, k, fn, init=0):
                step = self.stepper(a, a + n * k)

                def body(j, c):
                    step(a + k * j)
                    c = fn(j, c)

                    def rest(u, z):
                        step(a + k * j + u)
                        return z
                    lax.fori_loop(1, k, rest, 0)
                    return c
                return lax.fori_loop(0, n, body, init)

        def pairs(ref, ps):
            return jnp.stack([ref[p >> 7, p & 127] for p in ps])

        MARK('p_issue')
        for u in range(7):
            m_piece(0, u, 'all').start(priority=LO)
        smalls = [cp(s, d, ssem.at[n]) for n, (s, d) in enumerate(
            [(c_hbm, c_v), (x_hbm, x_v), (w1_hbm, w1_v), (b1_hbm, b1_v), (w2_hbm, w2_v),
             (b2_hbm, b2_v)])]
        for s in smalls:
            s.start(priority=HI)

        for b in range(1, 4):
            for u in range(7):
                m_piece(b, u, 'lo').start(priority=LO)
        for u0, u1 in ((0, 5), (5, 7)):
            def body(u, c):
                qb[pl.ds(m128(u * 768), 768), :] = jnp.zeros((768, 128), F32)
                m_piece(1, u, 'hi', u0).start(priority=HI)
                return c
            lax.fori_loop(u0, u1, body, 0)

        MARK('p_ma')
        for b0, b1 in ((0, 1), (1, 4), (4, 6), (6, 8)):
            def body(b, c):
                for u in range(7):
                    m_piece(b, u, 'lo' if b0 else 'all').wait()
                    lo = m_piece(b + 4, u, 'lo') if b0 < 4 else q_stream[0](7 * (b - 4) + u)
                    hi = m_piece(b + 2, u, 'hi') if b0 < 6 else q_stream[1](7 * (b - 6) + u)
                    lo.start(priority=LO)
                    hi.start(priority=HI)
                    if b0:
                        m_piece(b, u, 'hi').wait()
                return c
            lax.fori_loop(b0, b1, body, 0)
        for s in smalls:
            s.wait()

        MARK('p_moda')
        k0, v0 = k_stream(0, 0), v_stream(0, 0)
        LW = 28
        ph_q = Phase(q_stream, TB, LW, o_stream)
        ph_o = Phase(o_stream, TB, LW, k0)
        pos = [0]

        def qsteps(n):
            ph_q.run(pos[0], pos[0] + n)
            pos[0] += n

        def qloop(n, k, fn):
            def body(j, c):
                fn(j)
                return c
            ph_q.every(pos[0], n, k, body)
            pos[0] += n * k

        c32 = c_v[...].astype(F32)
        sc = (c32 * jax.nn.sigmoid(c32)).astype(BF16)
        sc16 = jnp.broadcast_to(sc, (16, D))
        w2h = w2_v[...].astype(F32) * 0.5
        w1f = w1_v[...].astype(F32)
        b1f = b1_v[...].astype(F32)
        scf = sc.astype(F32)
        for i in range(NV):
            rows[C_W1 + i:C_W1 + i + 1, :] = w1f[:, (NZ + i) * 128:(NZ + i + 1) * 128] * KS
        rows[C_B1:C_B1 + NV, :] = b1f[NZ:] * KS
        for i in range(ND):
            rows[C_SC + i:C_SC + i + 1, :] = scf[:, i * 128:(i + 1) * 128]

        def mod_a(i):
            c = pl.ds(m128(i * 384), 384)
            mods[:, c] = jnp.dot(sc16, wm_v[:, :, c].reshape(D, 384),
                                 preferred_element_type=F32)[0:8]
        qloop(5, 4, mod_a)

        def mod_b(i):
            c = pl.ds(m128(3 * D + i * 256), 256)
            mods[:, c] = jnp.dot(sc16[:, :D - DB], wm_v[0:DA - 1, :, c].reshape(D - DB, 256),
                                 preferred_element_type=F32)[0:8]
        qloop(5, 3, mod_b)

        x32 = x_v[0].astype(F32)
        h8 = (_layernorm(x32) * (1.0 + mods[:, D:2 * D]) + mods[:, :D]).astype(BF16).astype(F32)
        consts[2:3, :] = jnp.broadcast_to(jnp.mean(x32, axis=1, keepdims=True), (1, 128))
        sb = mods[:, 3 * D:4 * D]
        base = jnp.concatenate([sb - jnp.mean(sb, axis=1, keepdims=True), 1.0 + mods[:, 4 * D:]],
                               axis=1)
        mods[:, 3 * D:] = jnp.where(lax.broadcasted_iota(jnp.int32, base.shape, 0) == 0, base, 0.0)
        qsteps(4)

        b1row = jnp.concatenate([b1f[i:i + 1, :] for i in range(NF)], axis=1)
        pw = w1f * w2h
        pb = b1row * w2h
        lhs[...] = _stack_rows(_split(pw) + _split(pb), 8)
        sum_w = jnp.sum(pw, axis=1, keepdims=True)
        sum_b = jnp.sum(pb, axis=1, keepdims=True) + b2_v[...].astype(F32).reshape(1, 1)
        consts[0:1, :] = jnp.broadcast_to(sum_w, (1, 128))
        consts[1:2, :] = jnp.broadcast_to(sum_b, (1, 128))
        qsteps(4)

        al = w1f[:, :NZ * 128] * KS
        be = b1row[:, :NZ * 128] * KS
        a3h, a3l = _split(al * al * al)
        a2h, a2l = _split(3.0 * al * al * be)
        a1h, a1l = _split(al * (3.0 * be * be + CS))
        a0h, a0l = _split(be * (be * be + CS))
        at = _stack_rows([a3h, a3h, a3l, a2h, a2h, a2l, a1h, a1h, a1l, a0h] + _split(a0l), 16)
        for b in range(NZ):
            acol[b * 128:(b + 1) * 128, :] = jnp.concatenate(
                [at[:, b * 128:(b + 1) * 128], jnp.zeros((112, 128), F32)], axis=0).T
        qsteps(3)

        MARK('p_prep')

        def prep(i):
            for u in range(3):
                t = 3 * i + u
                cols[pl.ds(m128(t * 128), 128), :] = _col_bcast(rows[pl.ds(t, 1), :])
        qloop(C_N // 3, 5, prep)

        MARK('p_wq')
        qsteps(TB - pos[0])

        MARK('p_qproj')
        scale = DH ** -0.5

        def q_cols(i, q):
            for t in range(2):
                qb[pl.ds(m128(i * 256 + t * 128), 128), :] = _col_bcast(
                    q[0:1, t * 128:(t + 1) * 128])

        def qproj(i0):
            def fn(i, q_prev):
                q_cols(jnp.maximum(i + i0 - 1, 0), q_prev)
                w = pairs(wq_v, [24 * g + i + i0 for g in range(D // 8)]).astype(F32)
                w = jnp.concatenate([w[:, 0:8].reshape(D, 128), w[:, 8:16].reshape(D, 128)],
                                    axis=1)
                return jnp.dot(h8, w, precision=lax.Precision.DEFAULT,
                               preferred_element_type=F32) * scale
            return fn
        q = ph_o.every(0, 20, 5, qproj(0), jnp.zeros((8, 256), F32))
        q = ph_o.every(100, 2, 7, qproj(20), q)
        q = ph_o.every(114, 2, 7, qproj(22), q)
        for c in range(LW, NB):
            k0[0](c).start(priority=LO)
        MARK('p_k0')
        ph = Phase(k0, NB, NB, v0)
        ph.run(0, 1)
        q_cols(23, q)
        abuf[...] = jnp.zeros((DH, 128), F32)
        wo_last[...] = pairs(wo_v, [60 * (H - 1) + p for p in range(60)]).astype(F32).reshape(
            G * ND, 8, 128)
        ph.run(1, NB)

        def proj(h, a, out):
            o = jnp.sum(a, axis=1, keepdims=True)
            outs = [out, None]
            for jj in range(G // 2):
                w = pairs(wo_v, [60 * h + jj * ND + p for p in range(ND)]).astype(F32)
                tiles = _groups(w.reshape(16 * ND, 128))
                for e in range(2):
                    j = 2 * jj + e
                    w = jnp.concatenate(tiles[e * ND:(e + 1) * ND], axis=1)
                    t = o[j * 8:(j + 1) * 8] * w
                    outs[e] = t if outs[e] is None else outs[e] + t
            return outs[0] + outs[1]

        def phase_a(h, slot, out, ph, tps, n1):
            q = qb[pl.ds(pl.multiple_of(h * DH, 64), DH), :]

            def body(i, m):
                for u in range(tps):
                    c = tps * i + u
                    s = _tree_sum(_groups(kbuf[slot, c].astype(F32) * q))
                    s = jnp.broadcast_to(jnp.sum(s, axis=0, keepdims=True), (8, 128))
                    sbuf[c] = s
                    m = jnp.maximum(m, s)
                return m
            n0 = NB // tps
            m = ph.run(0, n0, body, jnp.full((8, 128), -jnp.inf, F32))
            ph.run(n0, n0 + n1)
            m = jnp.max(m, axis=1, keepdims=True)
            out = proj(jnp.maximum(h - 1, 0), abuf[...], out)
            ph.run(n0 + n1, n0 + n1 + 3)
            p = jnp.exp(sbuf[...] - m)
            sbuf[...] = p
            l = _tree_sum([p[c] for c in range(NB)])
            inv_l = 1.0 / jnp.sum(l, axis=1, keepdims=True)
            return inv_l, out

        def pv_tile(slot, c, acc):
            p = sbuf[c]
            return acc + vbuf[slot, c].astype(F32) * jnp.concatenate([p] * G, axis=0)

        def pv_done(acc, inv_l):
            return acc * jnp.concatenate([jnp.broadcast_to(inv_l, (8, 128))] * G, axis=0)

        def head(h, out):
            slot = h & 1
            nslot = 1 - slot
            knext = k_stream(h + 1, nslot)
            ph = Phase(v_stream(h, slot), NB, NB, knext)
            inv_l, out = phase_a(h, slot, out, ph, 2, 1)
            ph.run(20, NB)
            ph = Phase(knext, NB, NB, v_stream(h + 1, nslot))
            acc = ph.run(0, NB, lambda c, acc: pv_tile(slot, c, acc), jnp.zeros((DH, 128), F32))
            abuf[...] = pv_done(acc, inv_l)
            return out

        MARK('main')
        out = lax.fori_loop(0, H - 1, head, jnp.zeros((8, D), F32))

        MARK('qk31')
        hl = H - 1
        sl = hl % 2
        slab9(0).start(priority=LO)
        slab9(1).start(priority=LO)
        for b in range(8):
            gb_piece(b).start(priority=LO)
        ph = Phase(v_stream(hl, sl), NB, NB, None)
        inv_l, out = phase_a(hl, sl, out, ph, 4, 3)

        MARK('pv31')
        acc = ph.run(14, 28, lambda i, acc: pv_tile(sl, 2 * i - 27, pv_tile(sl, 2 * i - 28, acc)),
                     jnp.zeros((DH, 128), F32))
        ga = mods[:, 2 * D:3 * D]
        xp = x32 + ga * jnp.sum(out, axis=0, keepdims=True)
        gl = ga * inv_l
        acc = ph.run(28, NB - 1, lambda c, acc: pv_tile(sl, c, acc), acc)
        MARK('wlast')
        ph.run(NB - 1, NB)
        MARK('proj31')
        o = jnp.sum(pv_tile(sl, NB - 1, acc), axis=1, keepdims=True)
        outs = [None, None]
        for j in range(G):
            w = jnp.concatenate([wo_last[j * ND + n] for n in range(ND)], axis=1)
            t = o[j * 8:(j + 1) * 8] * w
            outs[j & 1] = t if outs[j & 1] is None else outs[j & 1] + t
        x1 = xp + gl * jnp.sum(outs[0] + outs[1], axis=0, keepdims=True)
        d1 = x1 - _tile(consts[2:3, :], ND)
        mom = _moments(d1)

        MARK('w9')
        slab9(0).wait()
        MARK('ln2')
        mom = _lane_sum(mom)
        macc = mods[:, 3 * D:]
        for u in range(DB // 8):
            if u == N9:
                MARK('w9b')
                slab9(1).wait()
                MARK('ln2b')
                m1, r1 = _stats(mom)
                z = (d1 - m1) * r1
            s = cols[pl.ds(C_SC * 128 + D - DB + u * 8, 8), :]
            macc = macc + _tile(s, 2 * ND) * wm_v[
                DA - 1, pl.ds(u * 8, 8), pl.ds(3 * D, 2 * D)].astype(F32)
        mod = jnp.sum(macc, axis=0, keepdims=True)
        d2 = z * mod[:, D:] + mod[:, :D]
        m2, r2 = _stats(_lane_sum(_moments(d2)))
        hn = (d2 - m2) * r2

        MARK('mlp')

        def tanh_rows(b, u, hn):
            w1c = cols[pl.ds((C_W1 + b - NZ) * 128 + u * 8, 8), :]
            b1c = cols[pl.ds((C_B1 + b - NZ) * 128 + u * 8, 8), :]
            v = hn * _tile(w1c, ND) + _tile(b1c, ND)
            return jnp.tanh(v * (v * v + CS))

        p2 = hn * hn
        sid = lax.broadcasted_iota(jnp.int32, (8, D), 0)
        phi, plo = _split(jnp.where(sid < 3, p2 * hn, jnp.where(sid < 6, p2, hn)))
        ptop = jnp.where((sid == 1) | (sid == 4) | (sid == 7), plo, phi)
        pbot = jnp.where(sid == 0, hn, jnp.where(sid < 4, 1.0, 0.0))
        pmat = jnp.concatenate([ptop, pbot], axis=0)
        r = None
        nz, nv = 0, NZ
        zs = []
        late = []
        for kind in ORDER:
            if kind == 'V':
                b = nv
                nv += 1
                ts = [tanh_rows(b, u, hn) for u in range(16)]
                t = jnp.concatenate(ts, axis=0)
            elif kind == 'Z':
                zs.append(jnp.dot(acol[len(zs) * 128:(len(zs) + 1) * 128, 0:16], pmat,
                                  precision=lax.Precision.DEFAULT, preferred_element_type=F32))
                continue
            else:
                b = nz
                nz += 1
                t = jnp.tanh(zs[b])
                if kind == 'S':
                    late.append(b)
                    tbuf[len(late)] = t
                    continue
            rb = jnp.dot(lhs[:, b * 128:(b + 1) * 128], t,
                         precision=lax.Precision.DEFAULT, preferred_element_type=F32)
            r = rb if r is None else r + rb
        hl_ = hn + _tile(_tree_sum(_blocks(ts[0])) * 0.0, ND)
        for u in range(16):
            tbuf[0, u * 8:(u + 1) * 8, :] = tanh_rows(NF - 1, u, hl_)

        def gate(accs, bs):
            for b in bs:
                for a in range(DA):
                    s = cols[pl.ds(C_SC * 128 + a * DB + b * 8, 8), :]
                    t = _tile(s, ND) * wm_v[a, pl.ds(b * 8, 8), pl.ds(5 * D, D)].astype(F32)
                    accs[a & 1] = t if accs[a & 1] is None else accs[a & 1] + t
            return accs

        MARK('gbw')
        for b in range(NG1):
            gb_piece(b).wait()
        MARK('gb')
        for k, b in enumerate([NF - 1] + late):
            r = r + jnp.dot(lhs[:, b * 128:(b + 1) * 128], tbuf[k],
                            precision=lax.Precision.DEFAULT, preferred_element_type=F32)
        gacc = gate([None, None], range(NG1))
        y = (hn[0:1] * (r[0:1] + r[1:2] + _tile(consts[0:1, :], ND))
             + (r[2:3] + r[3:4] + _tile(consts[1:2, :], ND)))
        MARK('gbw3')
        for b in range(NG1, 8):
            gb_piece(b).wait()
        MARK('gb3')
        gacc = gate(gacc, range(NG1, 8))
        gb = jnp.sum(gacc[0] + gacc[1], axis=0, keepdims=True)
        o_ref[0] = (x1[0:1] + gb * y).astype(o_ref.dtype)
        MARK(None)

    return kernel


@jax.jit
def pallas_adaLN_cond__sliding_block_cached__mixer_token_mlp__decode_kernel(
    A_x: jax.Array,
    A_k_cache: jax.Array,
    A_v_cache: jax.Array,
    A_wq: jax.Array,
    A_wo: jax.Array,
    B_x: jax.Array,
    B_w1: jax.Array,
    B_b1: jax.Array,
    B_w2: jax.Array,
    B_b2: jax.Array,
    c: jax.Array,
    w_mod: jax.Array,
):
    SK = A_k_cache.shape[2]
    W = min(4096, max(256, SK // 4))
    kt = jnp.swapaxes(A_k_cache, 2, 3).reshape(H * DH, SK)
    vt = jnp.swapaxes(A_v_cache, 2, 3).reshape(H * DH, SK)

    vmem = pltpu.VMEM
    dma = pltpu.SemaphoreType.DMA
    return pl.pallas_call(
        _make_kernel(SK, W),
        out_shape=jax.ShapeDtypeStruct(A_x.shape, A_x.dtype),
        in_specs=[pl.BlockSpec(memory_space=pl.ANY)] * 11,
        out_specs=pl.BlockSpec(memory_space=pltpu.VMEM),
        scratch_shapes=[
            vmem((2, W // 128, DH, 128), BF16), vmem((2, W // 128, DH, 128), BF16),
            vmem((TA, TB, 16, 128), BF16), vmem((TA, TB, 16, 128), BF16),
            vmem((DA, DB, 6 * D), BF16),
            vmem((1, 1, D), BF16), vmem((1, D), BF16),
            vmem((1, F), BF16), vmem((NF, 128), BF16), vmem((1, F), BF16),
            vmem((1,), BF16),
            vmem((H * DH, 128), F32), vmem((C_N, 128), F32), vmem((C_N * 128, 128), F32),
            vmem((8, F), F32), vmem((DH, 128), F32), vmem((W // 128, 8, 128), F32),
            vmem((3, 128), F32), vmem((8, 5 * D), F32),
            vmem((NZ * 128, 128), F32),
            vmem((G * ND, 8, 128), F32), vmem((1 + ORDER.count('S'), 128, D), F32),
            dma((2,)), dma((2,)), dma((64,)), dma((64,)), dma((10,)), dma((6,)),
        ],
        compiler_params=pltpu.CompilerParams(
            vmem_limit_bytes=64 * 1024 * 1024,
            disable_bounds_checks=True,
            disable_semaphore_checks=True,
        ),
    )(A_x, kt, vt, _pair_view(A_wq), _pair_view(A_wo), B_w1,
      B_b1.reshape(NF, 128), B_w2.reshape(1, F), B_b2, c, w_mod.reshape(DA, DB, 6 * D))
```

```python
import math

import jax
import jax.numpy as jnp
from jax import lax
import jax.experimental.pallas as pl
import jax.experimental.pallas.tpu as pltpu

F32 = jnp.float32
BF16 = jnp.bfloat16

D = 640
H = 32
DH = 192
F = 1536
EPS = 1e-5
G = DH // 8
ND = D // 128
NF = F // 128

LO, HI = 1, 0

_C0 = math.sqrt(2.0 / math.pi)
_C1 = 0.044715
KS = (_C0 * _C1) ** (1.0 / 3.0)
CS = _C0 / KS

ORDER = 'ZVZVVRZVRVZRVVS'
NZ = ORDER.count('Z')
NV = NF - NZ
C_W1, C_B1, C_SC, C_N = 0, NV, 2 * NV, 2 * NV + ND
assert C_N % 3 == 0

DA, DB = 10, 64
TA, TB = 15, 128


class _Group:
    def __init__(self, copies):
        self.copies = copies

    def start(self, priority):
        for c in self.copies:
            c.start(priority=priority)

    def wait(self):
        for c in self.copies:
            c.wait()


def _pair_view(w):
    r, c = w.shape
    t = w.reshape(r // 8, 8, c // 128, 128).transpose(0, 2, 1, 3)
    return t.reshape(TA, TB, 16, 128)


def _layernorm(x):
    m = jnp.mean(x, axis=-1, keepdims=True)
    xc = x - m
    v = jnp.mean(xc * xc, axis=-1, keepdims=True)
    return xc * lax.rsqrt(v + EPS)


def _moments(d):
    low = lax.broadcasted_iota(jnp.int32, d.shape, 0) < 4
    return _tree_sum(_blocks(d * jnp.where(low, 1.0, d)))


def _lane_sum(x):
    return jnp.broadcast_to(jnp.sum(x, axis=-1, keepdims=True), x.shape)


def _stats(s):
    s = s * (1.0 / D)
    m1, m2 = jnp.broadcast_to(s[0:1], s.shape), jnp.broadcast_to(s[4:5], s.shape)
    return _tile(m1, ND), _tile(lax.rsqrt(jnp.maximum(m2 - m1 * m1, 0.0) + EPS), ND)


def _col_bcast(row128):
    return jnp.broadcast_to(row128, (128, 128)).T


def _tile(x, n):
    return jnp.concatenate([x] * n, axis=1)


def _tree_sum(parts):
    while len(parts) > 1:
        nxt = [parts[2 * i] + parts[2 * i + 1] for i in range(len(parts) // 2)]
        if len(parts) % 2:
            nxt.append(parts[-1])
        parts = nxt
    return parts[0]


def _split(a):
    hi = a.astype(BF16).astype(F32)
    return [hi, a - hi]


def _stack_rows(xs, n):
    rid = lax.broadcasted_iota(jnp.int32, (n, xs[0].shape[1]), 0)
    out = jnp.zeros(rid.shape, F32)
    for k, x in enumerate(xs):
        out = jnp.where(rid == k, x, out)
    return out


def _blocks(x):
    return [x[:, j * 128:(j + 1) * 128] for j in range(x.shape[1] // 128)]


def _groups(x):
    return [x[j * 8:(j + 1) * 8, :] for j in range(x.shape[0] // 8)]


def _make_kernel(SK, W):
    LH = 14
    KV_HI = 16
    KV_LO = DH - KV_HI
    W0 = SK - W
    NB = W // 128
    assert NB == 32

    def kernel(x_hbm, k_hbm, v_hbm, wq_hbm, wo_hbm, w1_hbm, b1_hbm, w2_hbm, b2_hbm,
               c_hbm, wm_hbm, o_ref,
               kbuf, vbuf, wq_v, wo_v, wm_v, x_v, c_v, w1_v, b1_v, w2_v, b2_v,
               qb, rows, cols, lhs, abuf, sbuf, consts, mods, acol, wo_last, tbuf,
               klo, khi, vlo, vhi, wsem, ssem):
        cp = pltpu.make_async_copy
        m8 = lambda i: pl.multiple_of(i, 8)
        m128 = lambda i: pl.multiple_of(i, 128)
        MARK = lambda name: None

        def kv_stream(src, buf, lo_sem, hi_sem, h, slot, sem_of):
            def piece(c, r0, n, sem):
                return cp(src.at[pl.ds(m8(h * DH + r0), n), pl.ds(m128(W0 + c * 128), 128)],
                          buf.at[slot, c, pl.ds(r0, n), :], sem.at[sem_of(c)])
            return (lambda c: piece(c, 0, KV_LO, lo_sem),
                    lambda c: piece(c, KV_LO, KV_HI, hi_sem))

        k_stream = lambda h, slot: kv_stream(k_hbm, kbuf, klo, khi, h, slot, lambda c: slot)
        v_stream = lambda h, slot: kv_stream(v_hbm, vbuf, vlo, vhi, h, slot,
                                             lambda c: slot * NB + c)

        def w_piece(src, dst, a0, na, b, c0, n, sem):
            idx = (pl.ds(a0, na), pl.ds(m8(b * 8), 8), pl.ds(m128(c0), n))
            return cp(src.at[idx], dst.at[idx], sem)

        def m_piece(b, u, part, kind=None):
            kind = u if kind is None else kind
            na, c0, n = (DA, u * 384, 384) if kind < 5 else (DA - 1, (u - 2) * D, D)
            a0, na = {'all': (0, na), 'lo': (0, na - 1), 'hi': (na - 1, 1)}[part]
            return w_piece(wm_hbm, wm_v, a0, na, b, c0, n, wsem.at[5 if part == 'hi' else 0])

        def pair_stream(src, dst, s):
            def piece(i, a0, na, r0, nr, sem):
                idx = (pl.ds(a0, na), i, pl.ds(r0, nr))
                return cp(src.at[idx], dst.at[idx], sem)
            return (lambda i: _Group([piece(i, 0, TA, 0, 8, wsem.at[s]),
                                      piece(i, 0, TA - 3, 8, 8, wsem.at[s])]),
                    lambda i: piece(i, TA - 3, 3, 8, 8, wsem.at[s + 1]))
        q_stream = pair_stream(wq_hbm, wq_v, 1)
        o_stream = pair_stream(wo_hbm, wo_v, 3)

        N9 = 6

        def slab9(k):
            r = pl.ds(8 * N9, DB - 8 * N9) if k else pl.ds(0, 8 * N9)
            idx = (DA - 1, r, pl.ds(3 * D, 2 * D))
            return cp(wm_hbm.at[idx], wm_v.at[idx], wsem.at[9 if k else 6])

        NG1 = 6
        gb_piece = lambda b: w_piece(wm_hbm, wm_v, 0, DA, b, 5 * D, D,
                                     wsem.at[7 if b < NG1 else 8])

        class Phase:
            def __init__(self, cur, n, ll, nxt):
                self.cur, self.n, self.nxt = cur, n, nxt
                self.ahead = (ll, LH)
                self.edges = {n - ll, n - LH}

            def stepper(self, a, b):
                starts = []
                assert not any(a < e < b for e in self.edges), (a, b)
                for k, prio in ((0, LO), (1, HI)):
                    ahead = self.ahead[k]
                    if b <= self.n - ahead:
                        starts.append((self.cur[k], ahead, prio))
                    elif self.nxt is not None:
                        starts.append((self.nxt[k], ahead - self.n, prio))

                def step(i):
                    self.cur[0](i).wait()
                    for piece, off, prio in starts:
                        piece(i + off).start(priority=prio)
                    self.cur[1](i).wait()
                return step

            def run(self, a, b, fn=None, init=0):
                cuts = sorted({a, b} | {e for e in self.edges if a < e < b})
                for lo, hi in zip(cuts[:-1], cuts[1:]):
                    step = self.stepper(lo, hi)

                    def body(i, c):
                        step(i)
                        return c if fn is None else fn(i, c)
                    init = body(lo, init) if hi - lo == 1 else lax.fori_loop(lo, hi, body, init)
                return init

            def every(self, a, n, k, fn, init=0):
                step = self.stepper(a, a + n * k)

                def body(j, c):
                    step(a + k * j)
                    c = fn(j, c)

                    def rest(u, z):
                        step(a + k * j + u)
                        return z
                    lax.fori_loop(1, k, rest, 0)
                    return c
                return lax.fori_loop(0, n, body, init)

        def pairs(ref, ps):
            return jnp.stack([ref[p >> 7, p & 127] for p in ps])

        MARK('p_issue')
        for u in range(7):
            m_piece(0, u, 'all').start(priority=LO)
        smalls = [cp(s, d, ssem.at[n]) for n, (s, d) in enumerate(
            [(c_hbm, c_v), (x_hbm, x_v), (w1_hbm, w1_v), (b1_hbm, b1_v), (w2_hbm, w2_v),
             (b2_hbm, b2_v)])]
        for s in smalls:
            s.start(priority=HI)

        for b in range(1, 4):
            for u in range(7):
                m_piece(b, u, 'lo').start(priority=LO)
        for u0, u1 in ((0, 5), (5, 7)):
            def body(u, c):
                qb[pl.ds(m128(u * 768), 768), :] = jnp.zeros((768, 128), F32)
                m_piece(1, u, 'hi', u0).start(priority=HI)
                return c
            lax.fori_loop(u0, u1, body, 0)

        MARK('p_ma')
        for b0, b1 in ((0, 1), (1, 4), (4, 6), (6, 8)):
            def body(b, c):
                for u in range(7):
                    m_piece(b, u, 'lo' if b0 else 'all').wait()
                    lo = m_piece(b + 4, u, 'lo') if b0 < 4 else q_stream[0](7 * (b - 4) + u)
                    hi = m_piece(b + 2, u, 'hi') if b0 < 6 else q_stream[1](7 * (b - 6) + u)
                    lo.start(priority=LO)
                    hi.start(priority=HI)
                    if b0:
                        m_piece(b, u, 'hi').wait()
                return c
            lax.fori_loop(b0, b1, body, 0)
        for s in smalls:
            s.wait()

        MARK('p_moda')
        k0, v0 = k_stream(0, 0), v_stream(0, 0)
        LW = 28
        ph_q = Phase(q_stream, TB, LW, o_stream)
        ph_o = Phase(o_stream, TB, LW, k0)
        pos = [0]

        def qsteps(n):
            ph_q.run(pos[0], pos[0] + n)
            pos[0] += n

        def qloop(n, k, fn):
            def body(j, c):
                fn(j)
                return c
            ph_q.every(pos[0], n, k, body)
            pos[0] += n * k

        c32 = c_v[...].astype(F32)
        sc = (c32 * jax.nn.sigmoid(c32)).astype(BF16)
        sc16 = jnp.broadcast_to(sc, (16, D))
        w2h = w2_v[...].astype(F32) * 0.5
        w1f = w1_v[...].astype(F32)
        b1f = b1_v[...].astype(F32)
        scf = sc.astype(F32)
        for i in range(NV):
            rows[C_W1 + i:C_W1 + i + 1, :] = w1f[:, (NZ + i) * 128:(NZ + i + 1) * 128] * KS
        rows[C_B1:C_B1 + NV, :] = b1f[NZ:] * KS
        for i in range(ND):
            rows[C_SC + i:C_SC + i + 1, :] = scf[:, i * 128:(i + 1) * 128]

        def mod_a(i):
            c = pl.ds(m128(i * 384), 384)
            mods[:, c] = jnp.dot(sc16, wm_v[:, :, c].reshape(D, 384),
                                 preferred_element_type=F32)[0:8]
        qloop(5, 4, mod_a)

        def mod_b(i):
            c = pl.ds(m128(3 * D + i * 256), 256)
            mods[:, c] = jnp.dot(sc16[:, :D - DB], wm_v[0:DA - 1, :, c].reshape(D - DB, 256),
                                 preferred_element_type=F32)[0:8]
        qloop(5, 3, mod_b)

        x32 = x_v[0].astype(F32)
        h8 = (_layernorm(x32) * (1.0 + mods[:, D:2 * D]) + mods[:, :D]).astype(BF16).astype(F32)
        sb = mods[:, 3 * D:4 * D]
        base = jnp.concatenate([sb - jnp.mean(sb, axis=1, keepdims=True), 1.0 + mods[:, 4 * D:]],
                               axis=1)
        mods[:, 3 * D:] = jnp.where(lax.broadcasted_iota(jnp.int32, base.shape, 0) == 0, base, 0.0)
        qsteps(4)

        b1row = jnp.concatenate([b1f[i:i + 1, :] for i in range(NF)], axis=1)
        pw = w1f * w2h
        pb = b1row * w2h
        lhs[...] = _stack_rows(_split(pw) + _split(pb), 8)
        sum_w = jnp.sum(pw, axis=1, keepdims=True)
        sum_b = jnp.sum(pb, axis=1, keepdims=True) + b2_v[...].astype(F32).reshape(1, 1)
        consts[0:1, :] = jnp.broadcast_to(sum_w, (1, 128))
        consts[1:2, :] = jnp.broadcast_to(sum_b, (1, 128))
        qsteps(4)

        al = w1f[:, :NZ * 128] * KS
        be = b1row[:, :NZ * 128] * KS
        a3h, a3l = _split(al * al * al)
        a2h, a2l = _split(3.0 * al * al * be)
        a1h, a1l = _split(al * (3.0 * be * be + CS))
        a0h, a0l = _split(be * (be * be + CS))
        at = _stack_rows([a3h, a3h, a3l, a2h, a2h, a2l, a1h, a1h, a1l, a0h] + _split(a0l), 16)
        for b in range(NZ):
            acol[b * 128:(b + 1) * 128, :] = jnp.concatenate(
                [at[:, b * 128:(b + 1) * 128], jnp.zeros((112, 128), F32)], axis=0).T
        qsteps(3)

        MARK('p_prep')

        def prep(i):
            for u in range(3):
                t = 3 * i + u
                cols[pl.ds(m128(t * 128), 128), :] = _col_bcast(rows[pl.ds(t, 1), :])
        qloop(C_N // 3, 5, prep)

        MARK('p_wq')
        qsteps(TB - pos[0])

        MARK('p_qproj')
        scale = DH ** -0.5

        def q_cols(i, q):
            for t in range(2):
                qb[pl.ds(m128(i * 256 + t * 128), 128), :] = _col_bcast(
                    q[0:1, t * 128:(t + 1) * 128])

        def qproj(i0):
            def fn(i, q_prev):
                q_cols(jnp.maximum(i + i0 - 1, 0), q_prev)
                w = pairs(wq_v, [24 * g + i + i0 for g in range(D // 8)]).astype(F32)
                w = jnp.concatenate([w[:, 0:8].reshape(D, 128), w[:, 8:16].reshape(D, 128)],
                                    axis=1)
                return jnp.dot(h8, w, precision=lax.Precision.DEFAULT,
                               preferred_element_type=F32) * scale
            return fn
        q = ph_o.every(0, 20, 5, qproj(0), jnp.zeros((8, 256), F32))
        q = ph_o.every(100, 2, 7, qproj(20), q)
        q = ph_o.every(114, 2, 7, qproj(22), q)
        for c in range(LW, NB):
            k0[0](c).start(priority=LO)
        MARK('p_k0')
        ph = Phase(k0, NB, NB, v0)
        ph.run(0, 1)
        q_cols(23, q)
        abuf[...] = jnp.zeros((DH, 128), F32)
        wo_last[...] = pairs(wo_v, [60 * (H - 1) + p for p in range(60)]).astype(F32).reshape(
            G * ND, 8, 128)
        ph.run(1, NB)

        def proj(h, a, out):
            o = jnp.sum(a, axis=1, keepdims=True)
            outs = [out, None]
            for jj in range(G // 2):
                w = pairs(wo_v, [60 * h + jj * ND + p for p in range(ND)]).astype(F32)
                tiles = _groups(w.reshape(16 * ND, 128))
                for e in range(2):
                    j = 2 * jj + e
                    w = jnp.concatenate(tiles[e * ND:(e + 1) * ND], axis=1)
                    t = o[j * 8:(j + 1) * 8] * w
                    outs[e] = t if outs[e] is None else outs[e] + t
            return outs[0] + outs[1]

        def phase_a(h, slot, out, ph, tps, n1):
            q = qb[pl.ds(pl.multiple_of(h * DH, 64), DH), :]

            def body(i, m):
                for u in range(tps):
                    c = tps * i + u
                    s = _tree_sum(_groups(kbuf[slot, c].astype(F32) * q))
                    s = jnp.broadcast_to(jnp.sum(s, axis=0, keepdims=True), (8, 128))
                    sbuf[c] = s
                    m = jnp.maximum(m, s)
                return m
            n0 = NB // tps
            m = ph.run(0, n0, body, jnp.full((8, 128), -jnp.inf, F32))
            ph.run(n0, n0 + n1)
            m = jnp.max(m, axis=1, keepdims=True)
            out = proj(jnp.maximum(h - 1, 0), abuf[...], out)
            ph.run(n0 + n1, n0 + n1 + 3)
            p = jnp.exp(sbuf[...] - m)
            sbuf[...] = p
            l = _tree_sum([p[c] for c in range(NB)])
            inv_l = 1.0 / jnp.sum(l, axis=1, keepdims=True)
            return inv_l, out

        def pv_tile(slot, c, acc):
            p = sbuf[c]
            return acc + vbuf[slot, c].astype(F32) * jnp.concatenate([p] * G, axis=0)

        def pv_done(acc, inv_l):
            return acc * jnp.concatenate([jnp.broadcast_to(inv_l, (8, 128))] * G, axis=0)

        def head(h, out):
            slot = h & 1
            nslot = 1 - slot
            knext = k_stream(h + 1, nslot)
            ph = Phase(v_stream(h, slot), NB, NB, knext)
            inv_l, out = phase_a(h, slot, out, ph, 2, 1)
            ph.run(20, NB)
            ph = Phase(knext, NB, NB, v_stream(h + 1, nslot))
            acc = ph.run(0, NB, lambda c, acc: pv_tile(slot, c, acc), jnp.zeros((DH, 128), F32))
            abuf[...] = pv_done(acc, inv_l)
            return out

        MARK('main')
        out = lax.fori_loop(0, H - 1, head, jnp.zeros((8, D), F32))

        MARK('qk31')
        hl = H - 1
        sl = hl % 2
        slab9(0).start(priority=LO)
        slab9(1).start(priority=LO)
        for b in range(8):
            gb_piece(b).start(priority=LO)
        ph = Phase(v_stream(hl, sl), NB, NB, None)
        inv_l, out = phase_a(hl, sl, out, ph, 4, 3)
        ga = mods[:, 2 * D:3 * D]
        xp = x32 + ga * jnp.sum(out, axis=0, keepdims=True)
        dp = xp - jnp.mean(xp, axis=1, keepdims=True)
        gl = ga * inv_l

        MARK('pv31')
        acc = ph.run(14, 28, lambda i, acc: pv_tile(sl, 2 * i - 27, pv_tile(sl, 2 * i - 28, acc)),
                     jnp.zeros((DH, 128), F32))
        acc = ph.run(28, NB - 1, lambda c, acc: pv_tile(sl, c, acc), acc)
        MARK('wlast')
        ph.run(NB - 1, NB)
        MARK('proj31')
        o = jnp.sum(pv_tile(sl, NB - 1, acc), axis=1, keepdims=True)
        outs = [None, None]
        for j in range(G):
            w = jnp.concatenate([wo_last[j * ND + n] for n in range(ND)], axis=1)
            t = o[j * 8:(j + 1) * 8] * w
            outs[j & 1] = t if outs[j & 1] is None else outs[j & 1] + t
        upd = gl * jnp.sum(outs[0] + outs[1], axis=0, keepdims=True)
        d1 = dp + upd
        mom = _moments(d1)
        x1 = xp + upd

        MARK('w9')
        slab9(0).wait()
        MARK('ln2')
        mom = _lane_sum(mom)
        macc = mods[:, 3 * D:]
        for u in range(DB // 8):
            if u == N9:
                MARK('w9b')
                slab9(1).wait()
                MARK('ln2b')
                m1, r1 = _stats(mom)
                z = (d1 - m1) * r1
            s = cols[pl.ds(C_SC * 128 + D - DB + u * 8, 8), :]
            macc = macc + _tile(s, 2 * ND) * wm_v[
                DA - 1, pl.ds(u * 8, 8), pl.ds(3 * D, 2 * D)].astype(F32)
        mod = jnp.sum(macc, axis=0, keepdims=True)
        d2 = z * mod[:, D:] + mod[:, :D]
        m2, r2 = _stats(_lane_sum(_moments(d2)))
        hn = (d2 - m2) * r2

        MARK('mlp')

        def tanh_rows(b, u, hn):
            w1c = cols[pl.ds((C_W1 + b - NZ) * 128 + u * 8, 8), :]
            b1c = cols[pl.ds((C_B1 + b - NZ) * 128 + u * 8, 8), :]
            v = hn * _tile(w1c, ND) + _tile(b1c, ND)
            return jnp.tanh(v * (v * v + CS))

        p2 = hn * hn
        sid = lax.broadcasted_iota(jnp.int32, (8, D), 0)
        phi, plo = _split(jnp.where(sid < 3, p2 * hn, jnp.where(sid < 6, p2, hn)))
        ptop = jnp.where((sid == 1) | (sid == 4) | (sid == 7), plo, phi)
        pbot = jnp.where(sid == 0, hn, jnp.where(sid < 4, 1.0, 0.0))
        pmat = jnp.concatenate([ptop, pbot], axis=0)
        r = None
        nz, nv = 0, NZ
        zs = []
        late = []
        for kind in ORDER:
            if kind == 'V':
                b = nv
                nv += 1
                ts = [tanh_rows(b, u, hn) for u in range(16)]
                t = jnp.concatenate(ts, axis=0)
            elif kind == 'Z':
                zs.append(jnp.dot(acol[len(zs) * 128:(len(zs) + 1) * 128, 0:16], pmat,
                                  precision=lax.Precision.DEFAULT, preferred_element_type=F32))
                continue
            else:
                b = nz
                nz += 1
                t = jnp.tanh(zs[b])
                if kind == 'S':
                    late.append(b)
                    tbuf[len(late)] = t
                    continue
            rb = jnp.dot(lhs[:, b * 128:(b + 1) * 128], t,
                         precision=lax.Precision.DEFAULT, preferred_element_type=F32)
            r = rb if r is None else r + rb
        hl_ = hn + _tile(_tree_sum(_blocks(ts[0])) * 0.0, ND)
        for u in range(16):
            tbuf[0, u * 8:(u + 1) * 8, :] = tanh_rows(NF - 1, u, hl_)

        def gate(accs, bs):
            for b in bs:
                for a in range(DA):
                    s = cols[pl.ds(C_SC * 128 + a * DB + b * 8, 8), :]
                    t = _tile(s, ND) * wm_v[a, pl.ds(b * 8, 8), pl.ds(5 * D, D)].astype(F32)
                    accs[a & 1] = t if accs[a & 1] is None else accs[a & 1] + t
            return accs

        MARK('gbw')
        for b in range(NG1):
            gb_piece(b).wait()
        MARK('gb')
        for k, b in enumerate([NF - 1] + late):
            r = r + jnp.dot(lhs[:, b * 128:(b + 1) * 128], tbuf[k],
                            precision=lax.Precision.DEFAULT, preferred_element_type=F32)
        gacc = gate([None, None], range(NG1))
        y = (hn[0:1] * (r[0:1] + r[1:2] + _tile(consts[0:1, :], ND))
             + (r[2:3] + r[3:4] + _tile(consts[1:2, :], ND)))
        MARK('gbw3')
        for b in range(NG1, 8):
            gb_piece(b).wait()
        MARK('gb3')
        gacc = gate(gacc, range(NG1, 8))
        gb = jnp.sum(gacc[0] + gacc[1], axis=0, keepdims=True)
        o_ref[0] = (x1[0:1] + gb * y).astype(o_ref.dtype)
        MARK(None)

    return kernel


@jax.jit
def pallas_adaLN_cond__sliding_block_cached__mixer_token_mlp__decode_kernel(
    A_x: jax.Array,
    A_k_cache: jax.Array,
    A_v_cache: jax.Array,
    A_wq: jax.Array,
    A_wo: jax.Array,
    B_x: jax.Array,
    B_w1: jax.Array,
    B_b1: jax.Array,
    B_w2: jax.Array,
    B_b2: jax.Array,
    c: jax.Array,
    w_mod: jax.Array,
):
    SK = A_k_cache.shape[2]
    W = min(4096, max(256, SK // 4))
    kt = jnp.swapaxes(A_k_cache, 2, 3).reshape(H * DH, SK)
    vt = jnp.swapaxes(A_v_cache, 2, 3).reshape(H * DH, SK)

    vmem = pltpu.VMEM
    dma = pltpu.SemaphoreType.DMA
    return pl.pallas_call(
        _make_kernel(SK, W),
        out_shape=jax.ShapeDtypeStruct(A_x.shape, A_x.dtype),
        in_specs=[pl.BlockSpec(memory_space=pl.ANY)] * 11,
        out_specs=pl.BlockSpec(memory_space=pltpu.VMEM),
        scratch_shapes=[
            vmem((2, W // 128, DH, 128), BF16), vmem((2, W // 128, DH, 128), BF16),
            vmem((TA, TB, 16, 128), BF16), vmem((TA, TB, 16, 128), BF16),
            vmem((DA, DB, 6 * D), BF16),
            vmem((1, 1, D), BF16), vmem((1, D), BF16),
            vmem((1, F), BF16), vmem((NF, 128), BF16), vmem((1, F), BF16),
            vmem((1,), BF16),
            vmem((H * DH, 128), F32), vmem((C_N, 128), F32), vmem((C_N * 128, 128), F32),
            vmem((8, F), F32), vmem((DH, 128), F32), vmem((W // 128, 8, 128), F32),
            vmem((2, 128), F32), vmem((8, 5 * D), F32),
            vmem((NZ * 128, 128), F32),
            vmem((G * ND, 8, 128), F32), vmem((1 + ORDER.count('S'), 128, D), F32),
            dma((2,)), dma((2,)), dma((64,)), dma((64,)), dma((10,)), dma((6,)),
        ],
        compiler_params=pltpu.CompilerParams(
            vmem_limit_bytes=64 * 1024 * 1024,
            disable_bounds_checks=True,
            disable_semaphore_checks=True,
        ),
    )(A_x, kt, vt, _pair_view(A_wq), _pair_view(A_wo), B_w1,
      B_b1.reshape(NF, 128), B_w2.reshape(1, F), B_b2, c, w_mod.reshape(DA, DB, 6 * D))
```
